```python
import jax
import jax.numpy as jnp

def _softmax(x, axis=-1):
    return jax.nn.softmax(x, axis=axis)

def _gelu(x):
    return jax.nn.gelu(x, approximate=True)

def _silu(x):
    return jax.nn.silu(x)

def _sigmoid(x):
    return jax.nn.sigmoid(x)

def _layernorm(x, axis=-1, eps=1e-05):
    m = jnp.mean(x, axis=axis, keepdims=True)
    v = jnp.var(x, axis=axis, keepdims=True)
    return (x - m) / jnp.sqrt(v + eps)

def _scatter_add(tgt, idx, src, axis=0):
    return tgt.at[idx].add(src)

def _segment_sum(src, seg, n):
    return jax.ops.segment_sum(src, seg, n)

class _Rng:

    def __init__(self, key):
        self._k = key

    def _next(self):
        self._k, sub = jax.random.split(self._k)
        return sub

    def normal(self, shape):
        return jax.random.normal(self._next(), shape, dtype=jnp.bfloat16)

    def randint(self, lo, hi, shape):
        return jax.random.randint(self._next(), shape, lo, hi, dtype=jnp.int32)

    def uniform(self, shape, lo=0.0, hi=1.0):
        return jax.random.uniform(self._next(), shape, jnp.bfloat16, lo, hi)

    def permutation(self, n):
        return jax.random.permutation(self._next(), n)
kernel_name = 'adaLN_cond__memory_aug_recurrent_mem_tr__mixer_s_mlp__prompt'

def setup_inputs():
    _rng = _Rng(jax.random.key(int.from_bytes(__import__("os").urandom(4), "little")))
    _w = lambda a: (lambda t: t.astype(jnp.bfloat16) if jnp.issubdtype(t.dtype, jnp.floating) else t)(jnp.asarray(a))

    def _A_setup():
        B, S, Dm = (1, 2048, 1024)
        H, Dh = (32, 128)
        M, seg = (8, 32)
        seg = min(seg, S)
        S = S // seg * seg
        return {'x': _w((lambda *s: _rng.normal(s) * 0.05)(B, S, Dm)), 'mem0': _w((lambda *s: _rng.normal(s) * 0.05)(B, M, Dm)), 'Wq': _w((lambda *s: _rng.normal(s) * 0.05)(Dm, H, Dh) * Dm ** (-0.5)), 'Wk': _w((lambda *s: _rng.normal(s) * 0.05)(Dm, H, Dh) * Dm ** (-0.5)), 'Wv': _w((lambda *s: _rng.normal(s) * 0.05)(Dm, H, Dh) * Dm ** (-0.5)), 'Wo': _w((lambda *s: _rng.normal(s) * 0.05)(H, Dh, Dm) * (H * Dh) ** (-0.5)), 'seg_len': seg}
    _A_in = _A_setup()

    def _B_setup():
        B, S, D, F = (1, 2048, 1024, 3584)
        return {'x': _w((lambda *s: _rng.normal(s) * 0.05)(B, S, D)), 'w1': _w((lambda *s: _rng.normal(s) * 0.05)(D, D) * D ** (-0.5)), 'w2': _w((lambda *s: _rng.normal(s) * 0.05)(D, D) * D ** (-0.5)), 'w3': _w((lambda *s: _rng.normal(s) * 0.05)(D, F) * D ** (-0.5)), 'w4': _w((lambda *s: _rng.normal(s) * 0.05)(F, D) * F ** (-0.5))}
    _B_in = _B_setup()
    return {'A_x': _A_in['x'], 'A_mem0': _A_in['mem0'], 'A_Wq': _A_in['Wq'], 'A_Wk': _A_in['Wk'], 'A_Wv': _A_in['Wv'], 'A_Wo': _A_in['Wo'], 'A_seg_len': _A_in['seg_len'], 'B_x': _B_in['x'], 'B_w1': _B_in['w1'], 'B_w2': _B_in['w2'], 'B_w3': _B_in['w3'], 'B_w4': _B_in['w4'], 'c': _w((lambda *s: _rng.normal(s) * 0.05)(1, 1024)), 'w_mod': _w((lambda *s: _rng.normal(s) * 0.05)(1024, 6 * 1024) * 1024 ** (-0.5))}

def reference(A_x, A_mem0, A_Wq, A_Wk, A_Wv, A_Wo, A_seg_len, B_x, B_w1, B_w2, B_w3, B_w4, c, w_mod):

    def _A_ref(x, mem0, Wq, Wk, Wv, Wo, seg_len):
        B, S, Dm = x.shape
        H, Dh = (Wq.shape[1], Wq.shape[2])
        M = mem0.shape[1]
        scale = Dh ** (-0.5)
        n_seg = S // seg_len
        L = M + seg_len
        idx = jnp.arange(L)
        mask = (idx[:, None] < M) | (idx[:, None] >= idx[None, :])
        mem = mem0
        outs = []
        for s in range(n_seg):
            xs = x[:, s * seg_len:(s + 1) * seg_len, :].copy()
            h = jnp.concatenate([mem, xs], axis=1)
            q = jnp.einsum('btd,dhe->bhte', h, Wq)
            k = jnp.einsum('btd,dhe->bhte', h, Wk)
            v = jnp.einsum('btd,dhe->bhte', h, Wv)
            scores = jnp.einsum('bhqe,bhke->bhqk', q, k) * scale
            scores = jnp.where(mask[None, None], scores, -1000000000.0)
            p = _softmax(scores, axis=-1)
            o = jnp.einsum('bhqk,bhke->bhqe', p, v)
            o = jnp.einsum('bhte,hed->btd', o, Wo)
            mem = o[:, :M, :].copy()
            outs.append(o[:, M:, :])
        return jnp.concatenate(outs, axis=1)

    def _B_ref(x, w1, w2, w3, w4):
        B, S, D = x.shape
        h = _gelu(_layernorm(x, axis=-1) @ w1)
        c = D // 4
        g0 = jnp.pad(h[:, :, 0 * c:1 * c], ((0, 0), (1, 0), (0, 0)))[:, :S, :]
        g1 = jnp.pad(h[:, :, 1 * c:2 * c], ((0, 0), (0, 1), (0, 0)))[:, 1:, :]
        g2 = jnp.pad(h[:, :, 2 * c:3 * c], ((0, 0), (2, 0), (0, 0)))[:, :S, :]
        g3 = jnp.pad(h[:, :, 3 * c:], ((0, 0), (0, 2), (0, 0)))[:, 2:, :]
        hs = jnp.concatenate([g0, g1, g2, g3], axis=-1) @ w2
        x1 = x + hs
        h2 = _gelu(_layernorm(x1, axis=-1) @ w3) @ w4
        return x1 + h2
    x = A_x
    mod = (_silu(c) @ w_mod).reshape(c.shape[0], 6, 1, -1)
    sa, ca, ga, sb, cb, gb = (mod[:, 0].copy(), mod[:, 1].copy(), mod[:, 2].copy(), mod[:, 3].copy(), mod[:, 4].copy(), mod[:, 5].copy())
    h = _layernorm(x, axis=-1) * (1 + ca) + sa
    x = x + ga * _A_ref(h, A_mem0, A_Wq, A_Wk, A_Wv, A_Wo, A_seg_len)
    h = _layernorm(x, axis=-1) * (1 + cb) + sb
    x = x + gb * _B_ref(h, B_w1, B_w2, B_w3, B_w4)
    return x
```

```python
import functools
import math

import jax
import jax.numpy as jnp
import numpy as np
import jax.experimental.pallas as pl
import jax.experimental.pallas.tpu as pltpu

F32 = jnp.float32
BF16 = jnp.bfloat16
U32 = jnp.uint32

LN_EPS = 1e-5
MASK_FILL = -1000000000.0
NB = 8
CH = 256
HALO = 8


def _dot(a, b):
    return jnp.dot(a, b, preferred_element_type=F32)


def _dot_nt(a, b):
    return jax.lax.dot_general(a, b, (((1,), (1,)), ((), ())), preferred_element_type=F32)


def _layernorm(x):
    m = jnp.mean(x, axis=-1, keepdims=True)
    d = x - m
    v = jnp.mean(d * d, axis=-1, keepdims=True)
    return d * jax.lax.rsqrt(v + LN_EPS)


def _gelu(x):
    k0 = math.sqrt(2.0 / math.pi)
    t = jnp.tanh(x * (k0 + (k0 * 0.044715) * (x * x)))
    hx = 0.5 * x
    return hx + hx * t


def _rows(v, n):
    return jnp.concatenate([v] * (n // 8), axis=0) if n > 8 else v


def _kernel(x_hbm, mem0_ref, wq_hbm, wk_hbm, wv_hbm, wo_hbm, w1_hbm, w2_hbm, w3_hbm, w4_hbm,
            c_ref, wmod_hbm, out_hbm,
            wqkv, wo_s, w1_s, w2_s, w3_s, w4_s, wmod_s, x_s, xb_s, hb_s, qkvb, xa_s, h_s, g_s,
            mod_s, fill_s, lhs_s, o_s, out_s,
            sem_qkv, sem_wo, sem_misc, sem_out,
            *, nseg, seg, nmem, dm, nh, dh):
    hp_n = nh // 2
    kt_n = dm // 128
    scale = dh ** -0.5
    w_u32 = [w.bitcast(U32) for w in (wq_hbm, wk_hbm, wv_hbm)]
    wo_u32 = wo_hbm.bitcast(U32)

    def qkv_copy(w, hp):
        return pltpu.make_async_copy(w_u32[w].at[:, hp, :], wqkv.at[w, hp], sem_qkv.at[w, hp])

    def wo_copy(n):
        return pltpu.make_async_copy(wo_u32.at[:, pl.ds(pl.multiple_of(n * 128, 128), 128)],
                                     wo_s.at[n], sem_wo.at[n])

    cp_mod0 = pltpu.make_async_copy(wmod_hbm.at[:, 0:2 * dm], wmod_s.at[:, 0:2 * dm], sem_misc.at[0])
    cp_xb = pltpu.make_async_copy(x_hbm.at[:, 0:NB, :], xb_s, sem_misc.at[1])
    cp_x = pltpu.make_async_copy(x_hbm, x_s, sem_misc.at[2])
    cp_mod1 = pltpu.make_async_copy(wmod_hbm.at[:, 2 * dm:], wmod_s.at[:, 2 * dm:], sem_misc.at[3])
    cp_w1 = pltpu.make_async_copy(w1_hbm, w1_s, sem_misc.at[4])
    cp_w2 = pltpu.make_async_copy(w2_hbm, w2_s, sem_misc.at[5])
    cp_w3 = pltpu.make_async_copy(w3_hbm, w3_s, sem_misc.at[6])
    cp_w4 = pltpu.make_async_copy(w4_hbm, w4_s, sem_misc.at[7])

    cp_xb.start()
    cp_mod0.start()
    for w in range(3):
        qkv_copy(w, 0).start()

    def head_pos(i):
        head = jnp.where(i < 2 * seg, i // seg, (i - 2 * seg) // NB)
        r = i % seg
        pos = jnp.where(i < 2 * seg, jnp.where(r < nmem, r, r + NB), nmem + i % NB)
        return head, pos

    nq = 2 * (seg + NB)
    qh, qp = head_pos(jax.lax.broadcasted_iota(jnp.int32, (nq, nq), 0))
    kh, kp = head_pos(jax.lax.broadcasted_iota(jnp.int32, (nq, nq), 1))
    visible = (qp < nmem) | (qp >= kp)
    fill_s[...] = jnp.where(qh == kh, jnp.where(visible, 0.0, MASK_FILL / scale), -jnp.inf).astype(F32)
    zero_halo = jnp.zeros((kt_n, HALO, 128), F32)
    g_s[:, 0:HALO, :] = zero_halo
    g_s[:, HALO + nseg * seg:, :] = zero_halo

    cv = c_ref[...].astype(F32)
    sc = jnp.broadcast_to(cv * jax.nn.sigmoid(cv), (16, dm)).astype(BF16)
    cp_xb.wait()
    ln_b = _layernorm(xb_s[...].astype(F32).reshape(nseg * NB, dm))
    cp_mod0.wait()
    for w in range(3):
        qkv_copy(w, 1).start()
    sa = _dot(sc, wmod_s[:, 0:dm])[0:8]
    ca1 = 1.0 + _dot(sc, wmod_s[:, dm:2 * dm])[0:8]
    mod_s[0] = sa
    mod_s[1] = ca1
    hb_s[...] = (ln_b * _rows(ca1, nseg * NB) + _rows(sa, nseg * NB)).astype(BF16)

    def head_w(w, hp, j):
        return jnp.concatenate(
            [pltpu.bitcast(wqkv[w, hp, pl.ds(128 * k + 64 * j, 64), :], BF16) for k in range(kt_n)], axis=0)

    def bulk_body(hp, carry):
        for w in range(3):
            qkv_copy(w, hp).wait()

        @pl.when(hp + 2 < hp_n)
        def _():
            for w in range(3):
                qkv_copy(w, hp + 2).start()

        @pl.when(hp < kt_n)
        def _():
            wo_copy(hp).start()

        @pl.when(hp == kt_n)
        def _():
            cp_x.start()

        hb = hb_s[...]
        for w in range(3):
            for k in range(kt_n):
                a = wqkv[w, hp, pl.ds(128 * k, 64, stride=2), :]
                b = wqkv[w, hp, pl.ds(128 * k + 1, 64, stride=2), :]
                wqkv[w, hp, pl.ds(128 * k, 64), :] = (a & 0xFFFF) | (b << 16)
                wqkv[w, hp, pl.ds(128 * k + 64, 64), :] = (a >> 16) | (b & np.uint32(0xFFFF0000))
            ra = _dot(hb, head_w(w, hp, 0)).reshape(nseg, NB, dh)
            rb = _dot(hb, head_w(w, hp, 1)).reshape(nseg, NB, dh)
            qkvb[w, hp] = jnp.concatenate([ra, rb], axis=1).astype(BF16)
        return carry

    jax.lax.fori_loop(0, hp_n, bulk_body, 0)

    for n in range(kt_n):
        wo_copy(n).wait()
    cp_x.wait()
    cp_mod1.start()
    cp_w1.start()
    cp_w2.start()
    cp_w3.start()
    cp_w4.start()

    def seg_h(s):
        xs = x_s[s].astype(F32)[NB:]
        return _layernorm(xs) * _rows(mod_s[1], seg - NB) + _rows(mod_s[0], seg - NB)

    lhs_s[...] = jnp.concatenate([mem0_ref[...].astype(F32), seg_h(0)], axis=0).astype(BF16)
    exp_c = scale * math.log2(math.e)

    def step_body(s, carry):
        a = lhs_s[...]
        h_next = seg_h(jnp.minimum(s + 1, nseg - 1))
        for hp in range(hp_n):
            q, k, v = [
                jnp.concatenate([_dot(a, head_w(w, hp, 0)).astype(BF16),
                                 _dot(a, head_w(w, hp, 1)).astype(BF16),
                                 qkvb[w, hp, s]], axis=0)
                for w in range(3)]
            fill = fill_s[...]
            sco = jnp.where(fill == 0.0, _dot_nt(q, k), fill)
            e = jnp.exp2((sco - jnp.max(sco, axis=-1, keepdims=True)) * exp_c)
            p = e * (1.0 / jnp.sum(e, axis=-1, keepdims=True))
            o = _dot(p.astype(BF16), v).astype(BF16)
            o_s[:, (2 * hp) * dh:(2 * hp + 1) * dh] = o[0:seg]
            o_s[:, (2 * hp + 1) * dh:(2 * hp + 2) * dh] = o[seg:2 * seg]
            qkvb[0, hp, s] = o[2 * seg:]
        half = nh * dh // 2
        acc = None
        for part in range(2):
            lo = o_s[:, part * half:(part + 1) * half]
            r = jnp.concatenate(
                [_dot(lo, pltpu.bitcast(wo_s[n, part * half // 2:(part + 1) * half // 2, :], BF16))
                 for n in range(kt_n)], axis=1)
            acc = r if acc is None else acc + r
        xa_s[s, NB:, :] = acc[nmem:]
        lhs_s[...] = jnp.concatenate([acc[0:nmem], h_next], axis=0).astype(BF16)
        return carry

    jax.lax.fori_loop(0, nseg, step_body, 0)

    cp_mod1.wait()
    for i in range(2, 6):
        r = _dot(sc, wmod_s[:, i * dm:(i + 1) * dm])[0:8]
        mod_s[i] = 1.0 + r if i == 4 else r
    cp_w1.wait()
    cp_w2.wait()
    cp_w3.wait()
    cp_w4.wait()

    spc = CH // seg
    nch = nseg // spc

    def stage_a(ci, carry):
        s0 = pl.multiple_of(ci * spc, spc)
        parts = []
        for hp in range(hp_n):
            ob = qkvb[0, hp, pl.ds(s0, spc)].astype(F32)
            parts.append(ob[:, 0:NB, :].reshape(spc * NB, dh).astype(BF16))
            parts.append(ob[:, NB:, :].reshape(spc * NB, dh).astype(BF16))
        lo = jnp.concatenate(parts, axis=1)
        att_b = jnp.concatenate([_dot(lo, pltpu.bitcast(wo_s[n], BF16)) for n in range(kt_n)], axis=1)
        att = jnp.concatenate([att_b.reshape(spc, NB, dm), xa_s[pl.ds(s0, spc), NB:, :]], axis=1)
        att = att.reshape(CH, dm)
        xa = x_s[pl.ds(s0, spc)].astype(F32).reshape(CH, dm) + _rows(mod_s[2], CH) * att
        xa_s[pl.ds(s0, spc)] = xa.reshape(spc, seg, dm)
        h = _layernorm(xa) * _rows(mod_s[4], CH) + _rows(mod_s[3], CH)
        r0 = pl.multiple_of(ci * CH, CH)
        h_s[pl.ds(r0, CH), :] = h
        g = _gelu(_dot(_layernorm(h).astype(BF16), w1_s[...]))
        for k in range(kt_n):
            g_s[k, pl.ds(r0 + HALO, CH), :] = g[:, 128 * k:128 * (k + 1)]
        return carry

    jax.lax.fori_loop(0, nch, stage_a, 0)

    def out_copy(ci):
        r0 = pl.multiple_of(ci * CH, CH)
        return pltpu.make_async_copy(out_s.at[pl.ds(r0, CH)], out_hbm.at[pl.ds(r0, CH)], sem_out.at[ci])

    def stage_b(ci, carry):
        r0 = pl.multiple_of(ci * CH, CH)
        s0 = pl.multiple_of(ci * spc, spc)
        shifts = (-1, 1, -2, 2)
        gs = jnp.concatenate(
            [g_s[k, pl.ds(r0 + HALO + shifts[k * 4 // kt_n], CH), :].astype(BF16) for k in range(kt_n)], axis=1)
        x1 = h_s[pl.ds(r0, CH), :] + _dot(gs, w2_s[...])
        act = _gelu(_dot(_layernorm(x1).astype(BF16), w3_s[...])).astype(BF16)
        y = x1 + _dot(act, w4_s[...])
        out_s[pl.ds(r0, CH), :] = (xa_s[pl.ds(s0, spc)].reshape(CH, dm) + _rows(mod_s[5], CH) * y).astype(BF16)
        out_copy(ci).start()
        return carry

    jax.lax.fori_loop(0, nch, stage_b, 0)
    for ci in range(nch):
        out_copy(ci).wait()


@functools.partial(jax.jit, static_argnames=("A_seg_len",))
def pallas_adaLN_cond__memory_aug_recurrent_mem_tr__mixer_s_mlp__prompt_kernel(
    A_x: jax.Array,
    A_mem0: jax.Array,
    A_Wq: jax.Array,
    A_Wk: jax.Array,
    A_Wv: jax.Array,
    A_Wo: jax.Array,
    A_seg_len: int,
    B_x: jax.Array,
    B_w1: jax.Array,
    B_w2: jax.Array,
    B_w3: jax.Array,
    B_w4: jax.Array,
    c: jax.Array,
    w_mod: jax.Array,
):
    del B_x
    b, s, dm = A_x.shape
    _, nh, dh = A_Wq.shape
    nmem = A_mem0.shape[1]
    seg = int(A_seg_len)
    nseg = s // seg
    ff = B_w3.shape[1]
    assert (b, seg, nmem, dh) == (1, 32, NB, 128) and s % CH == 0 and dm % 512 == 0 and nh % 2 == 0
    hp_n = nh // 2
    kt_n = dm // 128
    hbm = pl.BlockSpec(memory_space=pl.ANY)
    vmem = pl.BlockSpec(memory_space=pltpu.VMEM)
    out = pl.pallas_call(
        functools.partial(_kernel, nseg=nseg, seg=seg, nmem=nmem, dm=dm, nh=nh, dh=dh),
        out_shape=jax.ShapeDtypeStruct((s, dm), BF16),
        in_specs=[hbm, vmem, hbm, hbm, hbm, hbm, hbm, hbm, hbm, hbm, vmem, hbm],
        out_specs=hbm,
        scratch_shapes=[
            pltpu.VMEM((3, hp_n, dm, dh), U32),
            pltpu.VMEM((kt_n, nh * dh // 2, 128), U32),
            pltpu.VMEM((dm, dm), BF16),
            pltpu.VMEM((dm, dm), BF16),
            pltpu.VMEM((dm, ff), BF16),
            pltpu.VMEM((ff, dm), BF16),
            pltpu.VMEM((dm, 6 * dm), BF16),
            pltpu.VMEM((nseg, seg, dm), BF16),
            pltpu.VMEM((nseg, NB, dm), BF16),
            pltpu.VMEM((nseg * NB, dm), BF16),
            pltpu.VMEM((3, hp_n, nseg, 2 * NB, dh), BF16),
            pltpu.VMEM((nseg, seg, dm), F32),
            pltpu.VMEM((s, dm), F32),
            pltpu.VMEM((kt_n, s + 2 * HALO, 128), F32),
            pltpu.VMEM((6, 8, dm), F32),
            pltpu.VMEM((2 * (seg + NB), 2 * (seg + NB)), F32),
            pltpu.VMEM((seg, dm), BF16),
            pltpu.VMEM((seg, nh * dh), BF16),
            pltpu.VMEM((s, dm), BF16),
            pltpu.SemaphoreType.DMA((3, hp_n)),
            pltpu.SemaphoreType.DMA((kt_n,)),
            pltpu.SemaphoreType.DMA((8,)),
            pltpu.SemaphoreType.DMA((s // CH,)),
        ],
        compiler_params=pltpu.CompilerParams(vmem_limit_bytes=126 * 1024 * 1024),
    )(A_x.reshape(nseg, seg, dm), A_mem0.reshape(nmem, dm), A_Wq, A_Wk, A_Wv,
      A_Wo.reshape(nh * dh, dm), B_w1, B_w2, B_w3, B_w4, c, w_mod)
    return out.reshape(b, s, dm)
```

```python
import functools
import math

import jax
import jax.numpy as jnp
import numpy as np
import jax.experimental.pallas as pl
import jax.experimental.pallas.tpu as pltpu

F32 = jnp.float32
BF16 = jnp.bfloat16
U32 = jnp.uint32

LN_EPS = 1e-5
MASK_FILL = -1000000000.0
NB = 8
CH = 256
HALO = 8


def _dot(a, b):
    return jnp.dot(a, b, preferred_element_type=F32)


def _dot_nt(a, b):
    return jax.lax.dot_general(a, b, (((1,), (1,)), ((), ())), preferred_element_type=F32)


def _layernorm(x):
    m = jnp.mean(x, axis=-1, keepdims=True)
    d = x - m
    v = jnp.mean(d * d, axis=-1, keepdims=True)
    return d * jax.lax.rsqrt(v + LN_EPS)


def _gelu(x):
    k0 = math.sqrt(2.0 / math.pi)
    t = jnp.tanh(x * (k0 + (k0 * 0.044715) * (x * x)))
    hx = 0.5 * x
    return hx + hx * t


def _rows(v, n):
    return jnp.concatenate([v] * (n // 8), axis=0) if n > 8 else v


def _kernel(x_hbm, mem0_ref, wq_hbm, wk_hbm, wv_hbm, wo_hbm, w1_hbm, w2_hbm, w3_hbm, w4_hbm,
            c_ref, wmod_hbm, out_hbm,
            wqkv, wo_s, w1_s, w2_s, w3_s, w4_s, wmod_s, x_s, xb_s, hb_s, qkvb, xa_s, h_s, g_s,
            mod_s, fill_s, lhs_s, o_s, out_s,
            sem_qkv, sem_wo, sem_misc, sem_out,
            *, nseg, seg, nmem, dm, nh, dh):
    hp_n = nh // 2
    kt_n = dm // 128
    scale = dh ** -0.5
    w_u32 = [w.bitcast(U32) for w in (wq_hbm, wk_hbm, wv_hbm)]
    wo_u32 = wo_hbm.bitcast(U32)

    def qkv_copy(w, hp):
        return pltpu.make_async_copy(w_u32[w].at[:, hp, :], wqkv.at[w, hp], sem_qkv.at[w, hp])

    def wo_copy(n):
        return pltpu.make_async_copy(wo_u32.at[:, pl.ds(pl.multiple_of(n * 128, 128), 128)],
                                     wo_s.at[n], sem_wo.at[n])

    cp_mod0 = pltpu.make_async_copy(wmod_hbm.at[:, 0:2 * dm], wmod_s.at[:, 0:2 * dm], sem_misc.at[0])
    cp_xb = pltpu.make_async_copy(x_hbm.at[:, 0:NB, :], xb_s, sem_misc.at[1])
    cp_x = pltpu.make_async_copy(x_hbm, x_s, sem_misc.at[2])
    cp_mod1 = pltpu.make_async_copy(wmod_hbm.at[:, 2 * dm:], wmod_s.at[:, 2 * dm:], sem_misc.at[3])
    cp_w1 = pltpu.make_async_copy(w1_hbm, w1_s, sem_misc.at[4])
    cp_w2 = pltpu.make_async_copy(w2_hbm, w2_s, sem_misc.at[5])
    cp_w3 = pltpu.make_async_copy(w3_hbm, w3_s, sem_misc.at[6])
    cp_w4 = pltpu.make_async_copy(w4_hbm, w4_s, sem_misc.at[7])

    cp_xb.start()
    cp_mod0.start()
    for w in range(3):
        qkv_copy(w, 0).start()

    def head_pos(i):
        head = jnp.where(i < 2 * seg, i // seg, (i - 2 * seg) // NB)
        r = i % seg
        pos = jnp.where(i < 2 * seg, jnp.where(r < nmem, r, r + NB), nmem + i % NB)
        return head, pos

    nq = 2 * (seg + NB)
    qh, qp = head_pos(jax.lax.broadcasted_iota(jnp.int32, (nq, nq), 0))
    kh, kp = head_pos(jax.lax.broadcasted_iota(jnp.int32, (nq, nq), 1))
    visible = (qp < nmem) | (qp >= kp)
    fill_s[...] = jnp.where(qh == kh, jnp.where(visible, 0.0, MASK_FILL / scale), -jnp.inf).astype(F32)
    zero_halo = jnp.zeros((kt_n, HALO, 128), F32)
    g_s[:, 0:HALO, :] = zero_halo
    g_s[:, HALO + nseg * seg:, :] = zero_halo

    cv = c_ref[...].astype(F32)
    sc = jnp.broadcast_to(cv * jax.nn.sigmoid(cv), (16, dm)).astype(BF16)
    cp_xb.wait()
    ln_b = _layernorm(xb_s[...].astype(F32).reshape(nseg * NB, dm))
    cp_mod0.wait()
    for w in range(3):
        qkv_copy(w, 1).start()
    sa = _dot(sc, wmod_s[:, 0:dm])[0:8]
    ca1 = 1.0 + _dot(sc, wmod_s[:, dm:2 * dm])[0:8]
    mod_s[0] = sa
    mod_s[1] = ca1
    hb_s[...] = (ln_b * _rows(ca1, nseg * NB) + _rows(sa, nseg * NB)).astype(BF16)

    def head_w(w, hp, j):
        return jnp.concatenate(
            [pltpu.bitcast(wqkv[w, hp, pl.ds(128 * k + 64 * j, 64), :], BF16) for k in range(kt_n)], axis=0)

    def bulk_body(hp, carry):
        for w in range(3):
            qkv_copy(w, hp).wait()

        @pl.when(hp + 2 < hp_n)
        def _():
            for w in range(3):
                qkv_copy(w, hp + 2).start()

        @pl.when(hp < kt_n)
        def _():
            wo_copy(hp).start()

        @pl.when(hp == kt_n)
        def _():
            cp_x.start()

        hb = hb_s[...]
        for w in range(3):
            for k in range(kt_n):
                a = wqkv[w, hp, pl.ds(128 * k, 64, stride=2), :]
                b = wqkv[w, hp, pl.ds(128 * k + 1, 64, stride=2), :]
                wqkv[w, hp, pl.ds(128 * k, 64), :] = (a & 0xFFFF) | (b << 16)
                wqkv[w, hp, pl.ds(128 * k + 64, 64), :] = (a >> 16) | (b & np.uint32(0xFFFF0000))
            ra = _dot(hb, head_w(w, hp, 0)).reshape(nseg, NB, dh)
            rb = _dot(hb, head_w(w, hp, 1)).reshape(nseg, NB, dh)
            qkvb[w, hp] = jnp.concatenate([ra, rb], axis=1).astype(BF16)
        return carry

    jax.lax.fori_loop(0, hp_n, bulk_body, 0)

    for n in range(kt_n):
        wo_copy(n).wait()
    cp_x.wait()
    cp_mod1.start()
    cp_w1.start()
    cp_w2.start()
    cp_w3.start()
    cp_w4.start()

    def seg_h(s):
        xs = x_s[s].astype(F32)[NB:]
        return _layernorm(xs) * _rows(mod_s[1], seg - NB) + _rows(mod_s[0], seg - NB)

    lhs_s[...] = jnp.concatenate([mem0_ref[...].astype(F32), seg_h(0)], axis=0).astype(BF16)
    exp_c = scale * math.log2(math.e)

    def step_body(s, carry):
        a = lhs_s[...]
        h_next = seg_h(jnp.minimum(s + 1, nseg - 1))

        def proj(w, hp):
            return jnp.concatenate([_dot(a, head_w(w, hp, 0)).astype(BF16),
                                    _dot(a, head_w(w, hp, 1)).astype(BF16),
                                    qkvb[w, hp, s]], axis=0)

        def probs(q, k):
            fill = fill_s[...]
            sco = jnp.where(fill == 0.0, _dot_nt(q, k), fill)
            e = jnp.exp2((sco - jnp.max(sco, axis=-1, keepdims=True)) * exp_c)
            return (e * (1.0 / jnp.sum(e, axis=-1, keepdims=True))).astype(BF16)

        def attend(hp, p, v):
            o = _dot(p, v).astype(BF16)
            o_s[:, (2 * hp) * dh:(2 * hp + 1) * dh] = o[0:seg]
            o_s[:, (2 * hp + 1) * dh:(2 * hp + 2) * dh] = o[seg:2 * seg]
            qkvb[0, hp, s] = o[2 * seg:]

        pend = []
        for hp in range(hp_n):
            q = proj(0, hp)
            k = proj(1, hp)
            if len(pend) == 2:
                attend(*pend.pop(0))
            v = proj(2, hp)
            pend.append((hp, probs(q, k), v))
        half = nh * dh // 2
        acc = None
        for part in range(2):
            lo = o_s[:, part * half:(part + 1) * half]
            r = []
            for n in range(kt_n):
                r.append(_dot(lo, pltpu.bitcast(wo_s[n, part * half // 2:(part + 1) * half // 2, :], BF16)))
                if pend and n in (1, 4):
                    attend(*pend.pop(0))
            r = jnp.concatenate(r, axis=1)
            acc = r if acc is None else acc + r
        xa_s[s, NB:, :] = acc[nmem:]
        lhs_s[...] = jnp.concatenate([acc[0:nmem], h_next], axis=0).astype(BF16)
        return carry

    jax.lax.fori_loop(0, nseg, step_body, 0)

    cp_mod1.wait()
    for i in range(2, 6):
        r = _dot(sc, wmod_s[:, i * dm:(i + 1) * dm])[0:8]
        mod_s[i] = 1.0 + r if i == 4 else r
    cp_w1.wait()
    cp_w2.wait()
    cp_w3.wait()
    cp_w4.wait()

    spc = CH // seg
    nch = nseg // spc

    def stage_a(ci, carry):
        s0 = pl.multiple_of(ci * spc, spc)
        parts = []
        for hp in range(hp_n):
            ob = qkvb[0, hp, pl.ds(s0, spc)].astype(F32)
            parts.append(ob[:, 0:NB, :].reshape(spc * NB, dh).astype(BF16))
            parts.append(ob[:, NB:, :].reshape(spc * NB, dh).astype(BF16))
        lo = jnp.concatenate(parts, axis=1)
        att_b = jnp.concatenate([_dot(lo, pltpu.bitcast(wo_s[n], BF16)) for n in range(kt_n)], axis=1)
        att = jnp.concatenate([att_b.reshape(spc, NB, dm), xa_s[pl.ds(s0, spc), NB:, :]], axis=1)
        att = att.reshape(CH, dm)
        xa = x_s[pl.ds(s0, spc)].astype(F32).reshape(CH, dm) + _rows(mod_s[2], CH) * att
        xa_s[pl.ds(s0, spc)] = xa.reshape(spc, seg, dm)
        h = _layernorm(xa) * _rows(mod_s[4], CH) + _rows(mod_s[3], CH)
        r0 = pl.multiple_of(ci * CH, CH)
        h_s[pl.ds(r0, CH), :] = h
        g = _gelu(_dot(_layernorm(h).astype(BF16), w1_s[...]))
        for k in range(kt_n):
            g_s[k, pl.ds(r0 + HALO, CH), :] = g[:, 128 * k:128 * (k + 1)]
        return carry

    jax.lax.fori_loop(0, nch, stage_a, 0)

    def out_copy(ci):
        r0 = pl.multiple_of(ci * CH, CH)
        return pltpu.make_async_copy(out_s.at[pl.ds(r0, CH)], out_hbm.at[pl.ds(r0, CH)], sem_out.at[ci])

    def stage_b(ci, carry):
        r0 = pl.multiple_of(ci * CH, CH)
        s0 = pl.multiple_of(ci * spc, spc)
        shifts = (-1, 1, -2, 2)
        gs = jnp.concatenate(
            [g_s[k, pl.ds(r0 + HALO + shifts[k * 4 // kt_n], CH), :].astype(BF16) for k in range(kt_n)], axis=1)
        x1 = h_s[pl.ds(r0, CH), :] + _dot(gs, w2_s[...])
        act = _gelu(_dot(_layernorm(x1).astype(BF16), w3_s[...])).astype(BF16)
        y = x1 + _dot(act, w4_s[...])
        out_s[pl.ds(r0, CH), :] = (xa_s[pl.ds(s0, spc)].reshape(CH, dm) + _rows(mod_s[5], CH) * y).astype(BF16)
        out_copy(ci).start()
        return carry

    jax.lax.fori_loop(0, nch, stage_b, 0)
    for ci in range(nch):
        out_copy(ci).wait()


@functools.partial(jax.jit, static_argnames=("A_seg_len",))
def pallas_adaLN_cond__memory_aug_recurrent_mem_tr__mixer_s_mlp__prompt_kernel(
    A_x: jax.Array,
    A_mem0: jax.Array,
    A_Wq: jax.Array,
    A_Wk: jax.Array,
    A_Wv: jax.Array,
    A_Wo: jax.Array,
    A_seg_len: int,
    B_x: jax.Array,
    B_w1: jax.Array,
    B_w2: jax.Array,
    B_w3: jax.Array,
    B_w4: jax.Array,
    c: jax.Array,
    w_mod: jax.Array,
):
    del B_x
    b, s, dm = A_x.shape
    _, nh, dh = A_Wq.shape
    nmem = A_mem0.shape[1]
    seg = int(A_seg_len)
    nseg = s // seg
    ff = B_w3.shape[1]
    assert (b, seg, nmem, dh) == (1, 32, NB, 128) and s % CH == 0 and dm % 512 == 0 and nh % 2 == 0
    hp_n = nh // 2
    kt_n = dm // 128
    hbm = pl.BlockSpec(memory_space=pl.ANY)
    vmem = pl.BlockSpec(memory_space=pltpu.VMEM)
    out = pl.pallas_call(
        functools.partial(_kernel, nseg=nseg, seg=seg, nmem=nmem, dm=dm, nh=nh, dh=dh),
        out_shape=jax.ShapeDtypeStruct((s, dm), BF16),
        in_specs=[hbm, vmem, hbm, hbm, hbm, hbm, hbm, hbm, hbm, hbm, vmem, hbm],
        out_specs=hbm,
        scratch_shapes=[
            pltpu.VMEM((3, hp_n, dm, dh), U32),
            pltpu.VMEM((kt_n, nh * dh // 2, 128), U32),
            pltpu.VMEM((dm, dm), BF16),
            pltpu.VMEM((dm, dm), BF16),
            pltpu.VMEM((dm, ff), BF16),
            pltpu.VMEM((ff, dm), BF16),
            pltpu.VMEM((dm, 6 * dm), BF16),
            pltpu.VMEM((nseg, seg, dm), BF16),
            pltpu.VMEM((nseg, NB, dm), BF16),
            pltpu.VMEM((nseg * NB, dm), BF16),
            pltpu.VMEM((3, hp_n, nseg, 2 * NB, dh), BF16),
            pltpu.VMEM((nseg, seg, dm), F32),
            pltpu.VMEM((s, dm), F32),
            pltpu.VMEM((kt_n, s + 2 * HALO, 128), F32),
            pltpu.VMEM((6, 8, dm), F32),
            pltpu.VMEM((2 * (seg + NB), 2 * (seg + NB)), F32),
            pltpu.VMEM((seg, dm), BF16),
            pltpu.VMEM((seg, nh * dh), BF16),
            pltpu.VMEM((s, dm), BF16),
            pltpu.SemaphoreType.DMA((3, hp_n)),
            pltpu.SemaphoreType.DMA((kt_n,)),
            pltpu.SemaphoreType.DMA((8,)),
            pltpu.SemaphoreType.DMA((s // CH,)),
        ],
        compiler_params=pltpu.CompilerParams(vmem_limit_bytes=126 * 1024 * 1024),
    )(A_x.reshape(nseg, seg, dm), A_mem0.reshape(nmem, dm), A_Wq, A_Wk, A_Wv,
      A_Wo.reshape(nh * dh, dm), B_w1, B_w2, B_w3, B_w4, c, w_mod)
    return out.reshape(b, s, dm)
```

```python
import functools
import math

import jax
import jax.numpy as jnp
import numpy as np
import jax.experimental.pallas as pl
import jax.experimental.pallas.tpu as pltpu

F32 = jnp.float32
BF16 = jnp.bfloat16
U32 = jnp.uint32

LN_EPS = 1e-5
MASK_FILL = -1000000000.0
NB = 8
CH = 256
HALO = 8


def _dot(a, b):
    return jnp.dot(a, b, preferred_element_type=F32)


def _dot_nt(a, b):
    return jax.lax.dot_general(a, b, (((1,), (1,)), ((), ())), preferred_element_type=F32)


def _layernorm(x):
    m = jnp.mean(x, axis=-1, keepdims=True)
    d = x - m
    v = jnp.mean(d * d, axis=-1, keepdims=True)
    return d * jax.lax.rsqrt(v + LN_EPS)


def _gelu(x):
    k0 = math.sqrt(2.0 / math.pi)
    t = jnp.tanh(x * (k0 + (k0 * 0.044715) * (x * x)))
    hx = 0.5 * x
    return hx + hx * t


def _rows(v, n):
    return jnp.concatenate([v] * (n // 8), axis=0) if n > 8 else v


def _kernel(x_hbm, mem0_ref, wq_hbm, wk_hbm, wv_hbm, wo_hbm, w1_hbm, w2_hbm, w3_hbm, w4_hbm,
            c_ref, wmod_hbm, out_hbm,
            wqkv, wo_s, w1_s, w2_s, w3_s, w4_s, wmod_s, x_s, xb_s, hb_s, qkvb, xa_s, h_s, g_s,
            mod_s, fill_s, lhs_s, o_s, out_s,
            sem_qkv, sem_wo, sem_misc, sem_out,
            *, nseg, seg, nmem, dm, nh, dh):
    hp_n = nh // 2
    kt_n = dm // 128
    scale = dh ** -0.5
    w_u32 = [w.bitcast(U32) for w in (wq_hbm, wk_hbm, wv_hbm)]
    wo_u32 = wo_hbm.bitcast(U32)

    def qkv_copy(w, hp):
        return pltpu.make_async_copy(w_u32[w].at[:, hp, :], wqkv.at[w, hp], sem_qkv.at[w, hp])

    def wo_copy(n):
        return pltpu.make_async_copy(wo_u32.at[:, pl.ds(pl.multiple_of(n * 128, 128), 128)],
                                     wo_s.at[n], sem_wo.at[n])

    cp_mod0 = pltpu.make_async_copy(wmod_hbm.at[:, 0:2 * dm], wmod_s.at[:, 0:2 * dm], sem_misc.at[0])
    cp_xb = pltpu.make_async_copy(x_hbm.at[:, 0:NB, :], xb_s, sem_misc.at[1])
    cp_x = pltpu.make_async_copy(x_hbm, x_s, sem_misc.at[2])
    cp_mod1 = pltpu.make_async_copy(wmod_hbm.at[:, 2 * dm:], wmod_s.at[:, 2 * dm:], sem_misc.at[3])
    cp_w1 = pltpu.make_async_copy(w1_hbm, w1_s, sem_misc.at[4])
    cp_w2 = pltpu.make_async_copy(w2_hbm, w2_s, sem_misc.at[5])
    cp_w3 = pltpu.make_async_copy(w3_hbm, w3_s, sem_misc.at[6])
    cp_w4 = pltpu.make_async_copy(w4_hbm, w4_s, sem_misc.at[7])

    cp_xb.start()
    cp_mod0.start()
    for w in range(3):
        qkv_copy(w, 0).start()

    def head_pos(i):
        head = jnp.where(i < 2 * seg, i // seg, (i - 2 * seg) // NB)
        r = i % seg
        pos = jnp.where(i < 2 * seg, jnp.where(r < nmem, r, r + NB), nmem + i % NB)
        return head, pos

    nq = 2 * (seg + NB)
    qh, qp = head_pos(jax.lax.broadcasted_iota(jnp.int32, (nq, nq), 0))
    kh, kp = head_pos(jax.lax.broadcasted_iota(jnp.int32, (nq, nq), 1))
    visible = (qp < nmem) | (qp >= kp)
    fill_s[...] = jnp.where(qh == kh, jnp.where(visible, 0.0, MASK_FILL / scale), -jnp.inf).astype(F32)
    zero_halo = jnp.zeros((kt_n, HALO, 128), F32)
    g_s[:, 0:HALO, :] = zero_halo
    g_s[:, HALO + nseg * seg:, :] = zero_halo

    cv = c_ref[...].astype(F32)
    sc = jnp.broadcast_to(cv * jax.nn.sigmoid(cv), (16, dm)).astype(BF16)
    cp_xb.wait()
    ln_b = _layernorm(xb_s[...].astype(F32).reshape(nseg * NB, dm))
    cp_mod0.wait()
    for w in range(3):
        qkv_copy(w, 1).start()
    sa = _dot(sc, wmod_s[:, 0:dm])[0:8]
    ca1 = 1.0 + _dot(sc, wmod_s[:, dm:2 * dm])[0:8]
    mod_s[0] = sa
    mod_s[1] = ca1
    hb_s[...] = (ln_b * _rows(ca1, nseg * NB) + _rows(sa, nseg * NB)).astype(BF16)

    def head_w(w, hp, j):
        return jnp.concatenate(
            [pltpu.bitcast(wqkv[w, hp, pl.ds(128 * k + 64 * j, 64), :], BF16) for k in range(kt_n)], axis=0)

    def bulk_body(hp, carry):
        for w in range(3):
            qkv_copy(w, hp).wait()

        @pl.when(hp + 2 < hp_n)
        def _():
            for w in range(3):
                qkv_copy(w, hp + 2).start()

        @pl.when(hp < kt_n)
        def _():
            wo_copy(hp).start()

        @pl.when(hp == kt_n)
        def _():
            cp_x.start()

        hb = hb_s[...]
        for w in range(3):
            for k in range(kt_n):
                a = wqkv[w, hp, pl.ds(128 * k, 64, stride=2), :]
                b = wqkv[w, hp, pl.ds(128 * k + 1, 64, stride=2), :]
                wqkv[w, hp, pl.ds(128 * k, 64), :] = (a & 0xFFFF) | (b << 16)
                wqkv[w, hp, pl.ds(128 * k + 64, 64), :] = (a >> 16) | (b & np.uint32(0xFFFF0000))
            ra = _dot(hb, head_w(w, hp, 0)).reshape(nseg, NB, dh)
            rb = _dot(hb, head_w(w, hp, 1)).reshape(nseg, NB, dh)
            qkvb[w, hp] = jnp.concatenate([ra, rb], axis=1).astype(BF16)
        return carry

    jax.lax.fori_loop(0, hp_n, bulk_body, 0)

    for n in range(kt_n):
        wo_copy(n).wait()
    cp_x.wait()
    cp_mod1.start()
    cp_w1.start()
    cp_w2.start()
    cp_w3.start()
    cp_w4.start()

    def seg_h(s):
        xs = x_s[s].astype(F32)[NB:]
        return _layernorm(xs) * _rows(mod_s[1], seg - NB) + _rows(mod_s[0], seg - NB)

    lhs_s[...] = jnp.concatenate([mem0_ref[...].astype(F32), seg_h(0)], axis=0).astype(BF16)
    exp_c = scale * math.log2(math.e)

    def step_body(s, carry):
        a = lhs_s[...]
        h_next = seg_h(jnp.minimum(s + 1, nseg - 1))

        def proj(w, hp):
            return jnp.concatenate([_dot(a, head_w(w, hp, 0)).astype(BF16),
                                    _dot(a, head_w(w, hp, 1)).astype(BF16),
                                    qkvb[w, hp, s]], axis=0)

        def probs(q, k):
            fill = fill_s[...]
            sco = jnp.where(fill == 0.0, _dot_nt(q, k), fill)
            e = jnp.exp2((sco - jnp.max(sco, axis=-1, keepdims=True)) * exp_c)
            return (e * (1.0 / jnp.sum(e, axis=-1, keepdims=True))).astype(BF16)

        def attend(hp, p, v):
            o = _dot(p, v).astype(BF16)
            o_s[:, (2 * hp) * dh:(2 * hp + 1) * dh] = o[0:seg]
            o_s[:, (2 * hp + 1) * dh:(2 * hp + 2) * dh] = o[seg:2 * seg]
            qkvb[0, hp, s] = o[2 * seg:]

        qk, ps, vs = {}, {}, {}

        def advance(i):
            if i - 1 in qk:
                ps[i - 1] = probs(*qk.pop(i - 1))
            if i - 2 in ps:
                attend(i - 2, ps.pop(i - 2), vs.pop(i - 2))

        for hp in range(hp_n):
            k = proj(1, hp)
            q = proj(0, hp)
            advance(hp)
            qk[hp] = (q, k)
            vs[hp] = proj(2, hp)
        half = nh * dh // 2
        acc = None
        for part in range(2):
            lo = o_s[:, part * half:(part + 1) * half]
            r = []
            for n in range(kt_n):
                r.append(_dot(lo, pltpu.bitcast(wo_s[n, part * half // 2:(part + 1) * half // 2, :], BF16)))
                if part == 0 and n in (1, 5):
                    advance(hp_n + (n == 5))
            r = jnp.concatenate(r, axis=1)
            acc = r if acc is None else acc + r
        xa_s[s, NB:, :] = acc[nmem:]
        lhs_s[...] = jnp.concatenate([acc[0:nmem], h_next], axis=0).astype(BF16)
        return carry

    jax.lax.fori_loop(0, nseg, step_body, 0)

    cp_mod1.wait()
    for i in range(2, 6):
        r = _dot(sc, wmod_s[:, i * dm:(i + 1) * dm])[0:8]
        mod_s[i] = 1.0 + r if i == 4 else r
    cp_w1.wait()
    cp_w2.wait()
    cp_w3.wait()
    cp_w4.wait()

    spc = CH // seg
    nch = nseg // spc

    def stage_a(ci, carry):
        s0 = pl.multiple_of(ci * spc, spc)
        parts = []
        for hp in range(hp_n):
            ob = qkvb[0, hp, pl.ds(s0, spc)].astype(F32)
            parts.append(ob[:, 0:NB, :].reshape(spc * NB, dh).astype(BF16))
            parts.append(ob[:, NB:, :].reshape(spc * NB, dh).astype(BF16))
        lo = jnp.concatenate(parts, axis=1)
        att_b = jnp.concatenate([_dot(lo, pltpu.bitcast(wo_s[n], BF16)) for n in range(kt_n)], axis=1)
        att = jnp.concatenate([att_b.reshape(spc, NB, dm), xa_s[pl.ds(s0, spc), NB:, :]], axis=1)
        att = att.reshape(CH, dm)
        xa = x_s[pl.ds(s0, spc)].astype(F32).reshape(CH, dm) + _rows(mod_s[2], CH) * att
        xa_s[pl.ds(s0, spc)] = xa.reshape(spc, seg, dm)
        h = _layernorm(xa) * _rows(mod_s[4], CH) + _rows(mod_s[3], CH)
        r0 = pl.multiple_of(ci * CH, CH)
        h_s[pl.ds(r0, CH), :] = h
        g = _gelu(_dot(_layernorm(h).astype(BF16), w1_s[...]))
        for k in range(kt_n):
            g_s[k, pl.ds(r0 + HALO, CH), :] = g[:, 128 * k:128 * (k + 1)]
        return carry

    jax.lax.fori_loop(0, nch, stage_a, 0)

    def out_copy(ci):
        r0 = pl.multiple_of(ci * CH, CH)
        return pltpu.make_async_copy(out_s.at[pl.ds(r0, CH)], out_hbm.at[pl.ds(r0, CH)], sem_out.at[ci])

    def stage_b(ci, carry):
        r0 = pl.multiple_of(ci * CH, CH)
        s0 = pl.multiple_of(ci * spc, spc)
        shifts = (-1, 1, -2, 2)
        gs = jnp.concatenate(
            [g_s[k, pl.ds(r0 + HALO + shifts[k * 4 // kt_n], CH), :].astype(BF16) for k in range(kt_n)], axis=1)
        x1 = h_s[pl.ds(r0, CH), :] + _dot(gs, w2_s[...])
        act = _gelu(_dot(_layernorm(x1).astype(BF16), w3_s[...])).astype(BF16)
        y = x1 + _dot(act, w4_s[...])
        out_s[pl.ds(r0, CH), :] = (xa_s[pl.ds(s0, spc)].reshape(CH, dm) + _rows(mod_s[5], CH) * y).astype(BF16)
        out_copy(ci).start()
        return carry

    jax.lax.fori_loop(0, nch, stage_b, 0)
    for ci in range(nch):
        out_copy(ci).wait()


@functools.partial(jax.jit, static_argnames=("A_seg_len",))
def pallas_adaLN_cond__memory_aug_recurrent_mem_tr__mixer_s_mlp__prompt_kernel(
    A_x: jax.Array,
    A_mem0: jax.Array,
    A_Wq: jax.Array,
    A_Wk: jax.Array,
    A_Wv: jax.Array,
    A_Wo: jax.Array,
    A_seg_len: int,
    B_x: jax.Array,
    B_w1: jax.Array,
    B_w2: jax.Array,
    B_w3: jax.Array,
    B_w4: jax.Array,
    c: jax.Array,
    w_mod: jax.Array,
):
    del B_x
    b, s, dm = A_x.shape
    _, nh, dh = A_Wq.shape
    nmem = A_mem0.shape[1]
    seg = int(A_seg_len)
    nseg = s // seg
    ff = B_w3.shape[1]
    assert (b, seg, nmem, dh) == (1, 32, NB, 128) and s % CH == 0 and dm % 512 == 0 and nh % 2 == 0
    hp_n = nh // 2
    kt_n = dm // 128
    hbm = pl.BlockSpec(memory_space=pl.ANY)
    vmem = pl.BlockSpec(memory_space=pltpu.VMEM)
    out = pl.pallas_call(
        functools.partial(_kernel, nseg=nseg, seg=seg, nmem=nmem, dm=dm, nh=nh, dh=dh),
        out_shape=jax.ShapeDtypeStruct((s, dm), BF16),
        in_specs=[hbm, vmem, hbm, hbm, hbm, hbm, hbm, hbm, hbm, hbm, vmem, hbm],
        out_specs=hbm,
        scratch_shapes=[
            pltpu.VMEM((3, hp_n, dm, dh), U32),
            pltpu.VMEM((kt_n, nh * dh // 2, 128), U32),
            pltpu.VMEM((dm, dm), BF16),
            pltpu.VMEM((dm, dm), BF16),
            pltpu.VMEM((dm, ff), BF16),
            pltpu.VMEM((ff, dm), BF16),
            pltpu.VMEM((dm, 6 * dm), BF16),
            pltpu.VMEM((nseg, seg, dm), BF16),
            pltpu.VMEM((nseg, NB, dm), BF16),
            pltpu.VMEM((nseg * NB, dm), BF16),
            pltpu.VMEM((3, hp_n, nseg, 2 * NB, dh), BF16),
            pltpu.VMEM((nseg, seg, dm), F32),
            pltpu.VMEM((s, dm), F32),
            pltpu.VMEM((kt_n, s + 2 * HALO, 128), F32),
            pltpu.VMEM((6, 8, dm), F32),
            pltpu.VMEM((2 * (seg + NB), 2 * (seg + NB)), F32),
            pltpu.VMEM((seg, dm), BF16),
            pltpu.VMEM((seg, nh * dh), BF16),
            pltpu.VMEM((s, dm), BF16),
            pltpu.SemaphoreType.DMA((3, hp_n)),
            pltpu.SemaphoreType.DMA((kt_n,)),
            pltpu.SemaphoreType.DMA((8,)),
            pltpu.SemaphoreType.DMA((s // CH,)),
        ],
        compiler_params=pltpu.CompilerParams(vmem_limit_bytes=126 * 1024 * 1024),
    )(A_x.reshape(nseg, seg, dm), A_mem0.reshape(nmem, dm), A_Wq, A_Wk, A_Wv,
      A_Wo.reshape(nh * dh, dm), B_w1, B_w2, B_w3, B_w4, c, w_mod)
    return out.reshape(b, s, dm)
```

```python
import functools
import math

import jax
import jax.numpy as jnp
import numpy as np
import jax.experimental.pallas as pl
import jax.experimental.pallas.tpu as pltpu

F32 = jnp.float32
BF16 = jnp.bfloat16
U32 = jnp.uint32

HIGH_HALF = np.uint32(0xFFFF0000)
LN_EPS = 1e-5
MASK_FILL = -1000000000.0
NB = 8
CH = 256
LAG_S, LAG_PV, GRP, ORDER, UNROLL = 4, 8, 0, (1, 0, 2), 2
RING = 4
HALO = 8


def _dot(a, b):
    return jnp.dot(a, b, preferred_element_type=F32)


def _dot_nt(a, b):
    return jax.lax.dot_general(a, b, (((1,), (1,)), ((), ())), preferred_element_type=F32)


def _layernorm(x):
    m = jnp.mean(x, axis=-1, keepdims=True)
    d = x - m
    v = jnp.mean(d * d, axis=-1, keepdims=True)
    return d * jax.lax.rsqrt(v + LN_EPS)


def _gelu(x):
    k0 = math.sqrt(2.0 / math.pi)
    t = jnp.tanh(x * (k0 + (k0 * 0.044715) * (x * x)))
    hx = 0.5 * x
    return hx + hx * t


def _rows(v, n):
    return jnp.concatenate([v] * (n // 8), axis=0) if n > 8 else v


def _halfs(w):
    return pltpu.bitcast(w, BF16)


def _lhs_terms(a11, a12, a21, a22):
    return [a11 + a22, a21 + a22, a11, a22, a11 + a12, a21 - a11, a12 - a22]


def _rhs_sums(b11, b12, b21, b22):
    return {0: b11 + b22, 2: b12 - b22, 3: b21 - b11, 5: b11 + b12, 6: b21 + b22}


_RHS_SLOT = {0: 0, 2: 1, 3: 2, 5: 3, 6: 4}


def _strassen(prod, m2=None, m4=None):
    m2 = prod(2) if m2 is None else m2
    m4 = prod(4) if m4 is None else m4
    c12 = m2 + m4
    m0 = prod(0)
    t11 = m0 - m4
    t22 = m0 + m2
    m3 = prod(3)
    t11 = t11 + m3
    c11 = t11 + prod(6)
    m1 = prod(1)
    c21 = m1 + m3
    t22 = t22 - m1
    c22 = t22 + prod(5)
    return c11, c12, c21, c22


def _kernel(x_hbm, mem0_ref, wq_hbm, wk_hbm, wv_hbm, wo_hbm, w1_hbm, w2_hbm, w3_hbm, w4_hbm,
            c_ref, wmod_hbm, out_hbm,
            wo_s, w1_s, w2_s, w3_s, w4_s, wmod_s, x_s, ob_s, xa_s, mod_s,
            sem_qkv, sem_wo, sem_misc, sem_out,
            *, nseg, seg, nmem, dm, nh, dh):
    hp_n = nh // 2
    kt_n = dm // 128
    ff = w3_s.shape[1]
    scale = dh ** -0.5
    w_u32 = [w.bitcast(U32) for w in (wq_hbm, wk_hbm, wv_hbm)]
    wo_u32 = wo_hbm.bitcast(U32)

    def wo_copy(i):
        n, per = i & (kt_n - 1), wo_s.shape[1] * kt_n // hp_n
        rows = pl.ds(pl.multiple_of((i >> (kt_n.bit_length() - 1)) * per, per), per)
        return pltpu.make_async_copy(wo_u32.at[rows, pl.ds(pl.multiple_of(n * 128, 128), 128)],
                                     wo_s.at[n, rows], sem_wo.at[i])

    cp_mod0 = pltpu.make_async_copy(wmod_hbm.at[:, 0:2 * dm], wmod_s.at[:, 0:2 * dm], sem_misc.at[0])
    cp_mod1 = pltpu.make_async_copy(wmod_hbm.at[:, 2 * dm:], wmod_s.at[:, 2 * dm:], sem_misc.at[3])
    cp_w1 = pltpu.make_async_copy(w1_hbm, w1_s, sem_misc.at[4])
    cp_w2 = pltpu.make_async_copy(w2_hbm, w2_s, sem_misc.at[5])
    cp_w3 = pltpu.make_async_copy(w3_hbm, w3_s, sem_misc.at[6])
    cp_w4 = pltpu.make_async_copy(w4_hbm, w4_s, sem_misc.at[7])

    def silu_c():
        cv = c_ref[...].astype(F32)
        return jnp.broadcast_to(cv * jax.nn.sigmoid(cv), (16, dm)).astype(BF16)

    def attention(wqkv, qkvb, xb_s, hb_s, fill_s, hx_s, o_s, raw_s):
        xs_n = nseg // hp_n

        def pair_copies(hp):
            cps = [pltpu.make_async_copy(w_u32[w].at[:, hp, :], raw_s.at[w, hp & (RING - 1)], sem_qkv.at[w, hp])
                   for w in range(3)]
            rows = pl.ds(hp * xs_n, xs_n)
            return cps + [pltpu.make_async_copy(x_hbm.at[rows], x_s.at[rows], sem_qkv.at[3, hp])]

        cp_xb = pltpu.make_async_copy(x_hbm.at[:, 0:NB, :], xb_s, sem_misc.at[1])
        cp_xb.start()
        cp_mod0.start()
        for cp in pair_copies(0):
            cp.start()

        def head_pos(i):
            head = jnp.where(i < 2 * seg, i // seg, (i - 2 * seg) // NB)
            r = i % seg
            pos = jnp.where(i < 2 * seg, jnp.where(r < nmem, r, r + NB), nmem + i % NB)
            return head, pos

        nq = 2 * (seg + NB)
        qh, qp = head_pos(jax.lax.broadcasted_iota(jnp.int32, (nq, nq), 0))
        kh, kp = head_pos(jax.lax.broadcasted_iota(jnp.int32, (nq, nq), 1))
        visible = (qp < nmem) | (qp >= kp)
        fill_s[...] = jnp.where(qh == kh, jnp.where(visible, 0.0, MASK_FILL / scale), -jnp.inf).astype(F32)

        sc = silu_c()
        cp_xb.wait()
        ln_b = _layernorm(xb_s[...].astype(F32).reshape(nseg * NB, dm))
        cp_mod0.wait()
        for cp in pair_copies(1):
            cp.start()
        sa = _dot(sc, wmod_s[:, 0:dm])[0:8]
        ca1 = 1.0 + _dot(sc, wmod_s[:, dm:2 * dm])[0:8]
        mod_s[0] = sa
        mod_s[1] = ca1
        hb = ln_b * _rows(ca1, nseg * NB) + _rows(sa, nseg * NB)
        mh, kh = nseg * NB // 2, dm // 2
        for i, t in enumerate(_lhs_terms(hb[:mh, :kh], hb[:mh, kh:], hb[mh:, :kh], hb[mh:, kh:])):
            hb_s[i] = t.astype(BF16)

        def head_w(w, hp, j, rows=slice(None)):
            return _halfs(wqkv[w, 2 * hp + j, rows, :])

        def bulk_body(hp, carry):
            @pl.when(hp + 2 < hp_n)
            def _():
                for cp in pair_copies(hp + 2):
                    cp.start()

            wo_copy(hp).start()
            for cp in pair_copies(hp):
                cp.wait()
            slot = hp & (RING - 1)
            for w in range(3):
                def quad(i):
                    word = raw_s[w, slot, (i // 2) * kh:(i // 2 + 1) * kh, :]
                    return pltpu.bitcast(word & HIGH_HALF if i % 2 else word << 16, F32)

                def prod(i):
                    q = [quad(j) for j in range(4)]
                    return _dot(hb_s[i], {1: q[0], 4: q[3], **_rhs_sums(*q)}[i].astype(BF16))

                m4 = prod(4)
                res = [t.reshape(nseg // 2, NB, dh) for t in _strassen(prod, None, m4)]
                for r in range(0, dm, 16):
                    a = raw_s[w, slot, pl.ds(r, 8, stride=2), :]
                    b = raw_s[w, slot, pl.ds(r + 1, 8, stride=2), :]
                    wqkv[w, 2 * hp, r // 2:r // 2 + 8, :] = (a & 0xFFFF) | (b << 16)
                    wqkv[w, 2 * hp + 1, r // 2:r // 2 + 8, :] = (a >> 16) | (b & HIGH_HALF)
                for i in range(xs_n * w // 3, xs_n * (w + 1) // 3):
                    xs = x_s[hp * xs_n + i, NB:, :].astype(F32)
                    hx_s[hp * xs_n + i] = _layernorm(xs) * _rows(mod_s[1], seg - NB) + _rows(mod_s[0], seg - NB)
                qkvb[w, hp, :nseg // 2] = jnp.concatenate(res[:2], axis=1).astype(BF16)
                qkvb[w, hp, nseg // 2:] = jnp.concatenate(res[2:], axis=1).astype(BF16)
            return carry

        jax.lax.fori_loop(0, hp_n, bulk_body, 0)

        for i in range(hp_n):
            wo_copy(i).wait()
        cp_mod1.start()
        cp_w1.start()
        cp_w2.start()
        cp_w3.start()
        cp_w4.start()

        exp_c = scale * math.log2(math.e)

        def step(s, mem):
            a = jnp.concatenate([mem, hx_s[s]], axis=0)
            a = [a[:, :kh].astype(BF16), a[:, kh:].astype(BF16)]

            first = {(w, j): _dot(a[0], head_w(w, 0, j, slice(0, kh // 2))) for w in ORDER for j in range(2)}

            def proj(w, hp):
                if hp == 0:
                    r = [first[w, j] + _dot(a[1], head_w(w, 0, j, slice(kh // 2, kh))) for j in range(2)]
                else:
                    r = [_dot(a[0], head_w(w, hp, j, slice(0, kh // 2)))
                         + _dot(a[1], head_w(w, hp, j, slice(kh // 2, kh))) for j in range(2)]
                return jnp.concatenate(r + [qkvb[w, hp, s].astype(F32)], axis=0).astype(BF16)

            def probs(q, k):
                fill = fill_s[...]
                sco = jnp.where(fill == 0.0, _dot_nt(q, k), fill)
                e = jnp.exp2((sco - jnp.max(sco, axis=-1, keepdims=True)) * exp_c)
                den = jnp.sum(e, axis=-1, keepdims=True)
                inv = pl.reciprocal(den, approx=True)
                return e.astype(BF16), inv * (2.0 - den * inv)

            def attend(hp, p, v):
                o = _dot(p[0], v) * p[1]
                cols = slice(2 * hp * dh, 2 * (hp + 1) * dh)
                o_s[:, cols] = jnp.concatenate([o[0:seg], o[seg:2 * seg]], axis=1).astype(BF16)
                ob_s[s, :, cols] = jnp.concatenate(
                    [o[2 * seg:2 * seg + NB], o[2 * seg + NB:]], axis=1).astype(BF16)

            val, ps = {}, {}
            clock = [0]

            def tick():
                t = clock[0]
                clock[0] += 1
                for i in range(hp_n):
                    if t == 3 * (i | GRP) + LAG_S:
                        ps[i] = probs(val.pop((0, i)), val.pop((1, i)))
                for i in range(hp_n):
                    if t == 3 * (i | GRP) + LAG_PV:
                        attend(i, ps.pop(i), val.pop((2, i)))

            for hp in range(hp_n):
                for w in ORDER:
                    val[w, hp] = proj(w, hp)
                    tick()
            half = nh * dh // 2
            acc = None
            for part in range(2):
                assert part == 0 or not val
                lo = o_s[:, part * half:(part + 1) * half]
                r = []
                for n in range(kt_n):
                    r.append(_dot(lo, _halfs(wo_s[n, part * half // 2:(part + 1) * half // 2, :])))
                    tick()
                r = jnp.concatenate(r, axis=1)
                acc = r if acc is None else acc + r
            xa_s[s, NB:, :] = acc[nmem:]
            return acc[0:nmem]

        def step_body(i, mem):
            for u in range(UNROLL):
                mem = step(i * UNROLL + u, mem)
            return mem

        jax.lax.fori_loop(0, nseg // UNROLL, step_body, mem0_ref[...].astype(F32))

    pl.run_scoped(
        attention,
        pltpu.VMEM((3, nh, dm // 2, dh), U32),
        pltpu.VMEM((3, hp_n, nseg, 2 * NB, dh), BF16),
        pltpu.VMEM((nseg, NB, dm), BF16),
        pltpu.VMEM((7, nseg * NB // 2, dm // 2), BF16),
        pltpu.VMEM((2 * (seg + NB), 2 * (seg + NB)), F32),
        pltpu.VMEM((nseg, seg - NB, dm), F32),
        pltpu.VMEM((seg, nh * dh), BF16),
        pltpu.VMEM((3, RING, dm, dh), U32),
    )

    spc = CH // seg
    nch = nseg // spc
    hc = CH // 2
    sh = spc // 2
    dm2, ff2 = dm // 2, ff // 2
    ft_n, nt_n = ff2 // 128, dm2 // 128

    def mlp(w3x_s, w4x_s, h_s, g_s, out_s, a3_s, a4_s, att_s, u_s):
        zero_halo = jnp.zeros((kt_n, HALO, 128), F32)
        g_s[:, 0:HALO, :] = zero_halo
        g_s[:, HALO + nseg * seg:, :] = zero_halo
        cp_mod1.wait()
        sc = silu_c()

        def mod_body(i, carry):
            r = _dot(sc, wmod_s[:, pl.ds(pl.multiple_of(i * dm, dm), dm)])[0:8]
            mod_s[i] = jnp.where(i == 4, 1.0 + r, r)
            return carry

        jax.lax.fori_loop(2, 6, mod_body, 0)
        cp_w1.wait()
        cp_w2.wait()
        cp_w3.wait()
        cp_w4.wait()

        def weight_sum_jobs(w_s, wx_s, ci):
            k2, n2 = w_s.shape[0] // 2, w_s.shape[1] // 2
            nr = k2 // nch

            def job(r, c0):
                r0 = pl.multiple_of(ci * nr + r, 16)
                quad = [w_s[pl.ds(r0 + kk, 16), nn + c0:nn + c0 + 256].astype(F32)
                        for kk in (0, k2) for nn in (0, n2)]
                for i, t in _rhs_sums(*quad).items():
                    wx_s[_RHS_SLOT[i], pl.ds(r0, 16), c0:c0 + 256] = t.astype(BF16)

            return [functools.partial(job, r, c0) for r in range(0, nr, 16) for c0 in range(0, n2, 256)]

        def rhs(w_s, wx_s, i, j):
            k2, n2 = w_s.shape[0] // 2, w_s.shape[1] // 2
            if i == 1:
                return w_s[0:k2, 128 * j:128 * (j + 1)]
            if i == 4:
                return w_s[k2:, n2 + 128 * j:n2 + 128 * (j + 1)]
            return wx_s[_RHS_SLOT[i], :, 128 * j:128 * (j + 1)]

        def stage_a(ci, carry):
            def spread(jobs, n):
                for job in jobs[len(jobs) * n // kt_n:len(jobs) * (n + 1) // kt_n]:
                    job()

            def out_proj(half, jobs):
                lo = ob_s[pl.ds(ci * spc + half * sh, sh)].reshape(sh * NB, nh * dh)
                for n in range(kt_n):
                    att_s[half, :, 128 * n:128 * (n + 1)] = _dot(lo, _halfs(wo_s[n]))
                    spread(jobs, n)

            def norm(half, i):
                si = ci * spc + half * sh + i
                att = jnp.concatenate([att_s[half, NB * i:NB * (i + 1), :], xa_s[si, NB:, :]], axis=0)
                xa = x_s[si].astype(F32) + _rows(mod_s[2], seg) * att
                xa_s[si] = xa
                h = _layernorm(xa) * _rows(mod_s[4], seg) + _rows(mod_s[3], seg)
                h_s[pl.ds(pl.multiple_of(si * seg, seg), seg), :] = h
                u_s[half, seg * i:seg * (i + 1), :] = _layernorm(h).astype(BF16)

            def mix_in(half, jobs):
                r0 = pl.multiple_of(ci * CH + half * hc, hc)
                u = u_s[half]
                for k in range(kt_n):
                    g_s[k, pl.ds(r0 + HALO, hc), :] = _gelu(_dot(u, w1_s[:, 128 * k:128 * (k + 1)]))
                    spread(jobs, k)

            out_proj(0, weight_sum_jobs(w3_s, w3x_s, ci) + weight_sum_jobs(w4_s, w4x_s, ci))
            out_proj(1, [functools.partial(norm, 0, i) for i in range(sh)])
            mix_in(0, [functools.partial(norm, 1, i) for i in range(sh)])
            mix_in(1, [])
            return carry

        jax.lax.fori_loop(0, nch, stage_a, 0)

        def out_copy(ci):
            r0 = pl.multiple_of(ci * CH, CH)
            return pltpu.make_async_copy(out_s.at[pl.ds(r0, CH)], out_hbm.at[pl.ds(r0, CH)], sem_out.at[ci])

        def stage_b(ci, carry):
            shifts = (-1, 1, -2, 2)
            x1, u = [], []
            for half in range(2):
                r0 = pl.multiple_of(ci * CH + half * hc, hc)
                gs = jnp.concatenate(
                    [g_s[k, pl.ds(r0 + HALO + shifts[k * 4 // kt_n], hc), :].astype(BF16)
                     for k in range(kt_n)], axis=1)
                x1.append(h_s[pl.ds(r0, hc), :] + _dot(gs, w2_s[...]))
                u.append(_layernorm(x1[-1]))
            for i, t in enumerate(_lhs_terms(u[0][:, :dm2], u[0][:, dm2:], u[1][:, :dm2], u[1][:, dm2:])):
                a3_s[i] = t.astype(BF16)

            def prod3(j, i):
                return _dot(a3_s[i], rhs(w3_s, w3x_s, i, j))

            early = {j: (prod3(j, 2), prod3(j, 4)) for j in range(4)}
            for j in range(ft_n):
                act = [_gelu(t) for t in _strassen(functools.partial(prod3, j), *early.get(j, ()))]
                for i, t in enumerate(_lhs_terms(*act)):
                    a4_s[i, :, 128 * j:128 * (j + 1)] = t.astype(BF16)

            def prod4(n, i):
                return _dot(a4_s[i], rhs(w4_s, w4x_s, i, n))

            for n in range(nt_n):
                for q, t in enumerate(_strassen(functools.partial(prod4, n))):
                    half, c0 = q // 2, (q % 2) * dm2 + 128 * n
                    r0 = pl.multiple_of(ci * CH + half * hc, hc)
                    xa = xa_s[pl.ds(ci * spc + half * sh, sh), :, c0:c0 + 128].reshape(hc, 128)
                    y = x1[half][:, c0:c0 + 128] + t
                    out_s[pl.ds(r0, hc), c0:c0 + 128] = (xa + _rows(mod_s[5, :, c0:c0 + 128], hc) * y).astype(BF16)
            out_copy(ci).start()
            return carry

        jax.lax.fori_loop(0, nch, stage_b, 0)
        for ci in range(nch):
            out_copy(ci).wait()

    pl.run_scoped(
        mlp,
        pltpu.VMEM((5, dm2, ff2), BF16),
        pltpu.VMEM((5, ff2, dm2), BF16),
        pltpu.VMEM((nseg * seg, dm), F32),
        pltpu.VMEM((kt_n, nseg * seg + 2 * HALO, 128), F32),
        pltpu.VMEM((nseg * seg, dm), BF16),
        pltpu.VMEM((7, hc, dm2), BF16),
        pltpu.VMEM((7, hc, ff2), BF16),
        pltpu.VMEM((2, sh * NB, dm), F32),
        pltpu.VMEM((2, hc, dm), BF16),
    )


@functools.partial(jax.jit, static_argnames=("A_seg_len",))
def pallas_adaLN_cond__memory_aug_recurrent_mem_tr__mixer_s_mlp__prompt_kernel(
    A_x: jax.Array,
    A_mem0: jax.Array,
    A_Wq: jax.Array,
    A_Wk: jax.Array,
    A_Wv: jax.Array,
    A_Wo: jax.Array,
    A_seg_len: int,
    B_x: jax.Array,
    B_w1: jax.Array,
    B_w2: jax.Array,
    B_w3: jax.Array,
    B_w4: jax.Array,
    c: jax.Array,
    w_mod: jax.Array,
):
    del B_x
    b, s, dm = A_x.shape
    _, nh, dh = A_Wq.shape
    nmem = A_mem0.shape[1]
    seg = int(A_seg_len)
    nseg = s // seg
    ff = B_w3.shape[1]
    assert (b, seg, nmem, dh) == (1, 32, NB, 128) and s % CH == 0 and dm % 512 == 0 and nh % 2 == 0
    hp_n = nh // 2
    kt_n = dm // 128
    hbm = pl.BlockSpec(memory_space=pl.ANY)
    vmem = pl.BlockSpec(memory_space=pltpu.VMEM)
    out = pl.pallas_call(
        functools.partial(_kernel, nseg=nseg, seg=seg, nmem=nmem, dm=dm, nh=nh, dh=dh),
        out_shape=jax.ShapeDtypeStruct((s, dm), BF16),
        in_specs=[hbm, vmem, hbm, hbm, hbm, hbm, hbm, hbm, hbm, hbm, vmem, hbm],
        out_specs=hbm,
        scratch_shapes=[
            pltpu.VMEM((kt_n, nh * dh // 2, 128), U32),
            pltpu.VMEM((dm, dm), BF16),
            pltpu.VMEM((dm, dm), BF16),
            pltpu.VMEM((dm, ff), BF16),
            pltpu.VMEM((ff, dm), BF16),
            pltpu.VMEM((dm, 6 * dm), BF16),
            pltpu.VMEM((nseg, seg, dm), BF16),
            pltpu.VMEM((nseg, NB, nh * dh), BF16),
            pltpu.VMEM((nseg, seg, dm), F32),
            pltpu.VMEM((6, 8, dm), F32),
            pltpu.SemaphoreType.DMA((4, hp_n)),
            pltpu.SemaphoreType.DMA((hp_n,)),
            pltpu.SemaphoreType.DMA((8,)),
            pltpu.SemaphoreType.DMA((s // CH,)),
        ],
        compiler_params=pltpu.CompilerParams(vmem_limit_bytes=120 * 1024 * 1024),
    )(A_x.reshape(nseg, seg, dm), A_mem0.reshape(nmem, dm), A_Wq, A_Wk, A_Wv,
      A_Wo.reshape(nh * dh, dm), B_w1, B_w2, B_w3, B_w4, c, w_mod)
    return out.reshape(b, s, dm)
```

```python
import functools
import math

import jax
import jax.numpy as jnp
import numpy as np
import jax.experimental.pallas as pl
import jax.experimental.pallas.tpu as pltpu

F32 = jnp.float32
BF16 = jnp.bfloat16
U32 = jnp.uint32

HIGH_HALF = np.uint32(0xFFFF0000)
LN_EPS = 1e-5
MASK_FILL = -1000000000.0
NB = 8
CH = 256
LAG_S, LAG_PV, GRP, ORDER, UNROLL = 4, 8, 0, (1, 0, 2), 2
RING = 4
HALO = 8


def _dot(a, b):
    return jnp.dot(a, b, preferred_element_type=F32)


def _dot_nt(a, b):
    return jax.lax.dot_general(a, b, (((1,), (1,)), ((), ())), preferred_element_type=F32)


def _layernorm(x):
    m = jnp.mean(x, axis=-1, keepdims=True)
    d = x - m
    v = jnp.mean(d * d, axis=-1, keepdims=True)
    return d * jax.lax.rsqrt(v + LN_EPS)


def _gelu(x):
    k0 = math.sqrt(2.0 / math.pi)
    t = jnp.tanh(x * (k0 + (k0 * 0.044715) * (x * x)))
    hx = 0.5 * x
    return hx + hx * t


def _rows(v, n):
    return jnp.concatenate([v] * (n // 8), axis=0) if n > 8 else v


def _halfs(w):
    return pltpu.bitcast(w, BF16)


def _lhs_terms(a11, a12, a21, a22):
    return [a11 + a22, a21 + a22, a11, a22, a11 + a12, a21 - a11, a12 - a22]


def _rhs_sums(b11, b12, b21, b22):
    return {0: b11 + b22, 2: b12 - b22, 3: b21 - b11, 5: b11 + b12, 6: b21 + b22}


_RHS_SLOT = {0: 0, 3: 1, 5: 2, 6: 3}


def _strassen(prod, m2=None, m4=None):
    m2 = prod(2) if m2 is None else m2
    m4 = prod(4) if m4 is None else m4
    c12 = m2 + m4
    m0 = prod(0)
    t11 = m0 - m4
    t22 = m0 + m2
    m3 = prod(3)
    t11 = t11 + m3
    c11 = t11 + prod(6)
    m1 = prod(1)
    c21 = m1 + m3
    t22 = t22 - m1
    c22 = t22 + prod(5)
    return c11, c12, c21, c22


def _kernel(x_hbm, mem0_hbm, wq_hbm, wk_hbm, wv_hbm, wo_hbm, w1_hbm, w2_hbm, w3_hbm, w4_hbm,
            c_hbm, wmod_hbm, out_hbm,
            wo_s, w1_s, w2_s, w3_s, w4_s, wmod_s, x_s, ob_s, xa_s, mod_s, c_ref, mem0_ref,
            sem_qkv, sem_misc, sem_mod,
            *, nseg, seg, nmem, dm, nh, dh):
    hp_n = nh // 2
    kt_n = dm // 128
    ff = w3_s.shape[1]
    scale = dh ** -0.5
    w_u32 = [w.bitcast(U32) for w in (wq_hbm, wk_hbm, wv_hbm)]
    wo_u32 = wo_hbm.bitcast(U32)

    def wo_copy(i):
        n, per = i & (kt_n - 1), wo_s.shape[1] * kt_n // hp_n
        rows = pl.ds(pl.multiple_of((i >> (kt_n.bit_length() - 1)) * per, per), per)
        return pltpu.make_async_copy(wo_u32.at[rows, pl.ds(pl.multiple_of(n * 128, 128), 128)],
                                     wo_s.at[n, rows], sem_misc.at[0])

    wmod_u32 = wmod_hbm.bitcast(U32)

    def mod_copy(t, group):
        return pltpu.make_async_copy(wmod_u32.at[:, pl.ds(pl.multiple_of(t * 128, 128), 128)],
                                     wmod_s.at[t], sem_mod.at[group])

    cp_c = pltpu.make_async_copy(c_hbm, c_ref, sem_misc.at[2])
    cp_mem0 = pltpu.make_async_copy(mem0_hbm, mem0_ref, sem_misc.at[3])
    cp_w1 = pltpu.make_async_copy(w1_hbm, w1_s, sem_misc.at[4])
    cp_w2 = pltpu.make_async_copy(w2_hbm, w2_s, sem_misc.at[5])
    cp_w3 = pltpu.make_async_copy(w3_hbm, w3_s, sem_misc.at[6])
    cp_w4 = pltpu.make_async_copy(w4_hbm, w4_s, sem_misc.at[7])

    def silu_c():
        cv = c_ref[...].astype(F32)
        return jnp.broadcast_to(cv * jax.nn.sigmoid(cv), (16, dm)).astype(BF16)

    def attention(wqkv, qkvb, xb_s, hb_s, fill_s, hx_s, o_s, raw_s, ln_s):
        xs_n = nseg // hp_n

        def pair_copies(hp):
            cps = [pltpu.make_async_copy(w_u32[w].at[:, hp, :], raw_s.at[w, hp & (RING - 1)], sem_qkv.at[hp & (RING - 1)])
                   for w in range(3)]
            rows = pl.ds(hp * xs_n, xs_n)
            return cps + [pltpu.make_async_copy(x_hbm.at[rows], x_s.at[rows], sem_qkv.at[hp & (RING - 1)])]

        cp_xb = pltpu.make_async_copy(x_hbm.at[:, 0:NB, :], xb_s, sem_misc.at[1])
        cp_xb.start()
        cp_c.start()
        cp_mem0.start()
        jt_n = kt_n // 2

        def mod_group(j):
            return [mod_copy(j + t * jt_n, j) for t in range(4)]

        for cp in mod_group(0):
            cp.start()

        def head_pos(i):
            head = jnp.where(i < 2 * seg, i // seg, (i - 2 * seg) // NB)
            r = i % seg
            pos = jnp.where(i < 2 * seg, jnp.where(r < nmem, r, r + NB), nmem + i % NB)
            return head, pos

        nq = 2 * (seg + NB)
        qh, qp = head_pos(jax.lax.broadcasted_iota(jnp.int32, (nq, nq), 0))
        kh, kp = head_pos(jax.lax.broadcasted_iota(jnp.int32, (nq, nq), 1))
        visible = (qp < nmem) | (qp >= kp)
        fill_s[...] = jnp.where(qh == kh, jnp.where(visible, 0.0, MASK_FILL / scale), -jnp.inf).astype(F32)

        mh, kh = nseg * NB // 2, dm // 2
        cp_c.wait()
        cp_mem0.wait()
        sc = silu_c()
        for cp in mod_group(1):
            cp.start()
        cp_xb.wait()
        for cp in mod_group(2):
            cp.start()

        def ln_body(i, carry):
            s0 = i * (nseg // 4)
            ln = _layernorm(xb_s[pl.ds(s0, nseg // 4)].astype(F32).reshape(mh // 2, dm))
            for k in range(kt_n):
                ln_s[k, pl.ds(pl.multiple_of(i * (mh // 2), mh // 2), mh // 2), :] = ln[:, 128 * k:128 * (k + 1)]
            return carry

        jax.lax.fori_loop(0, 4, ln_body, 0)

        def shift_scale_body(j, carry):
            for cp in mod_group(j):
                cp.wait()

            @pl.when(j == 0)
            def _():
                for cp in mod_group(3):
                    cp.start()

            @pl.when(j == 1)
            def _():
                for cp in pair_copies(0):
                    cp.start()

            shift, gain = [], []
            for k in (j, j + jt_n):
                cols = pl.ds(pl.multiple_of(k * 128, 128), 128)
                shift.append(_dot(sc, _halfs(wmod_s[k]))[0:8])
                gain.append(1.0 + _dot(sc, _halfs(wmod_s[kt_n + k]))[0:8])
                mod_s[0, :, cols] = shift[-1]
                mod_s[1, :, cols] = gain[-1]
            for r in range(0, mh, 32):
                quad = [ln_s[j + t * jt_n, r0 + r:r0 + r + 32, :] * _rows(gain[t], 32) + _rows(shift[t], 32)
                        for r0 in (0, mh) for t in range(2)]
                for i, t in enumerate(_lhs_terms(*quad)):
                    hb_s[i, r:r + 32, pl.ds(pl.multiple_of(j * 128, 128), 128)] = t.astype(BF16)
            return carry

        jax.lax.fori_loop(0, jt_n, shift_scale_body, 0)
        for cp in pair_copies(1):
            cp.start()

        def head_w(w, hp, j, rows=slice(None)):
            return _halfs(wqkv[w, 2 * hp + j, rows, :])

        def bulk_body(hp, carry):
            for cp in pair_copies(hp):
                cp.wait()

            @pl.when(hp + 2 < hp_n)
            def _():
                for cp in pair_copies(hp + 2):
                    cp.start()

            pl.when(hp == 0)(wo_copy(0).start)
            pl.when(hp + 1 < hp_n)(lambda: wo_copy(hp + 1).start())
            slot = hp & (RING - 1)
            for w in range(3):
                def quad(i):
                    word = raw_s[w, slot, (i // 2) * kh:(i // 2 + 1) * kh, :]
                    return pltpu.bitcast(word & HIGH_HALF if i % 2 else word << 16, F32)

                def prod(i):
                    q = [quad(j) for j in range(4)]
                    return _dot(hb_s[i], {1: q[0], 4: q[3], **_rhs_sums(*q)}[i].astype(BF16))

                m4 = prod(4)
                res = [t.reshape(nseg // 2, NB, dh) for t in _strassen(prod, None, m4)]
                for r in range(0, dm, 16):
                    a = raw_s[w, slot, pl.ds(r, 8, stride=2), :]
                    b = raw_s[w, slot, pl.ds(r + 1, 8, stride=2), :]
                    wqkv[w, 2 * hp, r // 2:r // 2 + 8, :] = (a & 0xFFFF) | (b << 16)
                    wqkv[w, 2 * hp + 1, r // 2:r // 2 + 8, :] = (a >> 16) | (b & HIGH_HALF)
                for i in range(xs_n * w // 3, xs_n * (w + 1) // 3):
                    xs = x_s[hp * xs_n + i, NB:, :].astype(F32)
                    hx_s[hp * xs_n + i] = _layernorm(xs) * _rows(mod_s[1], seg - NB) + _rows(mod_s[0], seg - NB)
                qkvb[w, hp, :nseg // 2] = jnp.concatenate(res[:2], axis=1).astype(BF16)
                qkvb[w, hp, nseg // 2:] = jnp.concatenate(res[2:], axis=1).astype(BF16)
            return carry

        jax.lax.fori_loop(0, hp_n, bulk_body, 0)

        pltpu.make_async_copy(wo_s, wo_s, sem_misc.at[0]).wait()

        mod_per_it = 4 * kt_n * UNROLL // nseg
        exp_c = scale * math.log2(math.e)

        def step(s, mem):
            a = jnp.concatenate([mem, hx_s[s]], axis=0)
            a = [a[:, :kh].astype(BF16), a[:, kh:].astype(BF16)]

            first = {(w, j): _dot(a[0], head_w(w, 0, j, slice(0, kh // 2))) for w in ORDER for j in range(2)}

            def proj(w, hp):
                if hp == 0:
                    r = [first[w, j] + _dot(a[1], head_w(w, 0, j, slice(kh // 2, kh))) for j in range(2)]
                else:
                    r = [_dot(a[0], head_w(w, hp, j, slice(0, kh // 2)))
                         + _dot(a[1], head_w(w, hp, j, slice(kh // 2, kh))) for j in range(2)]
                return jnp.concatenate(r + [qkvb[w, hp, s].astype(F32)], axis=0).astype(BF16)

            def probs(q, k):
                fill = fill_s[...]
                sco = jnp.where(fill == 0.0, _dot_nt(q, k), fill)
                e = jnp.exp2((sco - jnp.max(sco, axis=-1, keepdims=True)) * exp_c)
                den = jnp.sum(e, axis=-1, keepdims=True)
                inv = pl.reciprocal(den, approx=True)
                return e.astype(BF16), inv * (2.0 - den * inv)

            def attend(hp, p, v):
                o = _dot(p[0], v) * p[1]
                cols = slice(2 * hp * dh, 2 * (hp + 1) * dh)
                o_s[:, cols] = jnp.concatenate([o[0:seg], o[seg:2 * seg]], axis=1).astype(BF16)
                ob_s[s, :, cols] = jnp.concatenate(
                    [o[2 * seg:2 * seg + NB], o[2 * seg + NB:]], axis=1).astype(BF16)

            val, ps = {}, {}
            clock = [0]

            def tick():
                t = clock[0]
                clock[0] += 1
                for i in range(hp_n):
                    if t == 3 * (i | GRP) + LAG_S:
                        ps[i] = probs(val.pop((0, i)), val.pop((1, i)))
                for i in range(hp_n):
                    if t == 3 * (i | GRP) + LAG_PV:
                        attend(i, ps.pop(i), val.pop((2, i)))

            for hp in range(hp_n):
                for w in ORDER:
                    val[w, hp] = proj(w, hp)
                    tick()
            half = nh * dh // 2
            acc = None
            for part in range(2):
                assert part == 0 or not val
                lo = o_s[:, part * half:(part + 1) * half]
                r = []
                for n in range(kt_n):
                    r.append(_dot(lo, _halfs(wo_s[n, part * half // 2:(part + 1) * half // 2, :])))
                    tick()
                r = jnp.concatenate(r, axis=1)
                acc = r if acc is None else acc + r
            xa_s[s, NB:, :] = acc[nmem:]
            return acc[0:nmem]

        def step_body(i, mem):
            for t in range(mod_per_it):
                mod_copy(2 * kt_n + i * mod_per_it + t, jt_n).start()
            for n, cp in enumerate((cp_w1, cp_w2, cp_w3, cp_w4)):
                pl.when(i == n)(cp.start)
            for u in range(UNROLL):
                mem = step(i * UNROLL + u, mem)
            return mem

        jax.lax.fori_loop(0, nseg // UNROLL, step_body, mem0_ref[...].astype(F32))

    pl.run_scoped(
        attention,
        pltpu.VMEM((3, nh, dm // 2, dh), U32),
        pltpu.VMEM((3, hp_n, nseg, 2 * NB, dh), BF16),
        pltpu.VMEM((nseg, NB, dm), BF16),
        pltpu.VMEM((7, nseg * NB // 2, dm // 2), BF16),
        pltpu.VMEM((2 * (seg + NB), 2 * (seg + NB)), F32),
        pltpu.VMEM((nseg, seg - NB, dm), F32),
        pltpu.VMEM((seg, nh * dh), BF16),
        pltpu.VMEM((3, RING, dm, dh), U32),
        pltpu.VMEM((kt_n, nseg * NB, 128), F32),
    )

    spc = CH // seg
    nch = nseg // spc
    hc = CH // 2
    sh = spc // 2
    dm2, ff2 = dm // 2, ff // 2
    ft_n, nt_n = ff2 // 128, dm2 // 128

    def mlp(w3x_s, w4x_s, h_s, g_s, out_s, a3_s, a4_s, att_s, u_s, w1x_s, w2x_s):
        zero_halo = jnp.zeros((kt_n, HALO, 128), F32)
        g_s[:, 0:HALO, :] = zero_halo
        g_s[:, HALO + nseg * seg:, :] = zero_halo
        sc = silu_c()
        rest = wmod_s.at[2 * kt_n:]
        pltpu.make_async_copy(rest, rest, sem_mod.at[kt_n // 2]).wait()

        def weight_sum_jobs(w_s, wx_s, ci, parts=nch):
            k2, n2 = w_s.shape[0] // 2, w_s.shape[1] // 2
            nr = k2 // parts

            def job(r, c0):
                r0 = pl.multiple_of(ci * nr + r, 16)
                quad = [w_s[pl.ds(r0 + kk, 16), nn + c0:nn + c0 + 256].astype(F32)
                        for kk in (0, k2) for nn in (0, n2)]
                for i, t in _rhs_sums(*quad).items():
                    if i == 2:
                        w_s[pl.ds(r0, 16), n2 + c0:n2 + c0 + 256] = t.astype(BF16)
                    else:
                        wx_s[_RHS_SLOT[i], pl.ds(r0, 16), c0:c0 + 256] = t.astype(BF16)

            return [functools.partial(job, r, c0) for c0 in range(0, n2, 256) for r in range(0, nr, 16)]

        def rhs(w_s, wx_s, i, j):
            k2, n2 = w_s.shape[0] // 2, w_s.shape[1] // 2
            if i == 1:
                return w_s[0:k2, 128 * j:128 * (j + 1)]
            if i == 2:
                return w_s[0:k2, n2 + 128 * j:n2 + 128 * (j + 1)]
            if i == 4:
                return w_s[k2:, n2 + 128 * j:n2 + 128 * (j + 1)]
            return wx_s[_RHS_SLOT[i], :, 128 * j:128 * (j + 1)]

        def spread(jobs, n, slots=kt_n):
            for job in jobs[len(jobs) * n // slots:len(jobs) * (n + 1) // slots]:
                job()

        def halves(v):
            m2, k2 = v.shape[0] // 2, v.shape[1] // 2
            return v[:m2, :k2], v[:m2, k2:], v[m2:, :k2], v[m2:, k2:]

        cp_w1.wait()
        cp_w2.wait()
        cp_w3.wait()
        cp_w4.wait()

        def mod_body(i, carry):
            jobs = weight_sum_jobs(w1_s, w1x_s, i - 2, 4)
            for k in range(kt_n):
                r = _dot(sc, _halfs(wmod_s[i * kt_n + k]))[0:8]
                spread(jobs, k)
                mod_s[i, :, 128 * k:128 * (k + 1)] = jnp.where(i == 4, 1.0 + r, r)
            return carry

        jax.lax.fori_loop(2, 6, mod_body, 0)

        def stage_a(ci, carry):
            def out_proj(half, jobs):
                lo = ob_s[pl.ds(ci * spc + half * sh, sh)].reshape(sh * NB, nh * dh)
                for n in range(kt_n):
                    att_s[half, :, 128 * n:128 * (n + 1)] = _dot(lo, _halfs(wo_s[n]))
                    spread(jobs, n)

            def norm(half, i):
                si = ci * spc + half * sh + i
                att = jnp.concatenate([att_s[half, NB * i:NB * (i + 1), :], xa_s[si, NB:, :]], axis=0)
                xa = x_s[si].astype(F32) + _rows(mod_s[2], seg) * att
                xa_s[si] = xa
                h = _layernorm(xa) * _rows(mod_s[4], seg) + _rows(mod_s[3], seg)
                h_s[pl.ds(pl.multiple_of(si * seg, seg), seg), :] = h
                return _layernorm(h)

            def norm_pair(half, i):
                top, bot = norm(half, i), norm(half, i + sh // 2)
                for t, v in enumerate(_lhs_terms(top[:, :dm2], top[:, dm2:], bot[:, :dm2], bot[:, dm2:])):
                    u_s[half, t, seg * i:seg * (i + 1), :] = v.astype(BF16)

            def mix_in(half, jobs):
                r0 = pl.multiple_of(ci * CH + half * hc, hc)
                for n in range(nt_n):
                    res = _strassen(lambda i: _dot(u_s[half, i], rhs(w1_s, w1x_s, i, n)))
                    for q, t in enumerate(res):
                        g_s[n + (q % 2) * nt_n, pl.ds(r0 + HALO + (q // 2) * (hc // 2), hc // 2), :] = _gelu(t)
                    spread(jobs, n, nt_n)

            idle = [lambda: None]
            out_proj(0, weight_sum_jobs(w3_s, w3x_s, ci) + weight_sum_jobs(w2_s, w2x_s, ci))
            out_proj(1, [functools.partial(norm_pair, 0, i) for i in range(sh // 2)] + idle * 2)
            mix_in(0, [functools.partial(norm_pair, 1, i) for i in range(sh // 2)] + idle * 2)
            mix_in(1, weight_sum_jobs(w4_s, w4x_s, ci) + idle * 10)
            return carry

        jax.lax.fori_loop(0, nch, stage_a, 0)

        def out_copy(ci):
            r0 = pl.multiple_of(ci * CH, CH)
            return pltpu.make_async_copy(out_s.at[pl.ds(r0, CH)], out_hbm.at[pl.ds(r0, CH)], sem_misc.at[8])

        def stage_b(ci, carry):
            shifts = (-1, 1, -2, 2)
            x1, u = [], []
            for half in range(2):
                r0 = pl.multiple_of(ci * CH + half * hc, hc)
                gs = jnp.concatenate(
                    [g_s[k, pl.ds(r0 + HALO + shifts[k * 4 // kt_n], hc), :] for k in range(kt_n)], axis=1)
                terms = [t.astype(BF16) for t in _lhs_terms(*halves(gs))]
                res = [_strassen(lambda i: _dot(terms[i], rhs(w2_s, w2x_s, i, n))) for n in range(nt_n)]
                hs = jnp.concatenate(
                    [jnp.concatenate([r[q] for r in res] + [r[q + 1] for r in res], axis=1) for q in (0, 2)],
                    axis=0)
                x1.append(h_s[pl.ds(r0, hc), :] + hs)
                u.append(_layernorm(x1[-1]))
            for i, t in enumerate(_lhs_terms(u[0][:, :dm2], u[0][:, dm2:], u[1][:, :dm2], u[1][:, dm2:])):
                a3_s[i] = t.astype(BF16)

            def prod3(j, i):
                return _dot(a3_s[i], rhs(w3_s, w3x_s, i, j))

            early = {j: (prod3(j, 2), prod3(j, 4)) for j in range(4)}
            for j in range(ft_n):
                act = [_gelu(t) for t in _strassen(functools.partial(prod3, j), *early.get(j, ()))]
                for i, t in enumerate(_lhs_terms(*act)):
                    a4_s[i, :, 128 * j:128 * (j + 1)] = t.astype(BF16)

            def prod4(n, i):
                return _dot(a4_s[i], rhs(w4_s, w4x_s, i, n))

            for n in range(nt_n):
                for q, t in enumerate(_strassen(functools.partial(prod4, n))):
                    half, c0 = q // 2, (q % 2) * dm2 + 128 * n
                    r0 = pl.multiple_of(ci * CH + half * hc, hc)
                    xa = xa_s[pl.ds(ci * spc + half * sh, sh), :, c0:c0 + 128].reshape(hc, 128)
                    y = x1[half][:, c0:c0 + 128] + t
                    out_s[pl.ds(r0, hc), c0:c0 + 128] = (xa + _rows(mod_s[5, :, c0:c0 + 128], hc) * y).astype(BF16)
            out_copy(ci).start()
            return carry

        jax.lax.fori_loop(0, nch, stage_b, 0)
        for ci in range(nch):
            out_copy(ci).wait()

    pl.run_scoped(
        mlp,
        pltpu.VMEM((4, dm2, ff2), BF16),
        pltpu.VMEM((4, ff2, dm2), BF16),
        pltpu.VMEM((nseg * seg, dm), F32),
        pltpu.VMEM((kt_n, nseg * seg + 2 * HALO, 128), F32),
        pltpu.VMEM((nseg * seg, dm), BF16),
        pltpu.VMEM((7, hc, dm2), BF16),
        pltpu.VMEM((7, hc, ff2), BF16),
        pltpu.VMEM((2, sh * NB, dm), F32),
        pltpu.VMEM((2, 7, hc // 2, dm2), BF16),
        pltpu.VMEM((4, dm2, dm2), BF16),
        pltpu.VMEM((4, dm2, dm2), BF16),
    )


@functools.partial(jax.jit, static_argnames=("A_seg_len",))
def pallas_adaLN_cond__memory_aug_recurrent_mem_tr__mixer_s_mlp__prompt_kernel(
    A_x: jax.Array,
    A_mem0: jax.Array,
    A_Wq: jax.Array,
    A_Wk: jax.Array,
    A_Wv: jax.Array,
    A_Wo: jax.Array,
    A_seg_len: int,
    B_x: jax.Array,
    B_w1: jax.Array,
    B_w2: jax.Array,
    B_w3: jax.Array,
    B_w4: jax.Array,
    c: jax.Array,
    w_mod: jax.Array,
):
    del B_x
    b, s, dm = A_x.shape
    _, nh, dh = A_Wq.shape
    nmem = A_mem0.shape[1]
    seg = int(A_seg_len)
    nseg = s // seg
    ff = B_w3.shape[1]
    assert (b, seg, nmem, dh) == (1, 32, NB, 128) and s % CH == 0 and dm % 512 == 0 and nh % 2 == 0
    hp_n = nh // 2
    kt_n = dm // 128
    hbm = pl.BlockSpec(memory_space=pl.ANY)
    out = pl.pallas_call(
        functools.partial(_kernel, nseg=nseg, seg=seg, nmem=nmem, dm=dm, nh=nh, dh=dh),
        out_shape=jax.ShapeDtypeStruct((s, dm), BF16),
        in_specs=[hbm] * 12,
        out_specs=hbm,
        scratch_shapes=[
            pltpu.VMEM((kt_n, nh * dh // 2, 128), U32),
            pltpu.VMEM((dm, dm), BF16),
            pltpu.VMEM((dm, dm), BF16),
            pltpu.VMEM((dm, ff), BF16),
            pltpu.VMEM((ff, dm), BF16),
            pltpu.VMEM((6 * kt_n, dm // 2, 128), U32),
            pltpu.VMEM((nseg, seg, dm), BF16),
            pltpu.VMEM((nseg, NB, nh * dh), BF16),
            pltpu.VMEM((nseg, seg, dm), F32),
            pltpu.VMEM((6, 8, dm), F32),
            pltpu.VMEM((1, dm), BF16),
            pltpu.VMEM((nmem, dm), BF16),
            pltpu.SemaphoreType.DMA((RING,)),
            pltpu.SemaphoreType.DMA((9,)),
            pltpu.SemaphoreType.DMA((kt_n // 2 + 1,)),
        ],
        compiler_params=pltpu.CompilerParams(vmem_limit_bytes=120 * 1024 * 1024),
    )(A_x.reshape(nseg, seg, dm), A_mem0.reshape(nmem, dm), A_Wq, A_Wk, A_Wv,
      A_Wo.reshape(nh * dh, dm), B_w1, B_w2, B_w3, B_w4, c, w_mod)
    return out.reshape(b, s, dm)
```

```python
import functools
import math

import jax
import jax.numpy as jnp
import numpy as np
import jax.experimental.pallas as pl
import jax.experimental.pallas.tpu as pltpu

F32 = jnp.float32
BF16 = jnp.bfloat16
U32 = jnp.uint32

HIGH_HALF = np.uint32(0xFFFF0000)
LN_EPS = 1e-5
MASK_FILL = -1000000000.0
NB = 8
CH = 256
LAG_S, LAG_PV, GRP, ORDER, UNROLL = 4, 8, 0, (1, 0, 2), 2
RING = 4
HALO = 8


def _dot(a, b):
    return jnp.dot(a, b, preferred_element_type=F32)


def _dot_nt(a, b):
    return jax.lax.dot_general(a, b, (((1,), (1,)), ((), ())), preferred_element_type=F32)


def _layernorm(x):
    m = jnp.mean(x, axis=-1, keepdims=True)
    d = x - m
    v = jnp.mean(d * d, axis=-1, keepdims=True)
    return d * jax.lax.rsqrt(v + LN_EPS)


def _gelu(x):
    k0 = math.sqrt(2.0 / math.pi)
    t = jnp.tanh(x * (k0 + (k0 * 0.044715) * (x * x)))
    hx = 0.5 * x
    return hx + hx * t


def _rows(v, n):
    return jnp.concatenate([v] * (n // 8), axis=0) if n > 8 else v


def _halfs(w):
    return pltpu.bitcast(w, BF16)


def _lhs_terms(a11, a12, a21, a22):
    return [a11 + a22, a21 + a22, a11, a22, a11 + a12, a21 - a11, a12 - a22]


def _rhs_sums(b11, b12, b21, b22):
    return {0: b11 + b22, 2: b12 - b22, 3: b21 - b11, 5: b11 + b12, 6: b21 + b22}


_RHS_SLOT = {0: 0, 3: 1, 5: 2, 6: 3}


def _strassen(prod, m2=None, m4=None):
    m2 = prod(2) if m2 is None else m2
    m4 = prod(4) if m4 is None else m4
    c12 = m2 + m4
    m0 = prod(0)
    t11 = m0 - m4
    t22 = m0 + m2
    m3 = prod(3)
    t11 = t11 + m3
    c11 = t11 + prod(6)
    m1 = prod(1)
    c21 = m1 + m3
    t22 = t22 - m1
    c22 = t22 + prod(5)
    return c11, c12, c21, c22


def _kernel(x_hbm, mem0_hbm, wq_hbm, wk_hbm, wv_hbm, wo_hbm, w1_hbm, w2_hbm, w3_hbm, w4_hbm,
            c_hbm, wmod_hbm, out_hbm,
            wo_s, w1_s, w2_s, w3_s, w4_s, wmod_s, x_s, ob_s, xa_s, mod_s, c_ref, mem0_ref,
            sem_qkv, sem_misc, sem_mod,
            *, nseg, seg, nmem, dm, nh, dh):
    hp_n = nh // 2
    kt_n = dm // 128
    ff = w3_s.shape[1]
    scale = dh ** -0.5
    w_u32 = [w.bitcast(U32) for w in (wq_hbm, wk_hbm, wv_hbm)]
    wo_u32 = wo_hbm.bitcast(U32)

    def wo_copy(i):
        n, per = i & (kt_n - 1), wo_s.shape[1] * kt_n // hp_n
        rows = pl.ds(pl.multiple_of((i >> (kt_n.bit_length() - 1)) * per, per), per)
        return pltpu.make_async_copy(wo_u32.at[rows, pl.ds(pl.multiple_of(n * 128, 128), 128)],
                                     wo_s.at[n, rows], sem_misc.at[0])

    wmod_u32 = wmod_hbm.bitcast(U32)

    def mod_copy(t, group):
        return pltpu.make_async_copy(wmod_u32.at[:, pl.ds(pl.multiple_of(t * 128, 128), 128)],
                                     wmod_s.at[t], sem_mod.at[group])

    cp_c = pltpu.make_async_copy(c_hbm, c_ref, sem_misc.at[2])
    cp_mem0 = pltpu.make_async_copy(mem0_hbm, mem0_ref, sem_misc.at[3])
    cp_w1 = pltpu.make_async_copy(w1_hbm, w1_s, sem_misc.at[4])
    cp_w2 = pltpu.make_async_copy(w2_hbm, w2_s, sem_misc.at[5])
    cp_w3 = pltpu.make_async_copy(w3_hbm, w3_s, sem_misc.at[6])
    cp_w4 = pltpu.make_async_copy(w4_hbm, w4_s, sem_misc.at[7])

    def silu_c():
        cv = c_ref[...].astype(F32)
        return jnp.broadcast_to(cv * jax.nn.sigmoid(cv), (16, dm)).astype(BF16)

    def attention(wqkv, qkvb, xb_s, hb_s, fill_s, hx_s, o_s, raw_s, ln_s):
        xs_n = nseg // hp_n

        def pair_copies(hp):
            cps = [pltpu.make_async_copy(w_u32[w].at[:, hp, :], raw_s.at[w, hp & (RING - 1)], sem_qkv.at[hp & (RING - 1)])
                   for w in range(3)]
            rows = pl.ds(hp * xs_n, xs_n)
            return cps + [pltpu.make_async_copy(x_hbm.at[rows], x_s.at[rows], sem_qkv.at[hp & (RING - 1)])]

        cp_xb = pltpu.make_async_copy(x_hbm.at[:, 0:NB, :], xb_s, sem_misc.at[1])
        cp_xb.start()
        cp_c.start()
        cp_mem0.start()
        jt_n = kt_n // 2

        def mod_group(j):
            return [mod_copy(j + t * jt_n, j) for t in range(4)]

        for cp in mod_group(0):
            cp.start()

        def head_pos(i):
            head = jnp.where(i < 2 * seg, i // seg, (i - 2 * seg) // NB)
            r = i % seg
            pos = jnp.where(i < 2 * seg, jnp.where(r < nmem, r, r + NB), nmem + i % NB)
            return head, pos

        nq = 2 * (seg + NB)
        qh, qp = head_pos(jax.lax.broadcasted_iota(jnp.int32, (nq, nq), 0))
        kh, kp = head_pos(jax.lax.broadcasted_iota(jnp.int32, (nq, nq), 1))
        visible = (qp < nmem) | (qp >= kp)
        fill_s[...] = jnp.where(qh == kh, jnp.where(visible, 0.0, MASK_FILL / scale), -jnp.inf).astype(F32)

        mh, kh = nseg * NB // 2, dm // 2
        cp_c.wait()
        cp_mem0.wait()
        sc = silu_c()
        for cp in mod_group(1):
            cp.start()
        cp_xb.wait()
        for cp in mod_group(2):
            cp.start()

        def ln_body(i, carry):
            s0 = i * (nseg // 4)
            ln = _layernorm(xb_s[pl.ds(s0, nseg // 4)].astype(F32).reshape(mh // 2, dm))
            for k in range(kt_n):
                ln_s[k, pl.ds(pl.multiple_of(i * (mh // 2), mh // 2), mh // 2), :] = ln[:, 128 * k:128 * (k + 1)]
            return carry

        jax.lax.fori_loop(0, 4, ln_body, 0)

        def shift_scale_body(j, carry):
            for cp in mod_group(j):
                cp.wait()

            @pl.when(j == 0)
            def _():
                for cp in mod_group(3):
                    cp.start()

            @pl.when(j == 1)
            def _():
                for cp in pair_copies(0):
                    cp.start()

            shift, gain = [], []
            for k in (j, j + jt_n):
                cols = pl.ds(pl.multiple_of(k * 128, 128), 128)
                shift.append(_dot(sc, _halfs(wmod_s[k]))[0:8])
                gain.append(1.0 + _dot(sc, _halfs(wmod_s[kt_n + k]))[0:8])
                mod_s[0, :, cols] = shift[-1]
                mod_s[1, :, cols] = gain[-1]
            for r in range(0, mh, 32):
                quad = [ln_s[j + t * jt_n, r0 + r:r0 + r + 32, :] * _rows(gain[t], 32) + _rows(shift[t], 32)
                        for r0 in (0, mh) for t in range(2)]
                for i, t in enumerate(_lhs_terms(*quad)):
                    hb_s[i, r:r + 32, pl.ds(pl.multiple_of(j * 128, 128), 128)] = t.astype(BF16)
            return carry

        jax.lax.fori_loop(0, jt_n, shift_scale_body, 0)

        def head_w(w, hp, j, rows=slice(None)):
            return _halfs(wqkv[w, 2 * hp + j, rows, :])

        def bulk_body(hp, carry):
            for cp in pair_copies(hp):
                cp.wait()

            @pl.when(hp == 0)
            def _():
                for cp in pair_copies(1) + [wo_copy(0)]:
                    cp.start()

            @pl.when(hp + 2 < hp_n)
            def _():
                for cp in pair_copies(hp + 2):
                    cp.start()

            pl.when(hp + 1 < hp_n)(lambda: wo_copy(hp + 1).start())
            slot = hp & (RING - 1)
            for w in range(3):
                def quad(i):
                    word = raw_s[w, slot, (i // 2) * kh:(i // 2 + 1) * kh, :]
                    return pltpu.bitcast(word & HIGH_HALF if i % 2 else word << 16, F32)

                def prod(i):
                    q = [quad(j) for j in range(4)]
                    return _dot(hb_s[i], {1: q[0], 4: q[3], **_rhs_sums(*q)}[i].astype(BF16))

                m4 = prod(4)
                res = [t.reshape(nseg // 2, NB, dh) for t in _strassen(prod, None, m4)]
                for r in range(0, dm, 16):
                    a = raw_s[w, slot, pl.ds(r, 8, stride=2), :]
                    b = raw_s[w, slot, pl.ds(r + 1, 8, stride=2), :]
                    wqkv[w, 2 * hp, r // 2:r // 2 + 8, :] = (a & 0xFFFF) | (b << 16)
                    wqkv[w, 2 * hp + 1, r // 2:r // 2 + 8, :] = (a >> 16) | (b & HIGH_HALF)
                for i in range(xs_n * w // 3, xs_n * (w + 1) // 3):
                    xs = x_s[hp * xs_n + i, NB:, :].astype(F32)
                    hx_s[hp * xs_n + i] = _layernorm(xs) * _rows(mod_s[1], seg - NB) + _rows(mod_s[0], seg - NB)
                qkvb[w, hp, :nseg // 2] = jnp.concatenate(res[:2], axis=1).astype(BF16)
                qkvb[w, hp, nseg // 2:] = jnp.concatenate(res[2:], axis=1).astype(BF16)
            return carry

        jax.lax.fori_loop(0, hp_n, bulk_body, 0)

        pltpu.make_async_copy(wo_s, wo_s, sem_misc.at[0]).wait()

        mod_per_it = 4 * kt_n * UNROLL // nseg
        exp_c = scale * math.log2(math.e)

        def step(s, mem):
            a = jnp.concatenate([mem, hx_s[s]], axis=0)
            a = [a[:, :kh].astype(BF16), a[:, kh:].astype(BF16)]

            first = [_dot(a[t], jnp.concatenate(
                [head_w(w, 0, j, slice(t * kh // 2, (t + 1) * kh // 2)) for w in ORDER for j in range(2)], axis=1))
                for t in range(2)]

            def proj(w, hp):
                if hp == 0:
                    c0 = [(2 * ORDER.index(w) + j) * dh for j in range(2)]
                    r = [first[0][:, c:c + dh] + first[1][:, c:c + dh] for c in c0]
                else:
                    r = [_dot(a[0], head_w(w, hp, j, slice(0, kh // 2)))
                         + _dot(a[1], head_w(w, hp, j, slice(kh // 2, kh))) for j in range(2)]
                return jnp.concatenate(r + [qkvb[w, hp, s].astype(F32)], axis=0).astype(BF16)

            def probs(q, k):
                fill = fill_s[...]
                sco = jnp.where(fill == 0.0, _dot_nt(q, k), fill)
                e = jnp.exp2((sco - jnp.max(sco, axis=-1, keepdims=True)) * exp_c)
                den = jnp.sum(e, axis=-1, keepdims=True)
                inv = pl.reciprocal(den, approx=True)
                return e.astype(BF16), inv * (2.0 - den * inv)

            def attend(hp, p, v):
                o = _dot(p[0], v) * p[1]
                cols = slice(2 * hp * dh, 2 * (hp + 1) * dh)
                o_s[:, cols] = jnp.concatenate([o[0:seg], o[seg:2 * seg]], axis=1).astype(BF16)
                ob_s[s, :, cols] = jnp.concatenate(
                    [o[2 * seg:2 * seg + NB], o[2 * seg + NB:]], axis=1).astype(BF16)

            val, ps = {}, {}
            clock = [0]

            def tick():
                t = clock[0]
                clock[0] += 1
                for i in range(hp_n):
                    if t == 3 * (i | GRP) + LAG_S:
                        ps[i] = probs(val.pop((0, i)), val.pop((1, i)))
                for i in range(hp_n):
                    if t == 3 * (i | GRP) + LAG_PV:
                        attend(i, ps.pop(i), val.pop((2, i)))

            for hp in range(hp_n):
                for w in ORDER:
                    val[w, hp] = proj(w, hp)
                    tick()
            half = nh * dh // 2
            acc = None
            for part in range(2):
                assert part == 0 or not val
                lo = o_s[:, part * half:(part + 1) * half]
                r = []
                for n in range(kt_n):
                    r.append(_dot(lo, _halfs(wo_s[n, part * half // 2:(part + 1) * half // 2, :])))
                    tick()
                r = jnp.concatenate(r, axis=1)
                acc = r if acc is None else acc + r
            xa_s[s, NB:, :] = acc[nmem:]
            return acc[0:nmem]

        def step_body(i, mem):
            for t in range(mod_per_it):
                mod_copy(2 * kt_n + i * mod_per_it + t, jt_n).start()
            for n, cp in enumerate((cp_w1, cp_w2, cp_w3, cp_w4)):
                pl.when(i == n)(cp.start)
            for u in range(UNROLL):
                mem = step(i * UNROLL + u, mem)
            return mem

        jax.lax.fori_loop(0, nseg // UNROLL, step_body, mem0_ref[...].astype(F32))

    pl.run_scoped(
        attention,
        pltpu.VMEM((3, nh, dm // 2, dh), U32),
        pltpu.VMEM((3, hp_n, nseg, 2 * NB, dh), BF16),
        pltpu.VMEM((nseg, NB, dm), BF16),
        pltpu.VMEM((7, nseg * NB // 2, dm // 2), BF16),
        pltpu.VMEM((2 * (seg + NB), 2 * (seg + NB)), F32),
        pltpu.VMEM((nseg, seg - NB, dm), F32),
        pltpu.VMEM((seg, nh * dh), BF16),
        pltpu.VMEM((3, RING, dm, dh), U32),
        pltpu.VMEM((kt_n, nseg * NB, 128), F32),
    )

    spc = CH // seg
    nch = nseg // spc
    hc = CH // 2
    sh = spc // 2
    dm2, ff2 = dm // 2, ff // 2
    ft_n, nt_n = ff2 // 128, dm2 // 128

    def mlp(w3x_s, w4x_s, h_s, g_s, out_s, a3_s, a4_s, att_s, u_s, w1x_s, w2x_s):
        zero_halo = jnp.zeros((kt_n, HALO, 128), F32)
        g_s[:, 0:HALO, :] = zero_halo
        g_s[:, HALO + nseg * seg:, :] = zero_halo
        sc = silu_c()
        rest = wmod_s.at[2 * kt_n:]
        pltpu.make_async_copy(rest, rest, sem_mod.at[kt_n // 2]).wait()

        def weight_sum_jobs(w_s, wx_s, ci, parts=nch):
            k2, n2 = w_s.shape[0] // 2, w_s.shape[1] // 2
            nr = k2 // parts

            def job(r, c0):
                r0 = pl.multiple_of(ci * nr + r, 16)
                quad = [w_s[pl.ds(r0 + kk, 16), nn + c0:nn + c0 + 256].astype(F32)
                        for kk in (0, k2) for nn in (0, n2)]
                for i, t in _rhs_sums(*quad).items():
                    if i == 2:
                        w_s[pl.ds(r0, 16), n2 + c0:n2 + c0 + 256] = t.astype(BF16)
                    else:
                        wx_s[_RHS_SLOT[i], pl.ds(r0, 16), c0:c0 + 256] = t.astype(BF16)

            return [functools.partial(job, r, c0) for c0 in range(0, n2, 256) for r in range(0, nr, 16)]

        def rhs(w_s, wx_s, i, j):
            k2, n2 = w_s.shape[0] // 2, w_s.shape[1] // 2
            if i == 1:
                return w_s[0:k2, 128 * j:128 * (j + 1)]
            if i == 2:
                return w_s[0:k2, n2 + 128 * j:n2 + 128 * (j + 1)]
            if i == 4:
                return w_s[k2:, n2 + 128 * j:n2 + 128 * (j + 1)]
            return wx_s[_RHS_SLOT[i], :, 128 * j:128 * (j + 1)]

        def spread(jobs, n, slots=kt_n):
            for job in jobs[len(jobs) * n // slots:len(jobs) * (n + 1) // slots]:
                job()

        def halves(v):
            m2, k2 = v.shape[0] // 2, v.shape[1] // 2
            return v[:m2, :k2], v[:m2, k2:], v[m2:, :k2], v[m2:, k2:]

        cp_w1.wait()
        cp_w2.wait()
        cp_w3.wait()
        cp_w4.wait()

        def mod_body(i, carry):
            jobs = weight_sum_jobs(w1_s, w1x_s, i - 2, 4)
            for k in range(kt_n):
                r = _dot(sc, _halfs(wmod_s[i * kt_n + k]))[0:8]
                spread(jobs, k)
                mod_s[i, :, 128 * k:128 * (k + 1)] = jnp.where(i == 4, 1.0 + r, r)
            return carry

        jax.lax.fori_loop(2, 6, mod_body, 0)

        def stage_a(ci, carry):
            def out_proj(half, jobs):
                lo = ob_s[pl.ds(ci * spc + half * sh, sh)].reshape(sh * NB, nh * dh)
                for n in range(kt_n):
                    att_s[half, :, 128 * n:128 * (n + 1)] = _dot(lo, _halfs(wo_s[n]))
                    spread(jobs, n)

            def norm(half, i):
                si = ci * spc + half * sh + i
                att = jnp.concatenate([att_s[half, NB * i:NB * (i + 1), :], xa_s[si, NB:, :]], axis=0)
                xa = x_s[si].astype(F32) + _rows(mod_s[2], seg) * att
                xa_s[si] = xa
                h = _layernorm(xa) * _rows(mod_s[4], seg) + _rows(mod_s[3], seg)
                h_s[pl.ds(pl.multiple_of(si * seg, seg), seg), :] = h
                return _layernorm(h)

            def norm_pair(half, i):
                top, bot = norm(half, i), norm(half, i + sh // 2)
                for t, v in enumerate(_lhs_terms(top[:, :dm2], top[:, dm2:], bot[:, :dm2], bot[:, dm2:])):
                    u_s[half, t, seg * i:seg * (i + 1), :] = v.astype(BF16)

            def mix_in(half, jobs):
                r0 = pl.multiple_of(ci * CH + half * hc, hc)
                for n in range(nt_n):
                    res = _strassen(lambda i: _dot(u_s[half, i], rhs(w1_s, w1x_s, i, n)))
                    for q, t in enumerate(res):
                        g_s[n + (q % 2) * nt_n, pl.ds(r0 + HALO + (q // 2) * (hc // 2), hc // 2), :] = _gelu(t)
                    spread(jobs, n, nt_n)

            idle = [lambda: None]
            out_proj(0, weight_sum_jobs(w3_s, w3x_s, ci) + weight_sum_jobs(w2_s, w2x_s, ci))
            out_proj(1, [functools.partial(norm_pair, 0, i) for i in range(sh // 2)] + idle * 2)
            mix_in(0, [functools.partial(norm_pair, 1, i) for i in range(sh // 2)] + idle * 2)
            mix_in(1, weight_sum_jobs(w4_s, w4x_s, ci) + idle * 10)
            return carry

        jax.lax.fori_loop(0, nch, stage_a, 0)

        def out_copy(ci):
            r0 = pl.multiple_of(ci * CH, CH)
            return pltpu.make_async_copy(out_s.at[pl.ds(r0, CH)], out_hbm.at[pl.ds(r0, CH)], sem_misc.at[8])

        def stage_b(ci, carry):
            shifts = (-1, 1, -2, 2)
            x1, u = [], []
            for half in range(2):
                r0 = pl.multiple_of(ci * CH + half * hc, hc)
                gs = jnp.concatenate(
                    [g_s[k, pl.ds(r0 + HALO + shifts[k * 4 // kt_n], hc), :] for k in range(kt_n)], axis=1)
                terms = [t.astype(BF16) for t in _lhs_terms(*halves(gs))]
                res = [_strassen(lambda i: _dot(terms[i], rhs(w2_s, w2x_s, i, n))) for n in range(nt_n)]
                hs = jnp.concatenate(
                    [jnp.concatenate([r[q] for r in res] + [r[q + 1] for r in res], axis=1) for q in (0, 2)],
                    axis=0)
                x1.append(h_s[pl.ds(r0, hc), :] + hs)
                u.append(_layernorm(x1[-1]))
            for i, t in enumerate(_lhs_terms(u[0][:, :dm2], u[0][:, dm2:], u[1][:, :dm2], u[1][:, dm2:])):
                a3_s[i] = t.astype(BF16)

            def prod3(j, i):
                return _dot(a3_s[i], rhs(w3_s, w3x_s, i, j))

            early = {j: (prod3(j, 2), prod3(j, 4)) for j in range(4)}
            for j in range(ft_n):
                act = [_gelu(t) for t in _strassen(functools.partial(prod3, j), *early.get(j, ()))]
                for i, t in enumerate(_lhs_terms(*act)):
                    a4_s[i, :, 128 * j:128 * (j + 1)] = t.astype(BF16)

            def prod4(n, i):
                return _dot(a4_s[i], rhs(w4_s, w4x_s, i, n))

            for n in range(nt_n):
                for q, t in enumerate(_strassen(functools.partial(prod4, n))):
                    half, c0 = q // 2, (q % 2) * dm2 + 128 * n
                    r0 = pl.multiple_of(ci * CH + half * hc, hc)
                    xa = xa_s[pl.ds(ci * spc + half * sh, sh), :, c0:c0 + 128].reshape(hc, 128)
                    y = x1[half][:, c0:c0 + 128] + t
                    out_s[pl.ds(r0, hc), c0:c0 + 128] = (xa + _rows(mod_s[5, :, c0:c0 + 128], hc) * y).astype(BF16)
            out_copy(ci).start()
            return carry

        jax.lax.fori_loop(0, nch, stage_b, 0)
        for ci in range(nch):
            out_copy(ci).wait()

    pl.run_scoped(
        mlp,
        pltpu.VMEM((4, dm2, ff2), BF16),
        pltpu.VMEM((4, ff2, dm2), BF16),
        pltpu.VMEM((nseg * seg, dm), F32),
        pltpu.VMEM((kt_n, nseg * seg + 2 * HALO, 128), F32),
        pltpu.VMEM((nseg * seg, dm), BF16),
        pltpu.VMEM((7, hc, dm2), BF16),
        pltpu.VMEM((7, hc, ff2), BF16),
        pltpu.VMEM((2, sh * NB, dm), F32),
        pltpu.VMEM((2, 7, hc // 2, dm2), BF16),
        pltpu.VMEM((4, dm2, dm2), BF16),
        pltpu.VMEM((4, dm2, dm2), BF16),
    )


@functools.partial(jax.jit, static_argnames=("A_seg_len",))
def pallas_adaLN_cond__memory_aug_recurrent_mem_tr__mixer_s_mlp__prompt_kernel(
    A_x: jax.Array,
    A_mem0: jax.Array,
    A_Wq: jax.Array,
    A_Wk: jax.Array,
    A_Wv: jax.Array,
    A_Wo: jax.Array,
    A_seg_len: int,
    B_x: jax.Array,
    B_w1: jax.Array,
    B_w2: jax.Array,
    B_w3: jax.Array,
    B_w4: jax.Array,
    c: jax.Array,
    w_mod: jax.Array,
):
    del B_x
    b, s, dm = A_x.shape
    _, nh, dh = A_Wq.shape
    nmem = A_mem0.shape[1]
    seg = int(A_seg_len)
    nseg = s // seg
    ff = B_w3.shape[1]
    assert (b, seg, nmem, dh) == (1, 32, NB, 128) and s % CH == 0 and dm % 512 == 0 and nh % 2 == 0
    hp_n = nh // 2
    kt_n = dm // 128
    hbm = pl.BlockSpec(memory_space=pl.ANY)
    out = pl.pallas_call(
        functools.partial(_kernel, nseg=nseg, seg=seg, nmem=nmem, dm=dm, nh=nh, dh=dh),
        out_shape=jax.ShapeDtypeStruct((s, dm), BF16),
        in_specs=[hbm] * 12,
        out_specs=hbm,
        scratch_shapes=[
            pltpu.VMEM((kt_n, nh * dh // 2, 128), U32),
            pltpu.VMEM((dm, dm), BF16),
            pltpu.VMEM((dm, dm), BF16),
            pltpu.VMEM((dm, ff), BF16),
            pltpu.VMEM((ff, dm), BF16),
            pltpu.VMEM((6 * kt_n, dm // 2, 128), U32),
            pltpu.VMEM((nseg, seg, dm), BF16),
            pltpu.VMEM((nseg, NB, nh * dh), BF16),
            pltpu.VMEM((nseg, seg, dm), F32),
            pltpu.VMEM((6, 8, dm), F32),
            pltpu.VMEM((1, dm), BF16),
            pltpu.VMEM((nmem, dm), BF16),
            pltpu.SemaphoreType.DMA((RING,)),
            pltpu.SemaphoreType.DMA((9,)),
            pltpu.SemaphoreType.DMA((kt_n // 2 + 1,)),
        ],
        compiler_params=pltpu.CompilerParams(vmem_limit_bytes=120 * 1024 * 1024),
    )(A_x.reshape(nseg, seg, dm), A_mem0.reshape(nmem, dm), A_Wq, A_Wk, A_Wv,
      A_Wo.reshape(nh * dh, dm), B_w1, B_w2, B_w3, B_w4, c, w_mod)
    return out.reshape(b, s, dm)
```

```python
import functools
import math

import jax
import jax.numpy as jnp
import numpy as np
import jax.experimental.pallas as pl
import jax.experimental.pallas.tpu as pltpu

F32 = jnp.float32
BF16 = jnp.bfloat16
U32 = jnp.uint32

HIGH_HALF = np.uint32(0xFFFF0000)
LN_EPS = 1e-5
MASK_FILL = -1000000000.0
NB = 8
CH = 256
LAG_S, LAG_PV, GRP, ORDER, UNROLL = 4, 8, 0, (1, 0, 2), 2
RING = 4
HALO = 8


def _dot(a, b):
    return jnp.dot(a, b, preferred_element_type=F32)


def _dot_nt(a, b):
    return jax.lax.dot_general(a, b, (((1,), (1,)), ((), ())), preferred_element_type=F32)


def _layernorm(x):
    m = jnp.mean(x, axis=-1, keepdims=True)
    d = x - m
    v = jnp.mean(d * d, axis=-1, keepdims=True)
    return d * jax.lax.rsqrt(v + LN_EPS)


def _gelu(x):
    k0 = math.sqrt(2.0 / math.pi)
    t = jnp.tanh(x * (k0 + (k0 * 0.044715) * (x * x)))
    hx = 0.5 * x
    return hx + hx * t


def _rows(v, n):
    return jnp.concatenate([v] * (n // 8), axis=0) if n > 8 else v


def _halfs(w):
    return pltpu.bitcast(w, BF16)


def _lhs_terms(a11, a12, a21, a22):
    return [a11 + a22, a21 + a22, a11, a22, a11 + a12, a21 - a11, a12 - a22]


def _rhs_sums(b11, b12, b21, b22):
    return {0: b11 + b22, 2: b12 - b22, 3: b21 - b11, 5: b11 + b12, 6: b21 + b22}


_RHS_SLOT = {0: 0, 3: 1, 5: 2, 6: 3}


def _strassen(prod, m2=None, m4=None):
    m2 = prod(2) if m2 is None else m2
    m4 = prod(4) if m4 is None else m4
    c12 = m2 + m4
    m0 = prod(0)
    t11 = m0 - m4
    t22 = m0 + m2
    m3 = prod(3)
    t11 = t11 + m3
    c11 = t11 + prod(6)
    m1 = prod(1)
    c21 = m1 + m3
    t22 = t22 - m1
    c22 = t22 + prod(5)
    return c11, c12, c21, c22


def _kernel(x_hbm, mem0_hbm, wq_hbm, wk_hbm, wv_hbm, wo_hbm, w1_hbm, w2_hbm, w3_hbm, w4_hbm,
            c_hbm, wmod_hbm, out_hbm,
            wo_s, w1_s, w2_s, w3_s, w4_s, wmod_s, x_s, ob_s, xa_s, mod_s, c_ref, mem0_ref,
            sem_qkv, sem_misc, sem_mod,
            *, nseg, seg, nmem, dm, nh, dh):
    hp_n = nh // 2
    kt_n = dm // 128
    ff = w3_s.shape[1]
    scale = dh ** -0.5
    w_u32 = [w.bitcast(U32) for w in (wq_hbm, wk_hbm, wv_hbm)]
    wo_u32 = wo_hbm.bitcast(U32)

    def wo_copy(i):
        n, per = i & (kt_n - 1), wo_s.shape[1] * kt_n // hp_n
        rows = pl.ds(pl.multiple_of((i >> (kt_n.bit_length() - 1)) * per, per), per)
        return pltpu.make_async_copy(wo_u32.at[rows, pl.ds(pl.multiple_of(n * 128, 128), 128)],
                                     wo_s.at[n, rows], sem_misc.at[0])

    wmod_u32 = wmod_hbm.bitcast(U32)

    def mod_copy(t, group):
        return pltpu.make_async_copy(wmod_u32.at[:, pl.ds(pl.multiple_of(t * 128, 128), 128)],
                                     wmod_s.at[t], sem_mod.at[group])

    cp_c = pltpu.make_async_copy(c_hbm, c_ref, sem_misc.at[2])
    cp_mem0 = pltpu.make_async_copy(mem0_hbm, mem0_ref, sem_misc.at[3])
    cp_w1 = pltpu.make_async_copy(w1_hbm, w1_s, sem_misc.at[4])
    cp_w2 = pltpu.make_async_copy(w2_hbm, w2_s, sem_misc.at[5])
    cp_w3 = pltpu.make_async_copy(w3_hbm, w3_s, sem_misc.at[6])
    cp_w4 = pltpu.make_async_copy(w4_hbm, w4_s, sem_misc.at[7])

    def silu_c():
        cv = c_ref[...].astype(F32)
        return jnp.broadcast_to(cv * jax.nn.sigmoid(cv), (16, dm)).astype(BF16)

    def attention(wqkv, qkvb, xb_s, hb_s, fill_s, hx_s, o_s, raw_s, ln_s):
        xs_n = nseg // hp_n

        def pair_copies(hp):
            cps = [pltpu.make_async_copy(w_u32[w].at[:, hp, :], raw_s.at[w, hp & (RING - 1)], sem_qkv.at[hp & (RING - 1)])
                   for w in range(3)]
            rows = pl.ds(hp * xs_n, xs_n)
            return cps + [pltpu.make_async_copy(x_hbm.at[rows], x_s.at[rows], sem_qkv.at[hp & (RING - 1)])]

        cp_xb = pltpu.make_async_copy(x_hbm.at[:, 0:NB, :], xb_s, sem_misc.at[1])
        cp_xb.start()
        cp_c.start()
        cp_mem0.start()
        jt_n = kt_n // 2

        def mod_group(j):
            return [mod_copy(j + t * jt_n, j) for t in range(4)]

        for cp in mod_group(0):
            cp.start()

        def head_pos(i):
            head = jnp.where(i < 2 * seg, i // seg, (i - 2 * seg) // NB)
            r = i % seg
            pos = jnp.where(i < 2 * seg, jnp.where(r < nmem, r, r + NB), nmem + i % NB)
            return head, pos

        nq = 2 * (seg + NB)
        qh, qp = head_pos(jax.lax.broadcasted_iota(jnp.int32, (nq, nq), 0))
        kh, kp = head_pos(jax.lax.broadcasted_iota(jnp.int32, (nq, nq), 1))
        visible = (qp < nmem) | (qp >= kp)
        fill_s[...] = jnp.where(qh == kh, jnp.where(visible, 0.0, MASK_FILL / scale), -jnp.inf).astype(F32)

        mh, kh = nseg * NB // 2, dm // 2
        cp_c.wait()
        cp_mem0.wait()
        sc = silu_c()
        for cp in mod_group(1):
            cp.start()
        cp_xb.wait()
        for cp in mod_group(2):
            cp.start()

        def ln_body(i, carry):
            s0 = i * (nseg // 4)
            ln = _layernorm(xb_s[pl.ds(s0, nseg // 4)].astype(F32).reshape(mh // 2, dm))
            for k in range(kt_n):
                ln_s[k, pl.ds(pl.multiple_of(i * (mh // 2), mh // 2), mh // 2), :] = ln[:, 128 * k:128 * (k + 1)]
            return carry

        jax.lax.fori_loop(0, 4, ln_body, 0)

        def shift_scale_body(j, carry):
            for cp in mod_group(j):
                cp.wait()

            @pl.when(j == 0)
            def _():
                for cp in mod_group(3):
                    cp.start()

            @pl.when(j == 1)
            def _():
                for cp in pair_copies(0):
                    cp.start()

            shift, gain = [], []
            for k in (j, j + jt_n):
                cols = pl.ds(pl.multiple_of(k * 128, 128), 128)
                shift.append(_dot(sc, _halfs(wmod_s[k]))[0:8])
                gain.append(1.0 + _dot(sc, _halfs(wmod_s[kt_n + k]))[0:8])
                mod_s[0, :, cols] = shift[-1]
                mod_s[1, :, cols] = gain[-1]
            for r in range(0, mh, 32):
                quad = [ln_s[j + t * jt_n, r0 + r:r0 + r + 32, :] * _rows(gain[t], 32) + _rows(shift[t], 32)
                        for r0 in (0, mh) for t in range(2)]
                for i, t in enumerate(_lhs_terms(*quad)):
                    hb_s[i, r:r + 32, pl.ds(pl.multiple_of(j * 128, 128), 128)] = t.astype(BF16)
            return carry

        jax.lax.fori_loop(0, jt_n, shift_scale_body, 0)

        def head_w(w, hp, j, rows=slice(None)):
            return _halfs(wqkv[w, 2 * hp + j, rows, :])

        def bulk_body(hp, carry):
            for cp in pair_copies(hp):
                cp.wait()

            @pl.when(hp == 0)
            def _():
                for cp in pair_copies(1) + [wo_copy(0)]:
                    cp.start()

            @pl.when(hp + 2 < hp_n)
            def _():
                for cp in pair_copies(hp + 2):
                    cp.start()

            pl.when(hp + 1 < hp_n)(lambda: wo_copy(hp + 1).start())
            slot = hp & (RING - 1)
            for w in range(3):
                def quad(i):
                    word = raw_s[w, slot, (i // 2) * kh:(i // 2 + 1) * kh, :]
                    return pltpu.bitcast(word & HIGH_HALF if i % 2 else word << 16, F32)

                def prod(i):
                    q = [quad(j) for j in range(4)]
                    return _dot(hb_s[i], {1: q[0], 4: q[3], **_rhs_sums(*q)}[i].astype(BF16))

                m4 = prod(4)
                res = [t.reshape(nseg // 2, NB, dh) for t in _strassen(prod, None, m4)]
                for r in range(0, dm, 16):
                    a = raw_s[w, slot, pl.ds(r, 8, stride=2), :]
                    b = raw_s[w, slot, pl.ds(r + 1, 8, stride=2), :]
                    wqkv[w, 2 * hp, r // 2:r // 2 + 8, :] = (a & 0xFFFF) | (b << 16)
                    wqkv[w, 2 * hp + 1, r // 2:r // 2 + 8, :] = (a >> 16) | (b & HIGH_HALF)
                for i in range(xs_n * w // 3, xs_n * (w + 1) // 3):
                    xs = x_s[hp * xs_n + i, NB:, :].astype(F32)
                    hx_s[hp * xs_n + i] = _layernorm(xs) * _rows(mod_s[1], seg - NB) + _rows(mod_s[0], seg - NB)
                qkvb[w, hp, :nseg // 2] = jnp.concatenate(res[:2], axis=1).astype(BF16)
                qkvb[w, hp, nseg // 2:] = jnp.concatenate(res[2:], axis=1).astype(BF16)
            return carry

        jax.lax.fori_loop(0, hp_n, bulk_body, 0)

        pltpu.make_async_copy(wo_s, wo_s, sem_misc.at[0]).wait()

        mod_per_it = 4 * kt_n * UNROLL // nseg
        exp_c = scale * math.log2(math.e)

        def step(s, mem):
            a = jnp.concatenate([mem, hx_s[s]], axis=0)
            a = [a[:, :kh].astype(BF16), a[:, kh:].astype(BF16)]

            first = [_dot(a[t], jnp.concatenate(
                [head_w(w, 0, j, slice(t * kh // 2, (t + 1) * kh // 2)) for w in ORDER for j in range(2)], axis=1))
                for t in range(2)]

            def proj(w, hp):
                if hp == 0:
                    c0 = [(2 * ORDER.index(w) + j) * dh for j in range(2)]
                    r = [first[0][:, c:c + dh] + first[1][:, c:c + dh] for c in c0]
                else:
                    r = [_dot(a[0], head_w(w, hp, j, slice(0, kh // 2)))
                         + _dot(a[1], head_w(w, hp, j, slice(kh // 2, kh))) for j in range(2)]
                return jnp.concatenate(r + [qkvb[w, hp, s].astype(F32)], axis=0).astype(BF16)

            def probs(q, k):
                fill = fill_s[...]
                sco = jnp.where(fill == 0.0, _dot_nt(q, k), fill)
                e = jnp.exp2((sco - jnp.max(sco, axis=-1, keepdims=True)) * exp_c)
                den = jnp.sum(e, axis=-1, keepdims=True)
                inv = pl.reciprocal(den, approx=True)
                return e.astype(BF16), inv * (2.0 - den * inv)

            def attend(hp, p, v):
                o = _dot(p[0], v) * p[1]
                cols = slice(2 * hp * dh, 2 * (hp + 1) * dh)
                o_s[:, cols] = jnp.concatenate([o[0:seg], o[seg:2 * seg]], axis=1).astype(BF16)
                ob_s[s, :, cols] = jnp.concatenate(
                    [o[2 * seg:2 * seg + NB], o[2 * seg + NB:]], axis=1).astype(BF16)

            val, ps = {}, {}
            clock = [0]

            def tick():
                t = clock[0]
                clock[0] += 1
                for i in range(hp_n):
                    if t == 3 * (i | GRP) + LAG_S:
                        ps[i] = probs(val.pop((0, i)), val.pop((1, i)))
                for i in range(hp_n):
                    if t == 3 * (i | GRP) + LAG_PV:
                        attend(i, ps.pop(i), val.pop((2, i)))

            for hp in range(hp_n):
                for w in ORDER:
                    val[w, hp] = proj(w, hp)
                    tick()
            half = nh * dh // 2
            acc = None
            for part in range(2):
                assert part == 0 or not val
                lo = o_s[:, part * half:(part + 1) * half]
                r = []
                for n in range(kt_n):
                    r.append(_dot(lo, _halfs(wo_s[n, part * half // 2:(part + 1) * half // 2, :])))
                    tick()
                r = jnp.concatenate(r, axis=1)
                acc = r if acc is None else acc + r
            xa_s[s, NB:, :] = acc[nmem:]
            return acc[0:nmem]

        def step_body(i, mem):
            for t in range(mod_per_it):
                mod_copy(2 * kt_n + i * mod_per_it + t, jt_n).start()
            for n, cp in enumerate((cp_w1, cp_w2, cp_w3, cp_w4)):
                pl.when(i == n)(cp.start)
            for u in range(UNROLL):
                mem = step(i * UNROLL + u, mem)
            return mem

        jax.lax.fori_loop(0, nseg // UNROLL, step_body, mem0_ref[...].astype(F32))

    pl.run_scoped(
        attention,
        pltpu.VMEM((3, nh, dm // 2, dh), U32),
        pltpu.VMEM((3, hp_n, nseg, 2 * NB, dh), BF16),
        pltpu.VMEM((nseg, NB, dm), BF16),
        pltpu.VMEM((7, nseg * NB // 2, dm // 2), BF16),
        pltpu.VMEM((2 * (seg + NB), 2 * (seg + NB)), F32),
        pltpu.VMEM((nseg, seg - NB, dm), F32),
        pltpu.VMEM((seg, nh * dh), BF16),
        pltpu.VMEM((3, RING, dm, dh), U32),
        pltpu.VMEM((kt_n, nseg * NB, 128), F32),
    )

    spc = CH // seg
    nch = nseg // spc
    hc = CH // 2
    sh = spc // 2
    dm2, ff2 = dm // 2, ff // 2
    ft_n, nt_n = ff2 // 128, dm2 // 128

    def mlp(w3x_s, w4x_s, h_s, g_s, out_s, w1x_s, w2x_s):
        zero_halo = jnp.zeros((kt_n, HALO, 128), F32)
        g_s[:, 0:HALO, :] = zero_halo
        g_s[:, HALO + nseg * seg:, :] = zero_halo
        sc = silu_c()
        rest = wmod_s.at[2 * kt_n:]
        pltpu.make_async_copy(rest, rest, sem_mod.at[kt_n // 2]).wait()

        def weight_sum_jobs(w_s, wx_s, ci, parts=nch):
            k2, n2 = w_s.shape[0] // 2, w_s.shape[1] // 2
            nr = k2 // parts

            def job(r, c0):
                r0 = pl.multiple_of(ci * nr + r, 16)
                quad = [w_s[pl.ds(r0 + kk, 16), nn + c0:nn + c0 + 256].astype(F32)
                        for kk in (0, k2) for nn in (0, n2)]
                for i, t in _rhs_sums(*quad).items():
                    if i == 2:
                        w_s[pl.ds(r0, 16), n2 + c0:n2 + c0 + 256] = t.astype(BF16)
                    else:
                        wx_s[_RHS_SLOT[i], pl.ds(r0, 16), c0:c0 + 256] = t.astype(BF16)

            return [functools.partial(job, r, c0) for c0 in range(0, n2, 256) for r in range(0, nr, 16)]

        def rhs(w_s, wx_s, i, j):
            k2, n2 = w_s.shape[0] // 2, w_s.shape[1] // 2
            if i == 1:
                return w_s[0:k2, 128 * j:128 * (j + 1)]
            if i == 2:
                return w_s[0:k2, n2 + 128 * j:n2 + 128 * (j + 1)]
            if i == 4:
                return w_s[k2:, n2 + 128 * j:n2 + 128 * (j + 1)]
            return wx_s[_RHS_SLOT[i], :, 128 * j:128 * (j + 1)]

        def spread(jobs, n, slots=kt_n):
            for job in jobs[len(jobs) * n // slots:len(jobs) * (n + 1) // slots]:
                job()

        def halves(v):
            m2, k2 = v.shape[0] // 2, v.shape[1] // 2
            return v[:m2, :k2], v[:m2, k2:], v[m2:, :k2], v[m2:, k2:]

        cp_w1.wait()
        cp_w2.wait()
        cp_w3.wait()
        cp_w4.wait()

        def mod_body(i, carry):
            jobs = weight_sum_jobs(w1_s, w1x_s, i - 2, 4)
            for k in range(kt_n):
                r = _dot(sc, _halfs(wmod_s[i * kt_n + k]))[0:8]
                spread(jobs, k)
                mod_s[i, :, 128 * k:128 * (k + 1)] = jnp.where(i == 4, 1.0 + r, r)
            return carry

        jax.lax.fori_loop(2, 6, mod_body, 0)

        def out_proj(i):
            lo = ob_s[pl.ds(i * sh, sh)].reshape(sh * NB, nh * dh)
            return jnp.concatenate([_dot(lo, _halfs(wo_s[n])) for n in range(kt_n)], axis=1)

        def stage_a(ci, att0):
            def norm(half, att_b):
                si = pl.ds(ci * spc + half * sh, sh)
                att = jnp.concatenate([att_b.reshape(sh, NB, dm), xa_s[si, NB:, :]], axis=1).reshape(hc, dm)
                xa = x_s[si].astype(F32).reshape(hc, dm) + _rows(mod_s[2], hc) * att
                xa_s[si] = xa.reshape(sh, seg, dm)
                h = _layernorm(xa) * _rows(mod_s[4], hc) + _rows(mod_s[3], hc)
                h_s[pl.ds(pl.multiple_of(ci * CH + half * hc, hc), hc), :] = h
                return _layernorm(h)

            att1 = out_proj(2 * ci + 1)
            top = norm(0, att0)
            att_next = out_proj(jnp.minimum(2 * ci + 2, 2 * nch - 1))
            bot = norm(1, att1)
            terms = [t.astype(BF16) for t in _lhs_terms(top[:, :dm2], top[:, dm2:], bot[:, :dm2], bot[:, dm2:])]
            jobs = [weight_sum_jobs(*w, ci) for w in ((w2_s, w2x_s), (w3_s, w3x_s), (w4_s, w4x_s))]
            for n in range(nt_n):
                res = _strassen(lambda i: _dot(terms[i], rhs(w1_s, w1x_s, i, n)))
                for q, t in enumerate(res):
                    r0 = pl.multiple_of(ci * CH + (q // 2) * hc, hc)
                    g_s[n + (q % 2) * nt_n, pl.ds(r0 + HALO, hc), :] = _gelu(t)
                for j in jobs:
                    spread(j, n, nt_n)
            return att_next

        jax.lax.fori_loop(0, nch, stage_a, out_proj(0))

        def out_copy(ci):
            r0 = pl.multiple_of(ci * CH, CH)
            return pltpu.make_async_copy(out_s.at[pl.ds(r0, CH)], out_hbm.at[pl.ds(r0, CH)], sem_misc.at[8])

        def stage_b(ci, carry):
            shifts = (-1, 1, -2, 2)
            x1, u = [], []
            for half in range(2):
                r0 = pl.multiple_of(ci * CH + half * hc, hc)
                gs = jnp.concatenate(
                    [g_s[k, pl.ds(r0 + HALO + shifts[k * 4 // kt_n], hc), :] for k in range(kt_n)], axis=1)
                terms = [t.astype(BF16) for t in _lhs_terms(*halves(gs))]
                res = [_strassen(lambda i: _dot(terms[i], rhs(w2_s, w2x_s, i, n))) for n in range(nt_n)]
                hs = jnp.concatenate(
                    [jnp.concatenate([r[q] for r in res] + [r[q + 1] for r in res], axis=1) for q in (0, 2)],
                    axis=0)
                x1.append(h_s[pl.ds(r0, hc), :] + hs)
                u.append(_layernorm(x1[-1]))
            a3 = [t.astype(BF16) for t in _lhs_terms(u[0][:, :dm2], u[0][:, dm2:], u[1][:, :dm2], u[1][:, dm2:])]

            def prod3(j, i):
                return _dot(a3[i], rhs(w3_s, w3x_s, i, j))

            early = {j: (prod3(j, 2), prod3(j, 4)) for j in range(4)}
            a4 = []
            for j in range(ft_n):
                act = [_gelu(t) for t in _strassen(functools.partial(prod3, j), *early.get(j, ()))]
                a4.append(_lhs_terms(*act))
            a4 = [jnp.concatenate([t[i] for t in a4], axis=1).astype(BF16) for i in range(7)]

            def prod4(n, i):
                return _dot(a4[i], rhs(w4_s, w4x_s, i, n))

            for n in range(nt_n):
                for q, t in enumerate(_strassen(functools.partial(prod4, n))):
                    half, c0 = q // 2, (q % 2) * dm2 + 128 * n
                    r0 = pl.multiple_of(ci * CH + half * hc, hc)
                    xa = xa_s[pl.ds(ci * spc + half * sh, sh), :, c0:c0 + 128].reshape(hc, 128)
                    y = x1[half][:, c0:c0 + 128] + t
                    out_s[pl.ds(r0, hc), c0:c0 + 128] = (xa + _rows(mod_s[5, :, c0:c0 + 128], hc) * y).astype(BF16)
            out_copy(ci).start()
            return carry

        jax.lax.fori_loop(0, nch, stage_b, 0)
        for ci in range(nch):
            out_copy(ci).wait()

    pl.run_scoped(
        mlp,
        pltpu.VMEM((4, dm2, ff2), BF16),
        pltpu.VMEM((4, ff2, dm2), BF16),
        pltpu.VMEM((nseg * seg, dm), F32),
        pltpu.VMEM((kt_n, nseg * seg + 2 * HALO, 128), F32),
        pltpu.VMEM((nseg * seg, dm), BF16),
        pltpu.VMEM((4, dm2, dm2), BF16),
        pltpu.VMEM((4, dm2, dm2), BF16),
    )


@functools.partial(jax.jit, static_argnames=("A_seg_len",))
def pallas_adaLN_cond__memory_aug_recurrent_mem_tr__mixer_s_mlp__prompt_kernel(
    A_x: jax.Array,
    A_mem0: jax.Array,
    A_Wq: jax.Array,
    A_Wk: jax.Array,
    A_Wv: jax.Array,
    A_Wo: jax.Array,
    A_seg_len: int,
    B_x: jax.Array,
    B_w1: jax.Array,
    B_w2: jax.Array,
    B_w3: jax.Array,
    B_w4: jax.Array,
    c: jax.Array,
    w_mod: jax.Array,
):
    del B_x
    b, s, dm = A_x.shape
    _, nh, dh = A_Wq.shape
    nmem = A_mem0.shape[1]
    seg = int(A_seg_len)
    nseg = s // seg
    ff = B_w3.shape[1]
    assert (b, seg, nmem, dh) == (1, 32, NB, 128) and s % CH == 0 and dm % 512 == 0 and nh % 2 == 0
    hp_n = nh // 2
    kt_n = dm // 128
    hbm = pl.BlockSpec(memory_space=pl.ANY)
    out = pl.pallas_call(
        functools.partial(_kernel, nseg=nseg, seg=seg, nmem=nmem, dm=dm, nh=nh, dh=dh),
        out_shape=jax.ShapeDtypeStruct((s, dm), BF16),
        in_specs=[hbm] * 12,
        out_specs=hbm,
        scratch_shapes=[
            pltpu.VMEM((kt_n, nh * dh // 2, 128), U32),
            pltpu.VMEM((dm, dm), BF16),
            pltpu.VMEM((dm, dm), BF16),
            pltpu.VMEM((dm, ff), BF16),
            pltpu.VMEM((ff, dm), BF16),
            pltpu.VMEM((6 * kt_n, dm // 2, 128), U32),
            pltpu.VMEM((nseg, seg, dm), BF16),
            pltpu.VMEM((nseg, NB, nh * dh), BF16),
            pltpu.VMEM((nseg, seg, dm), F32),
            pltpu.VMEM((6, 8, dm), F32),
            pltpu.VMEM((1, dm), BF16),
            pltpu.VMEM((nmem, dm), BF16),
            pltpu.SemaphoreType.DMA((RING,)),
            pltpu.SemaphoreType.DMA((9,)),
            pltpu.SemaphoreType.DMA((kt_n // 2 + 1,)),
        ],
        compiler_params=pltpu.CompilerParams(vmem_limit_bytes=120 * 1024 * 1024),
    )(A_x.reshape(nseg, seg, dm), A_mem0.reshape(nmem, dm), A_Wq, A_Wk, A_Wv,
      A_Wo.reshape(nh * dh, dm), B_w1, B_w2, B_w3, B_w4, c, w_mod)
    return out.reshape(b, s, dm)
```

```python
import functools
import math

import jax
import jax.numpy as jnp
import numpy as np
import jax.experimental.pallas as pl
import jax.experimental.pallas.tpu as pltpu

F32 = jnp.float32
BF16 = jnp.bfloat16
U32 = jnp.uint32

HIGH_HALF = np.uint32(0xFFFF0000)
LN_EPS = 1e-5
MASK_FILL = -1000000000.0
NB = 8
CH = 256
LAG_S, LAG_PV, GRP, ORDER, UNROLL = 4, 8, 0, (1, 0, 2), 2
RING = 4
HALO = 8


def _dot(a, b):
    return jnp.dot(a, b, preferred_element_type=F32)


def _dot_nt(a, b):
    return jax.lax.dot_general(a, b, (((1,), (1,)), ((), ())), preferred_element_type=F32)


def _layernorm(x):
    m = jnp.mean(x, axis=-1, keepdims=True)
    d = x - m
    v = jnp.mean(d * d, axis=-1, keepdims=True)
    return d * jax.lax.rsqrt(v + LN_EPS)


def _gelu(x):
    k0 = math.sqrt(2.0 / math.pi)
    t = jnp.tanh(x * (k0 + (k0 * 0.044715) * (x * x)))
    hx = 0.5 * x
    return hx + hx * t


def _rows(v, n):
    return jnp.concatenate([v] * (n // 8), axis=0) if n > 8 else v


def _halfs(w):
    return pltpu.bitcast(w, BF16)


def _words(rows, cols):
    return pltpu.VMEM((rows // 2, cols), U32)


def _lhs_terms(a11, a12, a21, a22):
    return [a11 + a22, a21 + a22, a11, a22, a11 + a12, a21 - a11, a12 - a22]


def _rhs_sums(b11, b12, b21, b22):
    return {0: b11 + b22, 2: b12 - b22, 3: b21 - b11, 5: b11 + b12, 6: b21 + b22}


_RHS_SLOT = {0: 0, 3: 1, 5: 2, 6: 3}


def _strassen(prod, m2=None, m4=None):
    m2 = prod(2) if m2 is None else m2
    m4 = prod(4) if m4 is None else m4
    c12 = m2 + m4
    m0 = prod(0)
    t11 = m0 - m4
    t22 = m0 + m2
    m3 = prod(3)
    t11 = t11 + m3
    c11 = t11 + prod(6)
    m1 = prod(1)
    c21 = m1 + m3
    t22 = t22 - m1
    c22 = t22 + prod(5)
    return c11, c12, c21, c22


def _kernel(x_hbm, mem0_hbm, wq_hbm, wk_hbm, wv_hbm, wo_hbm, w1_hbm, w2_hbm, w3_hbm, w4_hbm,
            c_hbm, wmod_hbm, out_hbm,
            wo_s, w1_w, w2_w, w3_w, w4_w, wmod_s, x_s, ob_s, xa_s, mod_s, c_ref, mem0_ref,
            sem_qkv, sem_misc, sem_mod,
            *, nseg, seg, nmem, dm, nh, dh):
    hp_n = nh // 2
    kt_n = dm // 128
    w1_s, w2_s, w3_s, w4_s = [w.bitcast(BF16) for w in (w1_w, w2_w, w3_w, w4_w)]
    ff = w3_s.shape[1]
    scale = dh ** -0.5
    w_u32 = [w.bitcast(U32) for w in (wq_hbm, wk_hbm, wv_hbm)]
    wo_u32 = wo_hbm.bitcast(U32)

    def wo_copy(i):
        n, per = i & (kt_n - 1), wo_s.shape[1] * kt_n // hp_n
        rows = pl.ds(pl.multiple_of((i >> (kt_n.bit_length() - 1)) * per, per), per)
        return pltpu.make_async_copy(wo_u32.at[rows, pl.ds(pl.multiple_of(n * 128, 128), 128)],
                                     wo_s.at[n, rows], sem_misc.at[0])

    wmod_u32 = wmod_hbm.bitcast(U32)

    def mod_copy(t, group):
        return pltpu.make_async_copy(wmod_u32.at[:, pl.ds(pl.multiple_of(t * 128, 128), 128)],
                                     wmod_s.at[t], sem_mod.at[group])

    cp_c = pltpu.make_async_copy(c_hbm, c_ref, sem_misc.at[2])
    cp_mem0 = pltpu.make_async_copy(mem0_hbm, mem0_ref, sem_misc.at[3])
    cp_w1 = pltpu.make_async_copy(w1_hbm.bitcast(U32), w1_w, sem_misc.at[4])
    cp_w2 = pltpu.make_async_copy(w2_hbm.bitcast(U32), w2_w, sem_misc.at[5])
    cp_w3 = pltpu.make_async_copy(w3_hbm.bitcast(U32), w3_w, sem_misc.at[6])
    cp_w4 = pltpu.make_async_copy(w4_hbm.bitcast(U32), w4_w, sem_misc.at[7])

    def silu_c():
        cv = c_ref[...].astype(F32)
        return jnp.broadcast_to(cv * jax.nn.sigmoid(cv), (16, dm)).astype(BF16)

    def attention(wqkv, qkvb, xb_s, hb_s, fill_s, hx_s, o_s, raw_s, ln_s):
        hb_s, o_s = hb_s.bitcast(BF16), o_s.bitcast(BF16)
        xs_n = nseg // hp_n

        def pair_copies(hp):
            cps = [pltpu.make_async_copy(w_u32[w].at[:, hp, :], raw_s.at[w, hp & (RING - 1)], sem_qkv.at[hp & (RING - 1)])
                   for w in range(3)]
            rows = pl.ds(hp * xs_n, xs_n)
            return cps + [pltpu.make_async_copy(x_hbm.at[rows], x_s.at[rows], sem_qkv.at[hp & (RING - 1)])]

        cp_xb = pltpu.make_async_copy(x_hbm.at[:, 0:NB, :], xb_s, sem_misc.at[1])
        cp_xb.start()
        cp_c.start()
        cp_mem0.start()
        jt_n = kt_n // 2

        def mod_group(j):
            return [mod_copy(j + t * jt_n, j) for t in range(4)]

        for cp in mod_group(0):
            cp.start()

        def head_pos(i):
            head = jnp.where(i < 2 * seg, i // seg, (i - 2 * seg) // NB)
            r = i % seg
            pos = jnp.where(i < 2 * seg, jnp.where(r < nmem, r, r + NB), nmem + i % NB)
            return head, pos

        nq = 2 * (seg + NB)
        qh, qp = head_pos(jax.lax.broadcasted_iota(jnp.int32, (nq, nq), 0))
        kh, kp = head_pos(jax.lax.broadcasted_iota(jnp.int32, (nq, nq), 1))
        visible = (qp < nmem) | (qp >= kp)
        fill_s[...] = jnp.where(qh == kh, jnp.where(visible, 0.0, MASK_FILL / scale), -jnp.inf).astype(F32)

        mh, kh = nseg * NB // 2, dm // 2
        cp_c.wait()
        cp_mem0.wait()
        sc = silu_c()
        for cp in mod_group(1):
            cp.start()
        cp_xb.wait()
        for cp in mod_group(2):
            cp.start()

        def ln_body(i, carry):
            s0 = i * (nseg // 4)
            ln = _layernorm(xb_s[pl.ds(s0, nseg // 4)].astype(F32).reshape(mh // 2, dm))
            for k in range(kt_n):
                ln_s[k, pl.ds(pl.multiple_of(i * (mh // 2), mh // 2), mh // 2), :] = ln[:, 128 * k:128 * (k + 1)]
            return carry

        jax.lax.fori_loop(0, 4, ln_body, 0)

        def shift_scale_body(j, carry):
            for cp in mod_group(j):
                cp.wait()

            @pl.when(j == 0)
            def _():
                for cp in mod_group(3):
                    cp.start()

            @pl.when(j == 1)
            def _():
                for cp in pair_copies(0):
                    cp.start()

            shift, gain = [], []
            for k in (j, j + jt_n):
                cols = pl.ds(pl.multiple_of(k * 128, 128), 128)
                shift.append(_dot(sc, _halfs(wmod_s[k]))[0:8])
                gain.append(1.0 + _dot(sc, _halfs(wmod_s[kt_n + k]))[0:8])
                mod_s[0, :, cols] = shift[-1]
                mod_s[1, :, cols] = gain[-1]
            for r in range(0, mh, 32):
                quad = [ln_s[j + t * jt_n, r0 + r:r0 + r + 32, :] * _rows(gain[t], 32) + _rows(shift[t], 32)
                        for r0 in (0, mh) for t in range(2)]
                for i, t in enumerate(_lhs_terms(*quad)):
                    hb_s[i * mh + r:i * mh + r + 32, pl.ds(pl.multiple_of(j * 128, 128), 128)] = t.astype(BF16)
            return carry

        jax.lax.fori_loop(0, jt_n, shift_scale_body, 0)

        def head_w(w, hp, j, rows=slice(None)):
            return _halfs(wqkv[w, 2 * hp + j, rows, :])

        def bulk_body(hp, carry):
            for cp in pair_copies(hp):
                cp.wait()

            @pl.when(hp == 0)
            def _():
                for cp in pair_copies(1) + [wo_copy(0)]:
                    cp.start()

            @pl.when(hp + 2 < hp_n)
            def _():
                for cp in pair_copies(hp + 2):
                    cp.start()

            pl.when(hp + 1 < hp_n)(lambda: wo_copy(hp + 1).start())
            slot = hp & (RING - 1)
            for w in range(3):
                def quad(i):
                    word = raw_s[w, slot, (i // 2) * kh:(i // 2 + 1) * kh, :]
                    return pltpu.bitcast(word & HIGH_HALF if i % 2 else word << 16, F32)

                def prod(i):
                    q = [quad(j) for j in range(4)]
                    return _dot(hb_s[i * mh:(i + 1) * mh], {1: q[0], 4: q[3], **_rhs_sums(*q)}[i].astype(BF16))

                m4 = prod(4)
                res = [t.reshape(nseg // 2, NB, dh) for t in _strassen(prod, None, m4)]
                for r in range(0, dm, 16):
                    a = raw_s[w, slot, pl.ds(r, 8, stride=2), :]
                    b = raw_s[w, slot, pl.ds(r + 1, 8, stride=2), :]
                    wqkv[w, 2 * hp, r // 2:r // 2 + 8, :] = (a & 0xFFFF) | (b << 16)
                    wqkv[w, 2 * hp + 1, r // 2:r // 2 + 8, :] = (a >> 16) | (b & HIGH_HALF)
                for i in range(xs_n * w // 3, xs_n * (w + 1) // 3):
                    xs = x_s[hp * xs_n + i, NB:, :].astype(F32)
                    hx_s[hp * xs_n + i] = _layernorm(xs) * _rows(mod_s[1], seg - NB) + _rows(mod_s[0], seg - NB)
                qkvb[w, hp, :nseg // 2] = jnp.concatenate(res[:2], axis=1).astype(BF16)
                qkvb[w, hp, nseg // 2:] = jnp.concatenate(res[2:], axis=1).astype(BF16)
            return carry

        jax.lax.fori_loop(0, hp_n, bulk_body, 0)

        pltpu.make_async_copy(wo_s, wo_s, sem_misc.at[0]).wait()
        for cp in (cp_w1, cp_w2, cp_w3, cp_w4):
            cp.start()

        mod_per_it = 4 * kt_n * UNROLL // nseg
        exp_c = scale * math.log2(math.e)

        def step(s, mem):
            a = jnp.concatenate([mem, hx_s[s]], axis=0)
            a = [a[:, :kh].astype(BF16), a[:, kh:].astype(BF16)]

            first = [_dot(a[t], jnp.concatenate(
                [head_w(w, 0, j, slice(t * kh // 2, (t + 1) * kh // 2)) for w in ORDER for j in range(2)], axis=1))
                for t in range(2)]

            def proj(w, hp):
                if hp == 0:
                    c0 = [(2 * ORDER.index(w) + j) * dh for j in range(2)]
                    r = [first[0][:, c:c + dh] + first[1][:, c:c + dh] for c in c0]
                else:
                    r = [_dot(a[0], head_w(w, hp, j, slice(0, kh // 2)))
                         + _dot(a[1], head_w(w, hp, j, slice(kh // 2, kh))) for j in range(2)]
                return jnp.concatenate(r + [qkvb[w, hp, s].astype(F32)], axis=0).astype(BF16)

            def probs(q, k):
                fill = fill_s[...]
                sco = jnp.where(fill == 0.0, _dot_nt(q, k), fill)
                e = jnp.exp2((sco - jnp.max(sco, axis=-1, keepdims=True)) * exp_c)
                den = jnp.sum(e, axis=-1, keepdims=True)
                inv = pl.reciprocal(den, approx=True)
                return e.astype(BF16), inv * (2.0 - den * inv)

            def attend(hp, p, v):
                o = _dot(p[0], v) * p[1]
                cols = slice(2 * hp * dh, 2 * (hp + 1) * dh)
                o_s[:, cols] = jnp.concatenate([o[0:seg], o[seg:2 * seg]], axis=1).astype(BF16)
                ob_s[s, :, cols] = jnp.concatenate(
                    [o[2 * seg:2 * seg + NB], o[2 * seg + NB:]], axis=1).astype(BF16)

            val, ps = {}, {}
            clock = [0]

            def tick():
                t = clock[0]
                clock[0] += 1
                for i in range(hp_n):
                    if t == 3 * (i | GRP) + LAG_S:
                        ps[i] = probs(val.pop((0, i)), val.pop((1, i)))
                for i in range(hp_n):
                    if t == 3 * (i | GRP) + LAG_PV:
                        attend(i, ps.pop(i), val.pop((2, i)))

            for hp in range(hp_n):
                for w in ORDER:
                    val[w, hp] = proj(w, hp)
                    tick()
            half = nh * dh // 2
            acc = None
            for part in range(2):
                assert part == 0 or not val
                lo = o_s[:, part * half:(part + 1) * half]
                r = []
                for n in range(kt_n):
                    r.append(_dot(lo, _halfs(wo_s[n, part * half // 2:(part + 1) * half // 2, :])))
                    tick()
                r = jnp.concatenate(r, axis=1)
                acc = r if acc is None else acc + r
            xa_s[s, NB:, :] = acc[nmem:]
            return acc[0:nmem]

        def step_body(i, mem):
            for t in range(mod_per_it):
                mod_copy(2 * kt_n + i * mod_per_it + t, jt_n).start()
            for u in range(UNROLL):
                mem = step(i * UNROLL + u, mem)
            return mem

        jax.lax.fori_loop(0, nseg // UNROLL, step_body, mem0_ref[...].astype(F32))

    pl.run_scoped(
        attention,
        pltpu.VMEM((3, nh, dm // 2, dh), U32),
        pltpu.VMEM((3, hp_n, nseg, 2 * NB, dh), BF16),
        pltpu.VMEM((nseg, NB, dm), BF16),
        _words(7 * nseg * NB // 2, dm // 2),
        pltpu.VMEM((2 * (seg + NB), 2 * (seg + NB)), F32),
        pltpu.VMEM((nseg, seg - NB, dm), F32),
        _words(seg, nh * dh),
        pltpu.VMEM((3, RING, dm, dh), U32),
        pltpu.VMEM((kt_n, nseg * NB, 128), F32),
    )

    spc = CH // seg
    nch = nseg // spc
    hc = CH // 2
    sh = spc // 2
    dm2, ff2 = dm // 2, ff // 2
    ft_n, nt_n = ff2 // 128, dm2 // 128

    def mlp(w3x_s, w4x_s, h_s, g_s, out_s, w1x_s, w2x_s):
        w1x_s, w2x_s, w3x_s, w4x_s = [w.bitcast(BF16) for w in (w1x_s, w2x_s, w3x_s, w4x_s)]
        zero_halo = jnp.zeros((kt_n, HALO, 128), F32)
        g_s[:, 0:HALO, :] = zero_halo
        g_s[:, HALO + nseg * seg:, :] = zero_halo
        sc = silu_c()
        rest = wmod_s.at[2 * kt_n:]
        pltpu.make_async_copy(rest, rest, sem_mod.at[kt_n // 2]).wait()

        def weight_sum_jobs(w_s, wx_s, ci, parts=nch):
            k2, n2 = w_s.shape[0] // 2, w_s.shape[1] // 2
            nr = k2 // parts

            def job(r, c0):
                r0 = pl.multiple_of(ci * nr + r, 16)
                quad = [w_s[pl.ds(r0 + kk, 16), nn + c0:nn + c0 + 256].astype(F32)
                        for kk in (0, k2) for nn in (0, n2)]
                for i, t in _rhs_sums(*quad).items():
                    if i == 2:
                        w_s[pl.ds(r0, 16), n2 + c0:n2 + c0 + 256] = t.astype(BF16)
                    else:
                        wx_s[pl.ds(r0 + _RHS_SLOT[i] * k2, 16), c0:c0 + 256] = t.astype(BF16)

            return [functools.partial(job, r, c0) for c0 in range(0, n2, 256) for r in range(0, nr, 16)]

        def rhs(w_s, wx_s, i, j):
            k2, n2 = w_s.shape[0] // 2, w_s.shape[1] // 2
            if i == 1:
                return w_s[0:k2, 128 * j:128 * (j + 1)]
            if i == 2:
                return w_s[0:k2, n2 + 128 * j:n2 + 128 * (j + 1)]
            if i == 4:
                return w_s[k2:, n2 + 128 * j:n2 + 128 * (j + 1)]
            return wx_s[_RHS_SLOT[i] * k2:(_RHS_SLOT[i] + 1) * k2, 128 * j:128 * (j + 1)]

        def spread(jobs, n, slots=kt_n):
            for job in jobs[len(jobs) * n // slots:len(jobs) * (n + 1) // slots]:
                job()

        def halves(v):
            m2, k2 = v.shape[0] // 2, v.shape[1] // 2
            return v[:m2, :k2], v[:m2, k2:], v[m2:, :k2], v[m2:, k2:]

        cp_w1.wait()
        cp_w2.wait()
        cp_w3.wait()
        cp_w4.wait()

        def mod_body(i, carry):
            jobs = weight_sum_jobs(w1_s, w1x_s, i - 2, 4)
            for k in range(kt_n):
                r = _dot(sc, _halfs(wmod_s[i * kt_n + k]))[0:8]
                spread(jobs, k)
                mod_s[i, :, 128 * k:128 * (k + 1)] = jnp.where(i == 4, 1.0 + r, r)
            return carry

        jax.lax.fori_loop(2, 6, mod_body, 0)

        def out_proj(i):
            lo = ob_s[pl.ds(i * sh, sh)].reshape(sh * NB, nh * dh)
            return jnp.concatenate([_dot(lo, _halfs(wo_s[n])) for n in range(kt_n)], axis=1)

        def stage_a(ci, att0):
            def norm(half, att_b):
                si = pl.ds(ci * spc + half * sh, sh)
                att = jnp.concatenate([att_b.reshape(sh, NB, dm), xa_s[si, NB:, :]], axis=1).reshape(hc, dm)
                xa = x_s[si].astype(F32).reshape(hc, dm) + _rows(mod_s[2], hc) * att
                xa_s[si] = xa.reshape(sh, seg, dm)
                h = _layernorm(xa) * _rows(mod_s[4], hc) + _rows(mod_s[3], hc)
                h_s[pl.ds(pl.multiple_of(ci * CH + half * hc, hc), hc), :] = h
                return _layernorm(h)

            att1 = out_proj(2 * ci + 1)
            top = norm(0, att0)
            att_next = out_proj(jnp.minimum(2 * ci + 2, 2 * nch - 1))
            bot = norm(1, att1)
            terms = [t.astype(BF16) for t in _lhs_terms(top[:, :dm2], top[:, dm2:], bot[:, :dm2], bot[:, dm2:])]
            jobs = [weight_sum_jobs(*w, ci) for w in ((w2_s, w2x_s), (w3_s, w3x_s), (w4_s, w4x_s))]
            for n in range(nt_n):
                res = _strassen(lambda i: _dot(terms[i], rhs(w1_s, w1x_s, i, n)))
                for q, t in enumerate(res):
                    r0 = pl.multiple_of(ci * CH + (q // 2) * hc, hc)
                    g_s[n + (q % 2) * nt_n, pl.ds(r0 + HALO, hc), :] = _gelu(t)
                for j in jobs:
                    spread(j, n, nt_n)
            return att_next

        jax.lax.fori_loop(0, nch, stage_a, out_proj(0))

        def out_copy(ci):
            r0 = pl.multiple_of(ci * CH, CH)
            return pltpu.make_async_copy(out_s.at[pl.ds(r0, CH)], out_hbm.at[pl.ds(r0, CH)], sem_misc.at[8])

        def stage_b(ci, carry):
            shifts = (-1, 1, -2, 2)
            x1, u = [], []
            for half in range(2):
                r0 = pl.multiple_of(ci * CH + half * hc, hc)
                gs = jnp.concatenate(
                    [g_s[k, pl.ds(r0 + HALO + shifts[k * 4 // kt_n], hc), :] for k in range(kt_n)], axis=1)
                terms = [t.astype(BF16) for t in _lhs_terms(*halves(gs))]
                res = [_strassen(lambda i: _dot(terms[i], rhs(w2_s, w2x_s, i, n))) for n in range(nt_n)]
                hs = jnp.concatenate(
                    [jnp.concatenate([r[q] for r in res] + [r[q + 1] for r in res], axis=1) for q in (0, 2)],
                    axis=0)
                x1.append(h_s[pl.ds(r0, hc), :] + hs)
                u.append(_layernorm(x1[-1]))
            a3 = [t.astype(BF16) for t in _lhs_terms(u[0][:, :dm2], u[0][:, dm2:], u[1][:, :dm2], u[1][:, dm2:])]

            def prod3(j, i):
                return _dot(a3[i], rhs(w3_s, w3x_s, i, j))

            early = {j: (prod3(j, 2), prod3(j, 4)) for j in range(4)}
            a4 = []
            for j in range(ft_n):
                act = [_gelu(t) for t in _strassen(functools.partial(prod3, j), *early.get(j, ()))]
                a4.append(_lhs_terms(*act))
            a4 = [jnp.concatenate([t[i] for t in a4], axis=1).astype(BF16) for i in range(7)]

            def prod4(n, i):
                return _dot(a4[i], rhs(w4_s, w4x_s, i, n))

            for n in range(nt_n):
                for q, t in enumerate(_strassen(functools.partial(prod4, n))):
                    half, c0 = q // 2, (q % 2) * dm2 + 128 * n
                    r0 = pl.multiple_of(ci * CH + half * hc, hc)
                    xa = xa_s[pl.ds(ci * spc + half * sh, sh), :, c0:c0 + 128].reshape(hc, 128)
                    y = x1[half][:, c0:c0 + 128] + t
                    out_s[pl.ds(r0, hc), c0:c0 + 128] = (xa + _rows(mod_s[5, :, c0:c0 + 128], hc) * y).astype(BF16)
            out_copy(ci).start()
            return carry

        jax.lax.fori_loop(0, nch, stage_b, 0)
        for ci in range(nch):
            out_copy(ci).wait()

    pl.run_scoped(
        mlp,
        _words(4 * dm2, ff2),
        _words(4 * ff2, dm2),
        pltpu.VMEM((nseg * seg, dm), F32),
        pltpu.VMEM((kt_n, nseg * seg + 2 * HALO, 128), F32),
        pltpu.VMEM((nseg * seg, dm), BF16),
        _words(4 * dm2, dm2),
        _words(4 * dm2, dm2),
    )


@functools.partial(jax.jit, static_argnames=("A_seg_len",))
def pallas_adaLN_cond__memory_aug_recurrent_mem_tr__mixer_s_mlp__prompt_kernel(
    A_x: jax.Array,
    A_mem0: jax.Array,
    A_Wq: jax.Array,
    A_Wk: jax.Array,
    A_Wv: jax.Array,
    A_Wo: jax.Array,
    A_seg_len: int,
    B_x: jax.Array,
    B_w1: jax.Array,
    B_w2: jax.Array,
    B_w3: jax.Array,
    B_w4: jax.Array,
    c: jax.Array,
    w_mod: jax.Array,
):
    del B_x
    b, s, dm = A_x.shape
    _, nh, dh = A_Wq.shape
    nmem = A_mem0.shape[1]
    seg = int(A_seg_len)
    nseg = s // seg
    ff = B_w3.shape[1]
    assert (b, seg, nmem, dh) == (1, 32, NB, 128) and s % CH == 0 and dm % 512 == 0 and nh % 2 == 0
    hp_n = nh // 2
    kt_n = dm // 128
    hbm = pl.BlockSpec(memory_space=pl.ANY)
    out = pl.pallas_call(
        functools.partial(_kernel, nseg=nseg, seg=seg, nmem=nmem, dm=dm, nh=nh, dh=dh),
        out_shape=jax.ShapeDtypeStruct((s, dm), BF16),
        in_specs=[hbm] * 12,
        out_specs=hbm,
        scratch_shapes=[
            pltpu.VMEM((kt_n, nh * dh // 2, 128), U32),
            _words(dm, dm),
            _words(dm, dm),
            _words(dm, ff),
            _words(ff, dm),
            pltpu.VMEM((6 * kt_n, dm // 2, 128), U32),
            pltpu.VMEM((nseg, seg, dm), BF16),
            pltpu.VMEM((nseg, NB, nh * dh), BF16),
            pltpu.VMEM((nseg, seg, dm), F32),
            pltpu.VMEM((6, 8, dm), F32),
            pltpu.VMEM((1, dm), BF16),
            pltpu.VMEM((nmem, dm), BF16),
            pltpu.SemaphoreType.DMA((RING,)),
            pltpu.SemaphoreType.DMA((9,)),
            pltpu.SemaphoreType.DMA((kt_n // 2 + 1,)),
        ],
        compiler_params=pltpu.CompilerParams(vmem_limit_bytes=120 * 1024 * 1024),
    )(A_x.reshape(nseg, seg, dm), A_mem0.reshape(nmem, dm), A_Wq, A_Wk, A_Wv,
      A_Wo.reshape(nh * dh, dm), B_w1, B_w2, B_w3, B_w4, c, w_mod)
    return out.reshape(b, s, dm)
```

```python
import functools
import math

import jax
import jax.numpy as jnp
import numpy as np
import jax.experimental.pallas as pl
import jax.experimental.pallas.tpu as pltpu

F32 = jnp.float32
BF16 = jnp.bfloat16
U32 = jnp.uint32

HIGH_HALF = np.uint32(0xFFFF0000)
LN_EPS = 1e-5
MASK_FILL = -1000000000.0
NB = 8
CH = 256
RING = 4
HALO = 8
KQV = (1, 0, 2)
LAG_QK, LAG_PV = 3, 7


def _dot(a, b):
    return jnp.dot(a, b, preferred_element_type=F32)


def _dot_nt(a, b):
    return jax.lax.dot_general(a, b, (((1,), (1,)), ((), ())), preferred_element_type=F32)


def _layernorm(x):
    m = jnp.mean(x, axis=-1, keepdims=True)
    d = x - m
    v = jnp.mean(d * d, axis=-1, keepdims=True)
    return d * jax.lax.rsqrt(v + LN_EPS)


def _gelu(x):
    k0 = math.sqrt(2.0 / math.pi)
    t = jnp.tanh(x * (k0 + (k0 * 0.044715) * (x * x)))
    hx = 0.5 * x
    return hx + hx * t


def _rows(v, n):
    return jnp.concatenate([v] * (n // 8), axis=0)


def _tile(j):
    return slice(128 * j, 128 * (j + 1))


def _halfs(w):
    return pltpu.bitcast(w, BF16)


def _words(rows, cols):
    return pltpu.VMEM((rows // 2, cols), U32)


def _quadrants(v):
    m2, k2 = v.shape[0] // 2, v.shape[1] // 2
    return v[:m2, :k2], v[:m2, k2:], v[m2:, :k2], v[m2:, k2:]


def _lhs_terms(a11, a12, a21, a22):
    return [a11 + a22, a21 + a22, a11, a22, a11 + a12, a21 - a11, a12 - a22]


def _rhs_sums(b11, b12, b21, b22):
    return {0: b11 + b22, 2: b12 - b22, 3: b21 - b11, 5: b11 + b12, 6: b21 + b22}


def _strassen(prod, m2=None, m4=None):
    m2 = prod(2) if m2 is None else m2
    m4 = prod(4) if m4 is None else m4
    c12 = m2 + m4
    m0 = prod(0)
    t11 = m0 - m4
    t22 = m0 + m2
    m3 = prod(3)
    t11 = t11 + m3
    c11 = t11 + prod(6)
    m1 = prod(1)
    c21 = m1 + m3
    t22 = t22 - m1
    c22 = t22 + prod(5)
    return c11, c12, c21, c22


_SUM_SLOT = {0: 0, 3: 1, 5: 2, 6: 3}


def _weight_sum_jobs(w_s, sum_s, part, parts):
    k2, n2 = w_s.shape[0] // 2, w_s.shape[1] // 2
    nr = k2 // parts

    def job(r, c0):
        r0 = pl.multiple_of(part * nr + r, 16)
        quad = [w_s[pl.ds(r0 + kk, 16), nn + c0:nn + c0 + 128].astype(F32)
                for kk in (0, k2) for nn in (0, n2)]
        for i, t in _rhs_sums(*quad).items():
            if i == 2:
                w_s[pl.ds(r0, 16), n2 + c0:n2 + c0 + 128] = t.astype(BF16)
            else:
                sum_s[pl.ds(r0 + _SUM_SLOT[i] * k2, 16), c0:c0 + 128] = t.astype(BF16)

    return [functools.partial(job, r, c0) for c0 in range(0, n2, 128) for r in range(0, nr, 16)]


def _rhs(w_s, sum_s, i, j):
    k2, nt = w_s.shape[0] // 2, w_s.shape[1] // 256
    if i == 1:
        return w_s[0:k2, _tile(j)]
    if i == 2:
        return w_s[0:k2, _tile(nt + j)]
    if i == 4:
        return w_s[k2:, _tile(nt + j)]
    return sum_s[_SUM_SLOT[i] * k2:(_SUM_SLOT[i] + 1) * k2, _tile(j)]


def _spread(jobs, n, slots):
    for job in jobs[len(jobs) * n // slots:len(jobs) * (n + 1) // slots]:
        job()


def _kernel(x_hbm, mem0_hbm, wq_hbm, wk_hbm, wv_hbm, wo_hbm, w1_hbm, w2_hbm, w3_hbm, w4_hbm,
            c_hbm, wmod_hbm, out_hbm,
            wo_s, w1_w, w2_w, w3_w, w4_w, wmod_s, x_s, xa_s, h_s, ut_w, w1x_w, mod_s, c_s, mem0_s,
            sem_qkv, sem_misc, sem_mod):
    nseg, seg, dm = x_s.shape
    nmem = mem0_s.shape[0]
    _, nh, dh = wq_hbm.shape
    ntok = nseg * seg
    hp_n = nh // 2
    kt_n = dm // 128
    jt_n = kt_n // 2
    dm2 = dm // 2
    scale = dh ** -0.5
    w1_s, w2_s, w3_s, w4_s, ut_s, w1x_s = [w.bitcast(BF16) for w in (w1_w, w2_w, w3_w, w4_w, ut_w, w1x_w)]
    qkv_u32 = [w.bitcast(U32) for w in (wq_hbm, wk_hbm, wv_hbm)]
    wo_u32 = wo_hbm.bitcast(U32)
    wmod_u32 = wmod_hbm.bitcast(U32)

    def wo_copy(i):
        n, per = i & (kt_n - 1), wo_s.shape[1] * kt_n // hp_n
        rows = pl.ds(pl.multiple_of((i >> (kt_n.bit_length() - 1)) * per, per), per)
        return pltpu.make_async_copy(wo_u32.at[rows, pl.ds(pl.multiple_of(n * 128, 128), 128)],
                                     wo_s.at[n, rows], sem_misc.at[0])

    def mod_copy(t, group):
        return pltpu.make_async_copy(wmod_u32.at[:, pl.ds(pl.multiple_of(t * 128, 128), 128)],
                                     wmod_s.at[t], sem_mod.at[group])

    def wait_filled(buf, sem):
        pltpu.make_async_copy(buf, buf, sem).wait()

    cp_c = pltpu.make_async_copy(c_hbm, c_s, sem_misc.at[2])
    cp_mem0 = pltpu.make_async_copy(mem0_hbm, mem0_s, sem_misc.at[3])
    cp_w1 = pltpu.make_async_copy(w1_hbm.bitcast(U32), w1_w, sem_misc.at[4])
    cp_w2 = pltpu.make_async_copy(w2_hbm.bitcast(U32), w2_w, sem_misc.at[5])
    cp_w3 = pltpu.make_async_copy(w3_hbm.bitcast(U32), w3_w, sem_misc.at[6])
    cp_w4 = pltpu.make_async_copy(w4_hbm.bitcast(U32), w4_w, sem_misc.at[7])

    def silu_c():
        cv = c_s[...].astype(F32)
        return jnp.broadcast_to(cv * jax.nn.sigmoid(cv), (16, dm)).astype(BF16)

    def late_mod(n):
        jobs = _weight_sum_jobs(w1_s, w1x_s, n - 2, 4)
        sc = silu_c()
        for k in range(kt_n):
            r = _dot(sc, _halfs(wmod_s[n * kt_n + k]))[0:8]
            _spread(jobs, k, kt_n)
            mod_s[n, :, _tile(k)] = jnp.where(n == 4, 1.0 + r, r)

    def attention(wqkv, qkvb, xb_s, hb_w, fill_s, hx_s, o_w, raw_s, ln_s, ob_s, att_s):
        hb_s, o_s = hb_w.bitcast(BF16), o_w.bitcast(BF16)
        xs_n = nseg // hp_n
        mh = nseg * NB // 2

        def pair_copies(hp):
            slot = hp & (RING - 1)
            cps = [pltpu.make_async_copy(qkv_u32[w].at[:, hp, :], raw_s.at[w, slot, 0:dm], sem_qkv.at[slot])
                   for w in range(3)]
            rows = pl.ds(hp * xs_n, xs_n)
            return cps + [pltpu.make_async_copy(x_hbm.at[rows], x_s.at[rows], sem_qkv.at[slot])]

        def mod_group(j):
            return [mod_copy(j + t * jt_n, j) for t in range(4)]

        cp_xb = pltpu.make_async_copy(x_hbm.at[:, 0:NB, :], xb_s, sem_misc.at[1])
        for cp in [cp_xb, cp_c, cp_mem0] + mod_group(0):
            cp.start()

        def head_pos(i):
            head = jnp.where(i < 2 * seg, i // seg, (i - 2 * seg) // NB)
            r = i % seg
            pos = jnp.where(i < 2 * seg, jnp.where(r < nmem, r, r + NB), nmem + i % NB)
            return head, pos

        qh, qp = head_pos(jax.lax.broadcasted_iota(jnp.int32, fill_s.shape, 0))
        kh, kp = head_pos(jax.lax.broadcasted_iota(jnp.int32, fill_s.shape, 1))
        visible = (qp < nmem) | (qp >= kp)
        fill_s[...] = jnp.where(qh == kh, jnp.where(visible, 0.0, MASK_FILL / scale), -jnp.inf).astype(F32)

        cp_c.wait()
        cp_mem0.wait()
        sc = silu_c()
        for cp in mod_group(1):
            cp.start()
        cp_xb.wait()
        for cp in mod_group(2):
            cp.start()

        def ln_body(i, carry):
            ln = _layernorm(xb_s[pl.ds(i * (nseg // 4), nseg // 4)].astype(F32).reshape(mh // 2, dm))
            for k in range(kt_n):
                ln_s[k, pl.ds(pl.multiple_of(i * (mh // 2), mh // 2), mh // 2), :] = ln[:, _tile(k)]
            return carry

        jax.lax.fori_loop(0, 4, ln_body, 0)

        def shift_scale_body(j, carry):
            for cp in mod_group(j):
                cp.wait()

            @pl.when(j == 0)
            def _():
                for cp in mod_group(3):
                    cp.start()

            @pl.when(j == 1)
            def _():
                for cp in pair_copies(0):
                    cp.start()

            shift, gain = [], []
            for k in (j, j + jt_n):
                cols = pl.ds(pl.multiple_of(k * 128, 128), 128)
                shift.append(_dot(sc, _halfs(wmod_s[k]))[0:8])
                gain.append(1.0 + _dot(sc, _halfs(wmod_s[kt_n + k]))[0:8])
                mod_s[0, :, cols] = shift[-1]
                mod_s[1, :, cols] = gain[-1]
            for r in range(0, mh, 32):
                quad = [ln_s[j + t * jt_n, r0 + r:r0 + r + 32, :] * _rows(gain[t], 32) + _rows(shift[t], 32)
                        for r0 in (0, mh) for t in range(2)]
                for i, t in enumerate(_lhs_terms(*quad)):
                    hb_s[i * mh + r:i * mh + r + 32, pl.ds(pl.multiple_of(j * 128, 128), 128)] = t.astype(BF16)
            return carry

        jax.lax.fori_loop(0, jt_n, shift_scale_body, 0)

        def bulk_body(hp, carry):
            for cp in pair_copies(hp):
                cp.wait()

            @pl.when(hp == 0)
            def _():
                for cp in pair_copies(1) + [wo_copy(0)]:
                    cp.start()

            @pl.when(hp + 2 < hp_n)
            def _():
                for cp in pair_copies(hp + 2):
                    cp.start()

            pl.when(hp + 1 < hp_n)(lambda: wo_copy(hp + 1).start())
            slot = hp & (RING - 1)
            for w in range(3):
                def quad(i):
                    word = raw_s[w, slot, (i // 2) * dm2:(i // 2 + 1) * dm2, :]
                    return pltpu.bitcast(word & HIGH_HALF if i % 2 else word << 16, F32)

                def prod(i):
                    q = [quad(j) for j in range(4)]
                    return _dot(hb_s[i * mh:(i + 1) * mh], {1: q[0], 4: q[3], **_rhs_sums(*q)}[i].astype(BF16))

                m4 = prod(4)
                res = [t.reshape(nseg // 2, NB, dh) for t in _strassen(prod, None, m4)]
                for r in range(0, dm, 16):
                    even = raw_s[w, slot, pl.ds(r, 8, stride=2), :]
                    odd = raw_s[w, slot, pl.ds(r + 1, 8, stride=2), :]
                    wqkv[w, 2 * hp, r // 2:r // 2 + 8, :] = (even & 0xFFFF) | (odd << 16)
                    wqkv[w, 2 * hp + 1, r // 2:r // 2 + 8, :] = (even >> 16) | (odd & HIGH_HALF)
                for i in range(xs_n * w // 3, xs_n * (w + 1) // 3):
                    xs = x_s[hp * xs_n + i, NB:, :].astype(F32)
                    hx_s[hp * xs_n + i] = _layernorm(xs) * _rows(mod_s[1], seg - NB) + _rows(mod_s[0], seg - NB)
                qkvb[w, hp, :nseg // 2] = jnp.concatenate(res[:2], axis=1).astype(BF16)
                qkvb[w, hp, nseg // 2:] = jnp.concatenate(res[2:], axis=1).astype(BF16)
            return carry

        jax.lax.fori_loop(0, hp_n, bulk_body, 0)
        wait_filled(wo_s, sem_misc.at[0])
        cp_w1.start()
        pl.loop(2 * kt_n, 5 * kt_n)(lambda t: mod_copy(t, 0).start())

        exp_c = scale * math.log2(math.e)

        def head_w(w, head, t):
            return _halfs(wqkv[w, head, t * dm2 // 2:(t + 1) * dm2 // 2, :])

        def step(s, odd, mem):
            a = jnp.concatenate([mem, hx_s[s]], axis=0)
            a = [a[:, :dm2].astype(BF16), a[:, dm2:].astype(BF16)]

            first = [_dot(a[t], jnp.concatenate([head_w(w, j, t) for w in KQV for j in range(2)], axis=1))
                     for t in range(2)]

            def proj(w, hp):
                if hp == 0:
                    r = [first[0][:, _tile(n)] + first[1][:, _tile(n)]
                         for n in (2 * KQV.index(w), 2 * KQV.index(w) + 1)]
                else:
                    r = [_dot(a[0], head_w(w, head, 0)) + _dot(a[1], head_w(w, head, 1))
                         for head in (2 * hp, 2 * hp + 1)]
                return jnp.concatenate(r + [qkvb[w, hp, s].astype(F32)], axis=0).astype(BF16)

            def softmax_parts(q, k):
                fill = fill_s[...]
                sco = jnp.where(fill == 0.0, _dot_nt(q, k), fill)
                e = jnp.exp2((sco - jnp.max(sco, axis=-1, keepdims=True)) * exp_c)
                den = jnp.sum(e, axis=-1, keepdims=True)
                inv = pl.reciprocal(den, approx=True)
                return e.astype(BF16), inv * (2.0 - den * inv)

            def attend(hp, e, inv, v):
                o = _dot(e, v) * inv
                cols = slice(2 * hp * dh, 2 * (hp + 1) * dh)
                o_s[0:seg, cols] = jnp.concatenate([o[0:seg], o[seg:2 * seg]], axis=1).astype(BF16)
                ob = jnp.concatenate([o[2 * seg:2 * seg + NB], o[2 * seg + NB:]], axis=1)
                if odd:
                    o_s[seg:, cols] = jnp.concatenate([ob_s[:, cols], ob], axis=0).astype(BF16)
                else:
                    ob_s[:, cols] = ob

            val, probs = {}, {}

            def issued(t):
                hp, rem = divmod(t - LAG_QK, 3)
                if rem == 0 and 0 <= hp < hp_n:
                    probs[hp] = softmax_parts(val.pop((0, hp)), val.pop((1, hp)))
                hp, rem = divmod(t - LAG_PV, 3)
                if rem == 0 and 0 <= hp < hp_n:
                    attend(hp, *probs.pop(hp), val.pop((2, hp)))

            for hp in range(hp_n):
                for n, w in enumerate(KQV):
                    val[w, hp] = proj(w, hp)
                    issued(3 * hp + n)
            half = nh * dh // 2
            parts = []
            for part in range(2):
                assert part == 0 or not val
                lo = o_s[0:seg + 2 * NB * odd, part * half:(part + 1) * half]
                r = []
                for n in range(kt_n):
                    r.append(_dot(lo, _halfs(wo_s[n, part * half // 2:(part + 1) * half // 2, :])))
                    issued(3 * hp_n + part * kt_n + n)
                parts.append(jnp.concatenate(r, axis=1))
            acc = parts[0] + parts[1]
            att_s[odd * seg + NB:(odd + 1) * seg, :] = acc[nmem:seg]
            if odd:
                att_s[0:NB, :] = acc[seg:seg + NB]
                att_s[seg:seg + NB, :] = acc[seg + NB:]
            return acc[0:nmem]

        def residual_norm(i):
            rows = pl.ds(pl.multiple_of(i * 2 * seg, 2 * seg), 2 * seg)
            xa = x_s[pl.ds(2 * i, 2)].astype(F32).reshape(2 * seg, dm) + _rows(mod_s[2], 2 * seg) * att_s[...]
            xa_s[rows, :] = xa
            h = _layernorm(xa) * _rows(mod_s[4], 2 * seg) + _rows(mod_s[3], 2 * seg)
            h_s[rows, :] = h
            for n, t in enumerate(_lhs_terms(*_quadrants(_layernorm(h)))):
                ut_s[pl.ds(pl.multiple_of(n * (ntok // 2) + i * seg, seg), seg), :] = t.astype(BF16)

        def step_body(i, mem):
            @pl.when(i == 1)
            def _():
                cp_w1.wait()
                wait_filled(wmod_s.at[2 * kt_n:5 * kt_n], sem_mod.at[0])
                for cp in (cp_w2, cp_w3, cp_w4):
                    cp.start()
                pl.loop(5 * kt_n, 6 * kt_n)(lambda t: mod_copy(t, 1).start())
                pl.loop(2, 5)(late_mod)

            residual_norm(jnp.maximum(i - 1, 0))
            return step(2 * i + 1, 1, step(2 * i, 0, mem))

        att_s[...] = jnp.zeros(att_s.shape, F32)
        mod_s[2:] = jnp.zeros((4, 8, dm), F32)
        jax.lax.fori_loop(0, nseg // 2, step_body, mem0_s[...].astype(F32))
        wait_filled(wmod_s.at[5 * kt_n:], sem_mod.at[1])
        residual_norm(nseg // 2 - 1)
        late_mod(5)

    pl.run_scoped(
        attention,
        pltpu.VMEM((3, nh, dm2, dh), U32),
        pltpu.VMEM((3, hp_n, nseg, 2 * NB, dh), BF16),
        pltpu.VMEM((nseg, NB, dm), BF16),
        _words(7 * nseg * NB // 2, dm2),
        pltpu.VMEM((2 * (seg + NB), 2 * (seg + NB)), F32),
        pltpu.VMEM((nseg, seg - NB, dm), F32),
        _words(seg + 2 * NB, nh * dh),
        pltpu.VMEM((3, RING, dm + 32, dh), U32),
        pltpu.VMEM((kt_n, nseg * NB, 128), F32),
        pltpu.VMEM((NB, nh * dh), F32),
        pltpu.VMEM((2 * seg, dm), F32),
    )

    nch = ntok // CH
    hc = CH // 2
    ff2 = w3_s.shape[1] // 2

    def mlp(w2x_w, w3x_w, w4x_w, g_s, out_s):
        w2x_s, w3x_s, w4x_s = [w.bitcast(BF16) for w in (w2x_w, w3x_w, w4x_w)]
        zero_halo = jnp.zeros((kt_n, HALO, 128), F32)
        g_s[:, 0:HALO, :] = zero_halo
        g_s[:, HALO + ntok:, :] = zero_halo
        for cp in (cp_w2, cp_w3, cp_w4):
            cp.wait()

        def stage_a(ci, carry):
            jobs = [_weight_sum_jobs(*w, ci, nch // 2) for w in ((w2_s, w2x_s), (w3_s, w3x_s), (w4_s, w4x_s))]

            def prod1(c, n, i):
                rows = pl.ds(pl.multiple_of(i * (ntok // 2) + c * hc, hc), hc)
                return _dot(ut_s[rows, :], _rhs(w1_s, w1x_s, i, n))

            for t in range(2 * jt_n):
                c, n = 2 * ci + t // jt_n, t % jt_n
                res = [_gelu(v).reshape(hc // seg, seg, 128) for v in _strassen(functools.partial(prod1, c, n))]
                for q in range(2):
                    g_s[n + q * jt_n, pl.ds(pl.multiple_of(c * CH, CH) + HALO, CH), :] = jnp.concatenate(
                        [res[q], res[2 + q]], axis=1).reshape(CH, 128)
                for job_list in jobs:
                    _spread(job_list, t, 2 * jt_n)
            return carry

        jax.lax.fori_loop(0, nch // 2, stage_a, 0)

        def out_copy(ci):
            rows = pl.ds(pl.multiple_of(ci * CH, CH), CH)
            return pltpu.make_async_copy(out_s.at[rows], out_hbm.at[rows], sem_misc.at[8])

        def stage_b(ci, carry):
            shifts = (-1, 1, -2, 2)
            x1, u = [], []
            for half in range(2):
                r0 = pl.multiple_of(ci * CH + half * hc, hc)
                gs = jnp.concatenate(
                    [g_s[k, pl.ds(r0 + HALO + shifts[k * 4 // kt_n], hc), :] for k in range(kt_n)], axis=1)
                terms = [t.astype(BF16) for t in _lhs_terms(*_quadrants(gs))]
                res = [_strassen(lambda i: _dot(terms[i], _rhs(w2_s, w2x_s, i, n))) for n in range(jt_n)]
                hs = jnp.concatenate(
                    [jnp.concatenate([r[q] for r in res] + [r[q + 1] for r in res], axis=1) for q in (0, 2)],
                    axis=0)
                x1.append(h_s[pl.ds(r0, hc), :] + hs)
                u.append(_layernorm(x1[-1]))
            a3 = [t.astype(BF16) for t in _lhs_terms(u[0][:, :dm2], u[0][:, dm2:], u[1][:, :dm2], u[1][:, dm2:])]

            def prod3(j, i):
                return _dot(a3[i], _rhs(w3_s, w3x_s, i, j))

            early = {j: (prod3(j, 2), prod3(j, 4)) for j in range(4)}
            a4 = []
            for j in range(ff2 // 128):
                act = [_gelu(t) for t in _strassen(functools.partial(prod3, j), *early.get(j, ()))]
                a4.append(_lhs_terms(*act))
            a4 = [jnp.concatenate([t[i] for t in a4], axis=1).astype(BF16) for i in range(7)]

            def prod4(n, i):
                return _dot(a4[i], _rhs(w4_s, w4x_s, i, n))

            for n in range(jt_n):
                for q, t in enumerate(_strassen(functools.partial(prod4, n))):
                    half, cols = q // 2, _tile((q % 2) * jt_n + n)
                    rows = pl.ds(pl.multiple_of(ci * CH + half * hc, hc), hc)
                    y = x1[half][:, cols] + t
                    out_s[rows, cols] = (xa_s[rows, cols] + _rows(mod_s[5, :, cols], hc) * y).astype(BF16)
            out_copy(ci).start()
            return carry

        jax.lax.fori_loop(0, nch, stage_b, 0)
        for ci in range(nch):
            out_copy(ci).wait()

    pl.run_scoped(
        mlp,
        _words(4 * dm2, dm2),
        _words(4 * dm2, ff2),
        _words(4 * ff2, dm2),
        pltpu.VMEM((kt_n, ntok + 2 * HALO, 128), F32),
        pltpu.VMEM((ntok, dm), BF16),
    )


@functools.partial(jax.jit, static_argnames=("A_seg_len",))
def pallas_adaLN_cond__memory_aug_recurrent_mem_tr__mixer_s_mlp__prompt_kernel(
    A_x: jax.Array,
    A_mem0: jax.Array,
    A_Wq: jax.Array,
    A_Wk: jax.Array,
    A_Wv: jax.Array,
    A_Wo: jax.Array,
    A_seg_len: int,
    B_x: jax.Array,
    B_w1: jax.Array,
    B_w2: jax.Array,
    B_w3: jax.Array,
    B_w4: jax.Array,
    c: jax.Array,
    w_mod: jax.Array,
):
    del B_x
    b, s, dm = A_x.shape
    _, nh, dh = A_Wq.shape
    nmem = A_mem0.shape[1]
    seg = int(A_seg_len)
    ff = B_w3.shape[1]
    assert (b, s, dm, nh, dh, nmem, seg, ff) == (1, 2048, 1024, 32, 128, NB, 32, 3584)
    kt_n = dm // 128
    hbm = pl.BlockSpec(memory_space=pl.ANY)
    out = pl.pallas_call(
        _kernel,
        out_shape=jax.ShapeDtypeStruct((s, dm), BF16),
        in_specs=[hbm] * 12,
        out_specs=hbm,
        scratch_shapes=[
            pltpu.VMEM((kt_n, nh * dh // 2, 128), U32),
            _words(dm, dm),
            _words(dm, dm),
            _words(dm, ff),
            _words(ff, dm),
            pltpu.VMEM((6 * kt_n, dm // 2, 128), U32),
            pltpu.VMEM((s // seg, seg, dm), BF16),
            pltpu.VMEM((s, dm), F32),
            pltpu.VMEM((s, dm), F32),
            _words(7 * s // 2, dm // 2),
            _words(4 * dm // 2, dm // 2),
            pltpu.VMEM((6, 8, dm), F32),
            pltpu.VMEM((1, dm), BF16),
            pltpu.VMEM((nmem, dm), BF16),
            pltpu.SemaphoreType.DMA((RING,)),
            pltpu.SemaphoreType.DMA((9,)),
            pltpu.SemaphoreType.DMA((kt_n // 2,)),
        ],
        compiler_params=pltpu.CompilerParams(vmem_limit_bytes=127 * 1024 * 1024),
    )(A_x.reshape(s // seg, seg, dm), A_mem0.reshape(nmem, dm), A_Wq, A_Wk, A_Wv,
      A_Wo.reshape(nh * dh, dm), B_w1, B_w2, B_w3, B_w4, c, w_mod)
    return out.reshape(b, s, dm)
```
